```python
import jax
import jax.numpy as jnp

def _softmax(x, axis=-1):
    return jax.nn.softmax(x, axis=axis)
def _gelu(x):
    return jax.nn.gelu(x, approximate=True)
def _silu(x):
    return jax.nn.silu(x)
def _sigmoid(x):
    return jax.nn.sigmoid(x)
def _layernorm(x, axis=-1, eps=1e-5):
    m = jnp.mean(x, axis=axis, keepdims=True)
    v = jnp.var(x, axis=axis, keepdims=True)
    return (x - m) / jnp.sqrt(v + eps)
def _scatter_add(tgt, idx, src, axis=0):
    return tgt.at[idx].add(src)
def _segment_sum(src, seg, n):
    return jax.ops.segment_sum(src, seg, n)
class _Rng:
    def __init__(self, key):
        self._k = key
    def _next(self):
        self._k, sub = jax.random.split(self._k)
        return sub
    def normal(self, shape):
        return jax.random.normal(self._next(), shape, dtype=jnp.bfloat16)
    def randint(self, lo, hi, shape):
        return jax.random.randint(self._next(), shape, lo, hi, dtype=jnp.int32)
    def uniform(self, shape, lo=0.0, hi=1.0):
        return jax.random.uniform(self._next(), shape, jnp.bfloat16, lo, hi)
    def permutation(self, n):
        return jax.random.permutation(self._next(), n)


kernel_name = 'standalone__modern_conv_block_convnext_v2__vision'

def setup_inputs():
    _rng = _Rng(jax.random.key(int.from_bytes(__import__("os").urandom(4), "little")))
    _w = (lambda a: (lambda t: t.astype(jnp.bfloat16) if jnp.issubdtype(t.dtype, jnp.floating) else t)(jnp.asarray(a)))
    H = W = 512
    C = 96
    K = 3
    return {
        "x": _w((lambda *s: _rng.normal(s) * 0.05)(1, H, W, C)),
        "dw": _w((lambda *s: _rng.normal(s) * 0.05)(K, K, C)),
        "w1": _w((lambda *s: _rng.normal(s) * 0.05)(C, 4 * C)),
        "w2": _w((lambda *s: _rng.normal(s) * 0.05)(4 * C, C)),
        "grn_gamma": _w((lambda *s: _rng.normal(s) * 0.05)(4 * C)),
        "grn_beta": _w((lambda *s: _rng.normal(s) * 0.05)(4 * C)),
    }

def reference(x, dw, w1, w2, grn_gamma, grn_beta):
    B, H, W, C = x.shape
    K = dw.shape[0]
    pad = K // 2
    xp = jnp.pad(x, ((0,0),(pad,pad),(pad,pad),(0,0)))
    out = jnp.zeros_like(x)
    for i in range(K):
        for j in range(K):
            out = out + xp[:, i:i+H, j:j+W, :] * dw[i, j][None, None, None, :]
    h = _layernorm(out, axis=-1)
    h = jnp.einsum('bhwc,ce->bhwe', h, w1)
    h = _gelu(h)
    gx = jnp.sqrt((h * h).sum(axis=(1, 2), keepdims=True) + 1e-6)
    nx = gx / (gx.mean(axis=-1, keepdims=True) + 1e-6)
    h = grn_gamma * (h * nx) + grn_beta + h
    h = jnp.einsum('bhwe,ec->bhwc', h, w2)
    return x + h
```

```python
import math
import jax
import jax.numpy as jnp
from jax import lax
from jax.experimental import pallas as pl
from jax.experimental.pallas import tpu as pltpu

H = 512
W = 512
C = 96
E = 384
G = C // 8
NT = W // 128
TB = 8
NB = H // TB
NQ = TB // 2
REC = (1, 2, 3)
STO = tuple(r for r in range(TB) if r not in REC)
NSTO = len(STO)
NREC = len(REC)
EH = E // 2
CH = C // 2
SROWS = G * 24
NCH = 2
P2ORDER = "a"
NBH = NB

C0 = math.sqrt(2.0 / math.pi)
C1 = 0.044715
GA = (C0 * C1) ** (1.0 / 3.0)
GK = C0 / GA
LN_EPS = 1e-5

f32 = jnp.float32
bf16 = jnp.bfloat16
u32 = jnp.uint32


def _pack(v):
    return pltpu.bitcast(v.astype(bf16), u32)


def _unp(v):
    return pltpu.bitcast(v, bf16)


def _shift_r(a):
    lane = lax.broadcasted_iota(jnp.int32, (a.shape[0], 128), 1)
    r = [pltpu.roll(a[:, t * 128:(t + 1) * 128], 1, 1) for t in range(NT)]
    return jnp.concatenate(
        [jnp.where(lane == 0, r[t - 1] if t > 0 else jnp.zeros_like(r[t]), r[t]) for t in range(NT)], axis=1)


def _shift_l(a):
    lane = lax.broadcasted_iota(jnp.int32, (a.shape[0], 128), 1)
    r = [pltpu.roll(a[:, t * 128:(t + 1) * 128], 127, 1) for t in range(NT)]
    return jnp.concatenate(
        [jnp.where(lane == 127, r[t + 1] if t < NT - 1 else jnp.zeros_like(r[t]), r[t]) for t in range(NT)], axis=1)


def _tile4(v):
    return jnp.concatenate([v] * NT, axis=1)


def _merge(a, b, sh):
    sub = lax.broadcasted_iota(jnp.int32, (8, 128), 0)
    lo = (sub & sh) == 0
    p = jnp.where(lo, a, b)
    q = jnp.where(lo, b, a)
    if sh == 4:
        return p + pltpu.roll(q, 4, 0)
    raise NotImplementedError


def _rstd2(c0, c1):
    def sums(c):
        s1 = c[0]
        s2 = c[0] * c[0]
        for g in range(1, G):
            s1 = s1 + c[g]
            s2 = s2 + c[g] * c[g]
        return s1, s2
    a1, a2 = sums(c0)
    b1, b2 = sums(c1)
    m1 = _merge(a1, b1, 4)
    m2 = _merge(a2, b2, 4)
    sub = lax.broadcasted_iota(jnp.int32, (8, 128), 0)
    lo = (sub & 2) == 0
    n = jnp.where(lo, m1 + pltpu.roll(m1, 6, 0), m2 + pltpu.roll(m2, 2, 0))
    n = n + jnp.where((sub & 1) == 0, pltpu.roll(n, 7, 0), pltpu.roll(n, 1, 0))
    mean = n * (1.0 / (C * GA))
    msq = pltpu.roll(mean * mean, 2, 0)
    var = jnp.maximum(n * (1.0 / (C * GA * GA)) - msq, 0.0) + LN_EPS / (GA * GA)
    rstd = lax.rsqrt(var)
    return jnp.broadcast_to(rstd[2:3], (8, 128)), jnp.broadcast_to(rstd[6:7], (8, 128))


def _rstd1(c):
    s1 = c[0]
    s2 = c[0] * c[0]
    for g in range(1, G):
        s1 = s1 + c[g]
        s2 = s2 + c[g] * c[g]
    n = _merge(s1, s2, 4)
    sub = lax.broadcasted_iota(jnp.int32, (8, 128), 0)
    n = n + jnp.where((sub & 2) == 0, pltpu.roll(n, 6, 0), pltpu.roll(n, 2, 0))
    n = n + jnp.where((sub & 1) == 0, pltpu.roll(n, 7, 0), pltpu.roll(n, 1, 0))
    mean = n * (1.0 / (C * GA))
    msq = pltpu.roll(mean * mean, 4, 0)
    var = jnp.maximum(n * (1.0 / (C * GA * GA)) - msq, 0.0) + LN_EPS / (GA * GA)
    rstd = lax.rsqrt(var)
    return jnp.broadcast_to(rstd[4:5], (8, 128))


def _gelu2(y):
    u = y * (y * y + GK)
    return y * (jnp.tanh(u) + 1.0)


def kernel(x_hbm, dw_ref, w1_ref, w2t_ref, gam_ref, bet_ref, o_hbm,
           hbuf, dwb, dmat, w1s, w2s, biasb, acc):

    def w1t(c0=0, n=E):
        return _unp(w1s[c0 // 2:(c0 + n) // 2, :])[:, :C]

    def setup():
        sub = lax.broadcasted_iota(jnp.int32, (C, C), 0)
        lan = lax.broadcasted_iota(jnp.int32, (C, C), 1)
        eye = sub == lan
        for i in range(3):
            for j in range(3):
                row = dw_ref[i, j:j + 1, :].astype(f32)
                col = jnp.sum(jnp.where(eye, jnp.broadcast_to(row, (C, C)), 0.0), axis=1, keepdims=True)
                dwb[i * 3 + j] = jnp.broadcast_to(col, (C, 128))
        c_ = lax.broadcasted_iota(jnp.int32, (8, 128), 0)
        k_ = lax.broadcasted_iota(jnp.int32, (8, 128), 1)
        for g in range(G):
            halves = []
            for o in range(2):
                d = jnp.zeros((8, 128), f32)
                for i in range(3):
                    ri = i + o
                    for j in range(3):
                        kpos = (ri // 2) * 48 + j * 16 + (ri % 2) * 8
                        d = jnp.where(k_ == c_ + kpos, dwb[i * 3 + j, 8 * g:8 * g + 8, :], d)
                halves.append(d)
            dmat[8 * g:8 * g + 8, :] = _pack(jnp.concatenate(halves, axis=0))
        w1f = w1_ref[...].astype(f32)
        w1c = w1f - jnp.sum(w1f, axis=0, keepdims=True) * (1.0 / C)
        w1p = jnp.concatenate([w1c, jnp.zeros((128 - C, E), f32)], axis=0)
        w1s[...] = _pack(w1p.T)
        acc[...] = jnp.zeros_like(acc)

    def scope1(xb1, sbuf, xns, sem1):
        def lo(j, slot):
            return pltpu.make_async_copy(x_hbm.at[pl.ds(NQ * j - 1, NQ), 1],
                                         xb1.at[slot, :, :, pl.ds(0, 8), :], sem1.at[slot, 0])

        def hi(j, slot):
            return pltpu.make_async_copy(x_hbm.at[pl.ds(NQ * j, NQ), 0],
                                         xb1.at[slot, :, :, pl.ds(8, 8), :], sem1.at[slot, 1])

        def lo_first():
            return pltpu.make_async_copy(x_hbm.at[pl.ds(0, NQ - 1), 1],
                                         xb1.at[0, pl.ds(1, NQ - 1), :, pl.ds(0, 8), :], sem1.at[0, 0])

        def lo_last():
            return pltpu.make_async_copy(x_hbm.at[pl.ds(NQ * NB - 1, 1), 1],
                                         xb1.at[NB % 2, pl.ds(0, 1), :, pl.ds(0, 8), :], sem1.at[NB % 2, 0])

        def build(slot, k):
            for g in range(G):
                v = pltpu.bitcast(xb1[slot, k, g], u32)
                base = k * SROWS + g * 24
                sbuf[base:base + 8, :] = _shift_r(v)
                sbuf[base + 8:base + 16, :] = v
                sbuf[base + 16:base + 24, :] = _shift_l(v)

        def conv_ln(s0, t):
            ts = slice(t * 128, (t + 1) * 128)
            cv = []
            for g in range(G):
                b0 = (s0 % NQ) * SROWS + g * 24
                b1 = ((s0 + 1) % NQ) * SROWS + g * 24
                s = _unp(jnp.concatenate([sbuf[b0:b0 + 24, ts], sbuf[b1:b1 + 24, ts]], axis=0))
                d = _unp(dmat[8 * g:8 * g + 8, :])[:, :C]
                cv.append(jnp.dot(d, s, preferred_element_type=f32))
            c0 = [v[0:8] for v in cv]
            c1 = [v[8:16] for v in cv]
            r0, r1 = _rstd2(c0, c1)
            r = 2 * (s0 % NQ)
            xns[r * CH:(r + 1) * CH, ts] = _pack(jnp.concatenate([c * r0 for c in c0], axis=0))
            xns[(r + 1) * CH:(r + 2) * CH, ts] = _pack(jnp.concatenate([c * r1 for c in c1], axis=0))

        lo_first().start()
        hi(0, 0).start()
        lo(1, 1).start()
        hi(1, 1).start()
        setup()
        xb1[0, 0, :, 0:8, :] = jnp.zeros((G, 8, W), bf16)
        lo_first().wait()
        hi(0, 0).wait()
        for k in range(NQ):
            build(0, k)
        for t in range(NT):
            conv_ln(0, t)
        for t in range(NT):
            conv_ln(1, t)

        def pass1(b, carry):
            slot = (b + 1) % 2

            @pl.when(b + 1 < NB)
            def _():
                lo(b + 1, slot).wait()
                hi(b + 1, slot).wait()

            @pl.when(b + 1 == NB)
            def _():
                lo_last().wait()
                xb1[NB % 2, 0, :, 8:16, :] = jnp.zeros((G, 8, W), bf16)

            @pl.when(b + 2 < NB)
            def _():
                lo(b + 2, 1 - slot).start()
                hi(b + 2, 1 - slot).start()

            @pl.when(b + 2 == NB)
            def _():
                lo_last().start()

            def mm1(r, c):
                n = E // NCH
                y = jnp.dot(w1t(c * n, n), _unp(xns[r * CH:(r + 1) * CH, :]), preferred_element_type=f32)
                h = _gelu2(y)
                h2 = h * h
                acc[c * n:(c + 1) * n, :] += (h2[:, 0:128] + h2[:, 128:256]) + (h2[:, 256:384] + h2[:, 384:512])
                if r in STO:
                    row0 = pl.multiple_of(((b % NBH) * NSTO + STO.index(r)) * EH + c * (n // 2), 8)
                    hbuf[pl.ds(row0, n // 2), :] = _pack(h)

            for k in range(NQ):
                tiles = list(range(NT))
                if CONVFIRST:
                    for o in range(2):
                        for c in range(NCH):
                            if tiles:
                                conv_ln(k + 2, tiles.pop(0))
                            mm1(2 * k + o, c)
                else:
                    for o in range(2):
                        for c in range(NCH):
                            mm1(2 * k + o, c)
                            if tiles:
                                conv_ln(k + 2, tiles.pop(0))
                build(slot, k)
            return carry

        lax.fori_loop(0, NB, pass1, 0)

    pl.run_scoped(scope1,
                  pltpu.VMEM((2, NQ, G, 16, W), bf16),
                  pltpu.VMEM((NQ * SROWS, W), u32),
                  pltpu.VMEM((TB * CH, W), u32),
                  pltpu.SemaphoreType.DMA((2, 2)))

    def scope2(xb2, ob, hre, cbuf, sem2, semo):
        def in2(b, slot):
            return pltpu.make_async_copy(x_hbm.at[pl.ds(NQ * b, NQ)], xb2.at[slot], sem2.at[slot])

        def out2(b, slot):
            return pltpu.make_async_copy(ob.at[slot], o_hbm.at[pl.ds(NQ * b, NQ)], semo.at[slot])

        def conv_rec(slot):
            for g in range(G):
                q0 = REC[0] - 1
                xs = [xb2[slot, q // 2, q % 2, g].astype(f32) for q in range(q0, REC[-1] + 2)]
                wt = [_tile4(dwb[tap, 8 * g:8 * g + 8, :]) for tap in range(9)]
                for k, r in enumerate(REC):
                    a = []
                    for j in range(3):
                        t = xs[r - 1 - q0] * wt[j]
                        t = t + xs[r - q0] * wt[3 + j]
                        t = t + xs[r + 1 - q0] * wt[6 + j]
                        a.append(t)
                    cbuf[k * C + 8 * g:k * C + 8 * g + 8, :] = _shift_r(a[0]) + a[1] + _shift_l(a[2])

        def ln_rec(k):
            cols = []
            for t in range(NT):
                c = [cbuf[k * C + 8 * g:k * C + 8 * g + 8, t * 128:(t + 1) * 128] for g in range(G)]
                r = _rstd1(c)
                cols.append(jnp.concatenate([v * r for v in c], axis=0).astype(bf16))
            return jnp.concatenate(cols, axis=1)

        in2(0, 0).start()
        in2(1, 1).start()
        ssq = jnp.sum(acc[...].T, axis=0, keepdims=True) * (1.0 / (4.0 * GA * GA))
        gx = jnp.sqrt(ssq + 1e-6)
        nx = gx / (jnp.sum(gx, axis=1, keepdims=True) * (1.0 / E) + 1e-6)
        gam = gam_ref[...].astype(f32).reshape(1, E)
        bet = bet_ref[...].astype(f32).reshape(1, E)
        scale = (gam * nx + 1.0) * (1.0 / (2.0 * GA))
        w2f = w2t_ref[...].astype(f32)
        w2s[...] = _pack(w2f * scale)
        biasb[...] = jnp.broadcast_to(jnp.sum(w2f * bet, axis=1, keepdims=True), (C, 128))
        in2(0, 0).wait()
        conv_rec(0)

        def pass2(b, carry):
            slot = b % 3
            nslot = (b + 1) % 3
            oslot = b % 2

            @pl.when(b + 1 < NB)
            def _():
                in2(b + 1, nslot).wait()

            @pl.when(b + 2 < NB)
            def _():
                in2(b + 2, (b + 2) % 3).start()

            @pl.when(b >= 2)
            def _():
                out2(b - 2, oslot).wait()

            def finish(r, hp):
                o = jnp.dot(_unp(w2s[...]), _unp(hp), preferred_element_type=f32)
                for g in range(G):
                    xr = xb2[slot, r // 2, r % 2, g].astype(f32)
                    v = o[8 * g:8 * g + 8, :] + (xr + _tile4(biasb[8 * g:8 * g + 8, :]))
                    ob[oslot, r // 2, r % 2, g] = v.astype(bf16)

            def rec(k):
                y = jnp.dot(w1t(), ln_rec(k), preferred_element_type=f32)
                hre[k * EH:(k + 1) * EH, :] = _pack(_gelu2(y))

            def sto(k):
                row0 = pl.multiple_of(((b % NBH) * NSTO + k) * EH, 8)
                finish(STO[k], hbuf[pl.ds(row0, EH), :])

            def fin(k):
                finish(REC[k], hre[k * EH:(k + 1) * EH, :])

            seq = {"a": "s0 r0 r1 r2 c s1 s2 s3 s4 f0 f1 f2",
                   "b": "s0 r0 s1 r1 s2 r2 c s3 f0 s4 f1 f2",
                   "c": "s0 r0 s1 r1 f0 s2 r2 c f1 s3 s4 f2",
                   }[P2ORDER]
            for tok in seq.split():
                if tok == "c":
                    conv_rec(nslot)
                else:
                    {"s": sto, "r": rec, "f": fin}[tok[0]](int(tok[1]))

            out2(b, oslot).start()
            return carry

        lax.fori_loop(0, NB, pass2, 0)
        out2(NB - 2, 0).wait()
        out2(NB - 1, 1).wait()

    pl.run_scoped(scope2,
                  pltpu.VMEM((3, NQ, 2, G, 8, W), bf16),
                  pltpu.VMEM((2, NQ, 2, G, 8, W), bf16),
                  pltpu.VMEM((NREC * EH, W), u32),
                  pltpu.VMEM((NREC * C, W), f32),
                  pltpu.SemaphoreType.DMA((3,)),
                  pltpu.SemaphoreType.DMA((2,)))


CONVFIRST = "0" == "1"


@jax.jit
def pallas_standalone__modern_conv_block_convnext_v2__vision_kernel(x, dw, w1, w2, grn_gamma, grn_beta):
    xt = jnp.transpose(x, (0, 1, 3, 2)).reshape(H // 2, 2, G, 8, W)
    w2t = w2.T
    vm = pl.BlockSpec(memory_space=pltpu.VMEM)
    o = pl.pallas_call(
        kernel,
        out_shape=jax.ShapeDtypeStruct((H // 2, 2, G, 8, W), bf16),
        in_specs=[pl.BlockSpec(memory_space=pl.ANY), vm, vm, vm, vm, vm],
        out_specs=pl.BlockSpec(memory_space=pl.ANY),
        scratch_shapes=[
            pltpu.VMEM((NBH * NSTO * EH, W), u32),
            pltpu.VMEM((9, C, 128), f32),
            pltpu.VMEM((C, 128), u32),
            pltpu.VMEM((EH, 128), u32),
            pltpu.VMEM((CH, E), u32),
            pltpu.VMEM((C, 128), f32),
            pltpu.VMEM((E, 128), f32),
        ],
        compiler_params=pltpu.CompilerParams(vmem_limit_bytes=128 * 1024 * 1024),
        name="convnext",
    )(xt, dw, w1, w2t, grn_gamma, grn_beta)
    return jnp.transpose(o.reshape(1, H, C, W), (0, 1, 3, 2))
```

```python
import math
import jax
import jax.numpy as jnp
from jax import lax
from jax.experimental import pallas as pl
from jax.experimental.pallas import tpu as pltpu

H = 512
W = 512
C = 96
E = 384
G = C // 8
NT = W // 128
TB = 8
NB = H // TB
NQ = TB // 2
REC = tuple(int(ch) for ch in "123")
STO = tuple(r for r in range(TB) if r not in REC)
NSTO = len(STO)
NREC = len(REC)
EH = E // 2
CH = C // 2
SROWS = G * 24
NCH = 2
U1 = 2
PB = NQ * U1
NI = NB // U1
U2 = 1
P2ORDER = "f"
PADV = 7
TIE = 16
NOBC = "1" == "1"

C0 = math.sqrt(2.0 / math.pi)
C1 = 0.044715
GA = (C0 * C1) ** (1.0 / 3.0)
GK = C0 / GA
LN_EPS = 1e-5

f32 = jnp.float32
bf16 = jnp.bfloat16
u32 = jnp.uint32


def _pack(v):
    return pltpu.bitcast(v.astype(bf16), u32)


def _unp(v):
    return pltpu.bitcast(v, bf16)


def _shift_r(a):
    lane = lax.broadcasted_iota(jnp.int32, (a.shape[0], 128), 1)
    r = [pltpu.roll(a[:, t * 128:(t + 1) * 128], 1, 1) for t in range(NT)]
    return jnp.concatenate(
        [jnp.where(lane == 0, r[t - 1] if t > 0 else jnp.zeros_like(r[t]), r[t]) for t in range(NT)], axis=1)


def _shift_l(a):
    lane = lax.broadcasted_iota(jnp.int32, (a.shape[0], 128), 1)
    r = [pltpu.roll(a[:, t * 128:(t + 1) * 128], 127, 1) for t in range(NT)]
    return jnp.concatenate(
        [jnp.where(lane == 127, r[t + 1] if t < NT - 1 else jnp.zeros_like(r[t]), r[t]) for t in range(NT)], axis=1)


def _tile4(v):
    return jnp.concatenate([v] * NT, axis=1)


def _sums(c):
    s1 = c[0]
    s2 = c[0] * c[0]
    for g in range(1, G):
        s1 = s1 + c[g]
        s2 = s2 + c[g] * c[g]
    return s1, s2


def _merge4(a, b):
    lo = lax.broadcasted_iota(jnp.int32, (8, 128), 0) < 4
    return jnp.where(lo, a, b) + pltpu.roll(jnp.where(lo, b, a), 4, 0)


def _var_from(n, shift):
    eps = LN_EPS / (GA * GA)
    mean = n * (1.0 / (C * GA))
    msq = pltpu.roll(mean * mean, shift, 0)
    return jnp.maximum(n * (1.0 / (C * GA * GA)) + eps - msq, eps)


def _rstd_from(n, shift):
    return lax.rsqrt(_var_from(n, shift))


def _var2(c0, c1):
    a1, a2 = _sums(c0)
    b1, b2 = _sums(c1)
    m1 = _merge4(a1, b1)
    m2 = _merge4(a2, b2)
    sub = lax.broadcasted_iota(jnp.int32, (8, 128), 0)
    n = jnp.where((sub & 2) == 0, m1 + pltpu.roll(m1, 6, 0), m2 + pltpu.roll(m2, 2, 0))
    n = n + pltpu.roll(n, 1, 0)
    return _var_from(n, 2)


def _rstd1(c):
    s1, s2 = _sums(c)
    n = _merge4(s1, s2)
    n = n + pltpu.roll(n, 2, 0)
    n = n + pltpu.roll(n, 1, 0)
    rstd = _rstd_from(n, 4)
    return jnp.broadcast_to(rstd[7:8], (8, 128))


def _gelu2(y):
    u = y * (y * y + GK)
    return y * (jnp.tanh(u) + 1.0)


def kernel(x_hbm, dw_ref, w1_ref, w2t_ref, gam_ref, bet_ref, o_hbm,
           hbuf, dwb, dmat, w1s, acc, w2s, pad0, zs):
    zs[0] = 0
    pad0[...] = jnp.zeros_like(pad0)

    def w1t(c0=0, n=E):
        return _unp(w1s[c0 // 2:(c0 + n) // 2, :])[:, :C]

    def setup():
        sub = lax.broadcasted_iota(jnp.int32, (C, C), 0)
        lan = lax.broadcasted_iota(jnp.int32, (C, C), 1)
        eye = sub == lan
        for i in range(3):
            for j in range(3):
                row = dw_ref[i, j:j + 1, :].astype(f32)
                col = jnp.sum(jnp.where(eye, jnp.broadcast_to(row, (C, C)), 0.0), axis=1, keepdims=True)
                dwb[i * 3 + j] = jnp.broadcast_to(col, (C, 128))
        c_ = lax.broadcasted_iota(jnp.int32, (8, 128), 0)
        k_ = lax.broadcasted_iota(jnp.int32, (8, 128), 1)
        for g in range(G):
            halves = []
            for o in range(2):
                d = jnp.zeros((8, 128), f32)
                for i in range(3):
                    ri = i + o
                    for j in range(3):
                        kpos = (ri // 2) * 48 + j * 16 + (ri % 2) * 8
                        d = jnp.where(k_ == c_ + kpos, dwb[i * 3 + j, 8 * g:8 * g + 8, :], d)
                halves.append(d)
            dmat[8 * g:8 * g + 8, :] = _pack(jnp.concatenate(halves, axis=0))
        w1f = w1_ref[...].astype(f32)
        w1c = w1f - jnp.sum(w1f, axis=0, keepdims=True) * (1.0 / C)
        w1p = jnp.concatenate([w1c, jnp.zeros((128 - C, E), f32)], axis=0)
        w1s[...] = _pack(w1p.T)
        acc[...] = jnp.zeros_like(acc)

    def scope1(xb1, sbuf, xns, sem1):
        def halves(p0, n_lo, n_hi, slot, skip_lo=0):
            cps = []
            if n_lo:
                cps.append(pltpu.make_async_copy(
                    x_hbm.at[pl.ds(p0 - 1 + skip_lo, n_lo), 1],
                    xb1.at[slot, pl.ds(skip_lo, n_lo), :, pl.ds(0, 8), :], sem1.at[slot, 0]))
            if n_hi:
                cps.append(pltpu.make_async_copy(
                    x_hbm.at[pl.ds(p0, n_hi), 0],
                    xb1.at[slot, pl.ds(0, n_hi), :, pl.ds(8, 8), :], sem1.at[slot, 1]))
            return cps

        def grp_head():
            return halves(0, NQ - 1, NQ, 1, skip_lo=1)

        def grp(i, slot):
            return halves(PB * i + NQ, PB, PB, slot)

        def grp_last():
            return halves(PB * (NI - 1) + NQ, PB - 3, PB - 4, (NI - 1) % 2)

        def build(slot, k):
            for g in range(G):
                v = pltpu.bitcast(xb1[slot, k, g], u32)
                base = (k % NQ) * SROWS + g * 24
                sbuf[base:base + 8, :] = _shift_r(v)
                sbuf[base + 8:base + 16, :] = v
                sbuf[base + 16:base + 24, :] = _shift_l(v)

        def conv_var(s0, t):
            ts = slice(t * 128, (t + 1) * 128)
            cv = []
            for g in range(G):
                b0 = (s0 % NQ) * SROWS + g * 24
                b1 = ((s0 + 1) % NQ) * SROWS + g * 24
                s = _unp(jnp.concatenate([sbuf[b0:b0 + 24, ts], sbuf[b1:b1 + 24, ts]], axis=0))
                d = _unp(dmat[8 * g:8 * g + 8, :])[:, :C]
                cv.append(jnp.dot(d, s, preferred_element_type=f32))
            c0 = [v[0:8] for v in cv]
            c1 = [v[8:16] for v in cv]
            return (s0, t, c0, c1, _var2(c0, c1))

        def norm(st, tie=None):
            s0, t, c0, c1, var = st
            if tie is not None:
                never = lax.broadcasted_iota(jnp.int32, (8, 128), 0) < zs[0]
                var = jnp.where(never, tie, var)
            rstd = lax.rsqrt(var)
            r0 = jnp.broadcast_to(rstd[3:4], (8, 128))
            r1 = jnp.broadcast_to(rstd[7:8], (8, 128))
            ts = slice(t * 128, (t + 1) * 128)
            r = 2 * (s0 % NQ)
            xns[r * CH:(r + 1) * CH, ts] = _pack(jnp.concatenate([c * r0 for c in c0], axis=0))
            xns[(r + 1) * CH:(r + 2) * CH, ts] = _pack(jnp.concatenate([c * r1 for c in c1], axis=0))

        for cp in grp_head() + grp(0, 0):
            cp.start()
        setup()
        xb1[1, 0, :, 0:8, :] = jnp.zeros((G, 8, W), bf16)
        for cp in grp_head():
            cp.wait()
        for k in range(NQ):
            build(1, k)
        for s0 in range(2):
            for t in range(NT):
                norm(conv_var(s0, t))

        def dma1(i, slot):
            @pl.when(i < NI - 1)
            def _():
                for cp in grp(i, slot):
                    cp.wait()

            @pl.when(i == NI - 1)
            def _():
                for cp in grp_last():
                    cp.wait()
                xb1[(NI - 1) % 2, PB - 4, :, 8:16, :] = jnp.zeros((G, 8, W), bf16)

            @pl.when(i + 1 < NI - 1)
            def _():
                for cp in grp(i + 1, 1 - slot):
                    cp.start()

            @pl.when(i + 1 == NI - 1)
            def _():
                for cp in grp_last():
                    cp.start()

        def block1(b, slot, u, pend):
            def mm1(r, c):
                n = E // NCH
                y = jnp.dot(w1t(c * n, n), _unp(xns[r * CH:(r + 1) * CH, :]), preferred_element_type=f32)
                h = _gelu2(y)
                h2 = h * h
                acc[c * n:(c + 1) * n, :] += (h2[:, 0:128] + h2[:, 128:256]) + (h2[:, 256:384] + h2[:, 384:512])
                if r in STO:
                    row0 = pl.multiple_of((b * NSTO + STO.index(r)) * EH + c * (n // 2), 8)
                    hbuf[pl.ds(row0, n // 2), :] = _pack(h)
                return y

            for k in range(NQ):
                tiles = list(range(NT))
                for o in range(2):
                    for c in range(NCH):
                        y = mm1(2 * k + o, c)
                        if pend is not None:
                            norm(pend, y[TIE:TIE + 8, 0:128])
                        pend = conv_var(k + 2, tiles.pop(0))
                build(slot, u * NQ + k)
            return pend

        def pass1(i, carry):
            slot = i & 1
            dma1(i, slot)
            pend = None
            for u in range(U1):
                pend = block1(i * U1 + u, slot, u, pend)
            norm(pend)
            return carry

        lax.fori_loop(0, NB // U1, pass1, 0)

    pl.run_scoped(scope1,
                  pltpu.VMEM((2, PB, G, 16, W), bf16),
                  pltpu.VMEM((NQ * SROWS, W), u32),
                  pltpu.VMEM((TB * CH, W), u32),
                  pltpu.SemaphoreType.DMA((2, 2)))

    def scope2(xb2, ob, hre, cbuf, sem2, semo):
        def in2(b, slot):
            return pltpu.make_async_copy(x_hbm.at[pl.ds(NQ * b, NQ)], xb2.at[slot], sem2.at[slot])

        def out2(b, slot, half):
            return pltpu.make_async_copy(ob.at[slot, pl.ds(2 * half, 2)],
                                         o_hbm.at[pl.ds(NQ * b + 2 * half, 2)], semo.at[slot, half])

        def conv_rec(slot, groups=range(G)):
            for g in groups:
                need = sorted({r + d for r in REC for d in (-1, 0, 1)})
                xs = {q: xb2[slot, q // 2, q % 2, g].astype(f32) for q in need}
                wt = [_tile4(dwb[tap, 8 * g:8 * g + 8, :]) for tap in range(9)]
                for k, r in enumerate(REC):
                    a = []
                    for j in range(3):
                        t = xs[r - 1] * wt[j]
                        t = t + xs[r] * wt[3 + j]
                        t = t + xs[r + 1] * wt[6 + j]
                        a.append(t)
                    cbuf[(k + 1) * C + 8 * g:(k + 1) * C + 8 * g + 8, :] = _shift_r(a[0]) + a[1] + _shift_l(a[2])

        def ln_rec(k):
            cols = []
            for t in range(NT):
                c = [cbuf[(k + 1) * C + 8 * g:(k + 1) * C + 8 * g + 8, t * 128:(t + 1) * 128] for g in range(G)]
                r = _rstd1(c)
                cols.append(jnp.concatenate([v * r for v in c], axis=0))
            return jnp.concatenate(cols, axis=1).astype(bf16)

        in2(0, 0).start()
        in2(1, 1).start()
        ssq = jnp.sum(acc[...].T, axis=0, keepdims=True) * (1.0 / (4.0 * GA * GA))
        gx = jnp.sqrt(ssq + 1e-6)
        nx = gx / (jnp.sum(gx, axis=1, keepdims=True) * (1.0 / E) + 1e-6)
        gam = gam_ref[...].astype(f32).reshape(1, E)
        bet = bet_ref[...].astype(f32).reshape(1, E)
        scale = (gam * nx + 1.0) * (1.0 / (2.0 * GA))
        w2f = w2t_ref[...].astype(f32)
        w2s[...] = _pack(w2f * scale)
        cbuf[0:C, :] = jnp.broadcast_to(jnp.sum(w2f * bet, axis=1, keepdims=True), (C, W))
        in2(0, 0).wait()
        conv_rec(0)

        def block2(b, slot, oslot, dma=3):
            nslot = jnp.where(slot == 2, 0, slot + 1)
            pslot = jnp.where(slot == 0, 2, slot - 1)

            def wait_in():
                @pl.when(b + 1 < NB)
                def _():
                    in2(b + 1, nslot).wait()

            def start_in():
                @pl.when(b + 2 < NB)
                def _():
                    in2(b + 2, pslot).start()

            def wait_out(half):
                @pl.when(b >= 2)
                def _():
                    out2(b - 2, oslot, half).wait()

            def mm2(hp):
                return jnp.dot(_unp(w2s[...]), _unp(hp), preferred_element_type=f32)

            def finish(r, o):
                for g in range(G):
                    xr = xb2[slot, r // 2, r % 2, g].astype(f32)
                    v = o[8 * g:8 * g + 8, :] + (xr + cbuf[pl.ds(pl.multiple_of(zs[0] + 8 * g, 8), 8), :])
                    ob[oslot, r // 2, r % 2, g] = v.astype(bf16)

            def rec(k):
                y = jnp.dot(w1t(), ln_rec(k), preferred_element_type=f32)
                hre[k * EH:(k + 1) * EH, :] = _pack(_gelu2(y))

            def sto_mm(k):
                row0 = pl.multiple_of((b * NSTO + k) * EH, 8)
                return mm2(hbuf[pl.ds(row0, EH), :])

            def sto(k):
                finish(STO[k], sto_mm(k))

            def fin(k):
                finish(REC[k], mm2(hre[pl.ds(pl.multiple_of(zs[0] + k * EH, 8), EH), :]))

            rec_hi = [k for k in range(NREC) if REC[k] >= NQ]
            rec_lo = [k for k in range(NREC) if REC[k] < NQ]
            sto_hi = [k for k in range(NSTO) if STO[k] >= NQ]
            sto_lo = [k for k in range(NSTO) if STO[k] < NQ]
            first = sto_lo.pop(0)
            tail = ([f"s{k}" for k in sto_hi] + [f"f{k}" for k in rec_hi] + ["o"]
                    + [f"s{k}" for k in sto_lo] + [f"f{k}" for k in rec_lo])
            cs = ["c03", "c36", "c69", "c9c"]
            mixed = []
            for tok in tail:
                mixed.append(tok)
                if tok != "o" and cs:
                    mixed.append(cs.pop(0))
            seq = " ".join(["I W0 W1 J", f"s{first}"] + [f"r{k}" for k in rec_hi + rec_lo] + mixed)
            for tok in seq.split():
                if tok in "IJ" and not dma & 1 or tok[0] in "Wo" and not dma & 2:
                    continue
                if tok[0] == "c":
                    conv_rec(nslot, range(int(tok[1], 16), int(tok[2], 16)))
                elif tok == "o":
                    out2(b, oslot, 1).start()
                elif tok == "I":
                    start_in()
                elif tok == "J":
                    wait_in()
                elif tok[0] == "W":
                    wait_out(int(tok[1]))
                elif tok == "S0":
                    o = sto_mm(0)
                    start_in()
                    wait_out(0)
                    finish(STO[0], o)
                else:
                    {"s": sto, "r": rec, "f": fin}[tok[0]](int(tok[1]))
            if dma & 2:
                out2(b, oslot, 0).start()
            return nslot

        def pass2(i, slot, dma=3):
            for u in range(U2):
                b = i * U2 + u
                oslot = (u % 2) if U2 % 2 == 0 else (b & 1)
                slot = block2(b, slot, oslot, dma)
            return slot

        lax.fori_loop(0, NB // U2, pass2, jnp.int32(0))
        for hf in range(2):
            out2(NB - 2, 0, hf).wait()
            out2(NB - 1, 1, hf).wait()
        x2 = 9
        if x2 < 9:
            if x2 & 1:
                in2(1, 1).start()
            lax.fori_loop(0, NB // U2, functools.partial(pass2, dma=x2), jnp.int32(0))
            if x2 & 2:
                for hf in range(2):
                    out2(NB - 2, 0, hf).wait()
                    out2(NB - 1, 1, hf).wait()

    pl.run_scoped(scope2,
                  pltpu.VMEM((3, NQ, 2, G, 8, W), bf16),
                  pltpu.VMEM((2, NQ, 2, G, 8, W), bf16),
                  pltpu.VMEM((NREC * EH, W), u32),
                  pltpu.VMEM(((NREC + 1) * C, W), f32),
                  pltpu.SemaphoreType.DMA((3,)),
                  pltpu.SemaphoreType.DMA((2, 2)))


@jax.jit
def pallas_standalone__modern_conv_block_convnext_v2__vision_kernel(x, dw, w1, w2, grn_gamma, grn_beta):
    xt = jnp.transpose(x, (0, 1, 3, 2)).reshape(H // 2, 2, G, 8, W)
    w2t = w2.T
    vm = pl.BlockSpec(memory_space=pltpu.VMEM)
    o = pl.pallas_call(
        kernel,
        out_shape=jax.ShapeDtypeStruct((H // 2, 2, G, 8, W), bf16),
        in_specs=[pl.BlockSpec(memory_space=pl.ANY), vm, vm, vm, vm, vm],
        out_specs=pl.BlockSpec(memory_space=pl.ANY),
        scratch_shapes=[
            pltpu.VMEM((NB * NSTO * EH, W), u32),
            pltpu.VMEM((9, C, 128), f32),
            pltpu.VMEM((C, 128), u32),
            pltpu.VMEM((EH, 128), u32),
            pltpu.VMEM((E, 128), f32),
            pltpu.VMEM((CH, E), u32),
            pltpu.VMEM((PADV, 3, C), bf16),
            pltpu.SMEM((1,), jnp.int32),
        ],
        compiler_params=pltpu.CompilerParams(vmem_limit_bytes=128 * 1024 * 1024,
                                             disable_bounds_checks=NOBC),
        name="convnext",
    )(xt, dw, w1, w2t, grn_gamma, grn_beta)
    return jnp.transpose(o.reshape(1, H, C, W), (0, 1, 3, 2))
```

```python
import math
import jax
import jax.numpy as jnp
from jax import lax
from jax.experimental import pallas as pl
from jax.experimental.pallas import tpu as pltpu

H = 512
W = 512
C = 96
E = 384
G = C // 8
NT = W // 128
TB = 8
NB = H // TB
NQ = TB // 2
REC = tuple(int(ch) for ch in "123")
STO = tuple(r for r in range(TB) if r not in REC)
NSTO = len(STO)
NREC = len(REC)
EH = E // 2
CH = C // 2
SROWS = G * 24
NCH = 2
U1 = 2
PB = NQ * U1
NI = NB // U1
U2 = 1
P2ORDER = "f"
PADV = 15
TIE = 16
LOGR = "1" == "1"
EARLY = "0" == "1"
CV2 = "0" == "1"
PLAN = "2222220"
DEADL = "0" == "1"
NOBC = "1" == "1"

C0 = math.sqrt(2.0 / math.pi)
C1 = 0.044715
GA = (C0 * C1) ** (1.0 / 3.0)
GK = C0 / GA
LN_EPS = 1e-5

f32 = jnp.float32
bf16 = jnp.bfloat16
u32 = jnp.uint32


def _pack(v):
    return pltpu.bitcast(v.astype(bf16), u32)


def _unp(v):
    return pltpu.bitcast(v, bf16)


def _zero_lane(a, l):
    lane = lax.broadcasted_iota(jnp.int32, a.shape, 1)
    return jnp.where(lane == l, jnp.zeros_like(a), a)


def _shift_r(a, edge=True):
    lane = lax.broadcasted_iota(jnp.int32, (a.shape[0], 128), 1)
    r = [pltpu.roll(a[:, t * 128:(t + 1) * 128], 1, 1) for t in range(NT)]
    return jnp.concatenate(
        [_zero_lane(r[0], 0) if edge else r[0]]
        + [jnp.where(lane == 0, r[t - 1], r[t]) for t in range(1, NT)], axis=1)


def _shift_l(a, edge=True):
    lane = lax.broadcasted_iota(jnp.int32, (a.shape[0], 128), 1)
    r = [pltpu.roll(a[:, t * 128:(t + 1) * 128], 127, 1) for t in range(NT)]
    return jnp.concatenate(
        [jnp.where(lane == 127, r[t + 1], r[t]) for t in range(NT - 1)]
        + [_zero_lane(r[NT - 1], 127) if edge else r[NT - 1]], axis=1)


def _tile4(v):
    return jnp.concatenate([v] * NT, axis=1)


def _sums(c):
    s1 = c[0]
    s2 = c[0] * c[0]
    for g in range(1, G):
        s1 = s1 + c[g]
        s2 = s2 + c[g] * c[g]
    return s1, s2


def _merge4(a, b):
    lo = lax.broadcasted_iota(jnp.int32, (8, 128), 0) < 4
    return jnp.where(lo, a, b) + pltpu.roll(jnp.where(lo, b, a), 4, 0)


def _var_from(n, shift):
    eps = LN_EPS / (GA * GA)
    mean = n * (1.0 / (C * GA))
    msq = pltpu.roll(mean * mean, shift, 0)
    return jnp.maximum(n * (1.0 / (C * GA * GA)) + eps - msq, eps)


def _rstd_from(n, shift):
    return lax.rsqrt(_var_from(n, shift))


def _var2(c0, c1):
    a1, a2 = _sums(c0)
    b1, b2 = _sums(c1)
    m1 = _merge4(a1, b1)
    m2 = _merge4(a2, b2)
    sub = lax.broadcasted_iota(jnp.int32, (8, 128), 0)
    n = jnp.where((sub & 2) == 0, m1 + pltpu.roll(m1, 6, 0), m2 + pltpu.roll(m2, 2, 0))
    n = n + pltpu.roll(n, 1, 0)
    return _var_from(n, 2)


def _rstd1(c):
    s1, s2 = _sums(c)
    n = _merge4(s1, s2)
    n = n + pltpu.roll(n, 2, 0)
    n = n + pltpu.roll(n, 1, 0)
    rstd = _rstd_from(n, 4)
    return jnp.broadcast_to(rstd[7:8], (8, 128))


def _gelu2(y):
    u = y * (y * y + GK)
    return y * (jnp.tanh(u) + 1.0)


def kernel(x_hbm, dw_ref, w1_ref, w2t_ref, gam_ref, bet_ref, o_hbm,
           hbuf, dwb, dmat, w1s, acc, w2s, pad0, zs):
    zs[0] = 0
    pad0[...] = jnp.zeros_like(pad0)

    def w1t(c0=0, n=E):
        return _unp(w1s[c0 // 2:(c0 + n) // 2, :])[:, :C]

    def setup():
        sub = lax.broadcasted_iota(jnp.int32, (C, C), 0)
        lan = lax.broadcasted_iota(jnp.int32, (C, C), 1)
        eye = sub == lan
        for i in range(3):
            for j in range(3):
                row = dw_ref[i, j:j + 1, :].astype(f32)
                col = jnp.sum(jnp.where(eye, jnp.broadcast_to(row, (C, C)), 0.0), axis=1, keepdims=True)
                dwb[i * 3 + j] = jnp.broadcast_to(col, (C, 128))
        c_ = lax.broadcasted_iota(jnp.int32, (8, 128), 0)
        k_ = lax.broadcasted_iota(jnp.int32, (8, 128), 1)
        for g in range(G):
            halves = []
            for o in range(2):
                d = jnp.zeros((8, 128), f32)
                for i in range(3):
                    ri = i + o
                    for j in range(3):
                        kpos = (ri // 2) * 48 + j * 16 + (ri % 2) * 8
                        d = jnp.where(k_ == c_ + kpos, dwb[i * 3 + j, 8 * g:8 * g + 8, :], d)
                halves.append(d)
            dmat[8 * g:8 * g + 8, :] = _pack(jnp.concatenate(halves, axis=0))
        w1f = w1_ref[...].astype(f32)
        w1c = w1f - jnp.sum(w1f, axis=0, keepdims=True) * (1.0 / C)
        w1p = jnp.concatenate([w1c, jnp.zeros((128 - C, E), f32)], axis=0)
        w1s[...] = _pack(w1p.T)
        acc[...] = jnp.zeros_like(acc)

    def scope1(xb1, sbuf, xns, sem1):
        def halves(p0, n_lo, n_hi, slot, skip_lo=0):
            cps = []
            if n_lo:
                cps.append(pltpu.make_async_copy(
                    x_hbm.at[pl.ds(p0 - 1 + skip_lo, n_lo), 1],
                    xb1.at[slot, pl.ds(skip_lo, n_lo), :, pl.ds(0, 8), :], sem1.at[slot, 0]))
            if n_hi:
                cps.append(pltpu.make_async_copy(
                    x_hbm.at[pl.ds(p0, n_hi), 0],
                    xb1.at[slot, pl.ds(0, n_hi), :, pl.ds(8, 8), :], sem1.at[slot, 1]))
            return cps

        def grp_head():
            return halves(0, NQ - 1, NQ, 1, skip_lo=1)

        def grp(i, slot):
            return halves(PB * i + NQ, PB, PB, slot)

        def grp_last():
            return halves(PB * (NI - 1) + NQ, PB - 3, PB - 4, (NI - 1) % 2)

        def build(slot, k):
            for g in range(G):
                v = pltpu.bitcast(xb1[slot, k, g], u32)
                base = (k % NQ) * SROWS + g * 24
                sbuf[base:base + 8, :] = _shift_r(v, False)
                sbuf[base + 8:base + 16, :] = v
                sbuf[base + 16:base + 24, :] = _shift_l(v, False)

        def conv_var(s0, t):
            ts = slice(t * 128, (t + 1) * 128)
            cv = []
            for g in range(G):
                b0 = (s0 % NQ) * SROWS + g * 24
                b1 = ((s0 + 1) % NQ) * SROWS + g * 24
                parts = []
                for bb in (b0, b1):
                    lft, mid, rgt = (sbuf[bb + 8 * j:bb + 8 * j + 8, ts] for j in range(3))
                    parts += [_zero_lane(lft, 0) if t == 0 else lft, mid,
                              _zero_lane(rgt, 127) if t == NT - 1 else rgt]
                s = _unp(jnp.concatenate(parts, axis=0))
                d = _unp(dmat[8 * g:8 * g + 8, :])[:, :C]
                cv.append(jnp.dot(d, s, preferred_element_type=f32))
            c0 = [v[0:8] for v in cv]
            c1 = [v[8:16] for v in cv]
            return (s0, t, c0, c1, _var2(c0, c1))

        def norm(st, tie=None):
            s0, t, c0, c1, var = st
            if tie is not None:
                never = lax.broadcasted_iota(jnp.int32, (8, 128), 0) < zs[0]
                var = jnp.where(never, tie, var)
            if LOGR:
                rstd = jnp.exp2(jnp.log(var) * (-0.5 / math.log(2.0)))
            else:
                rstd = lax.rsqrt(var)
            r0 = jnp.broadcast_to(rstd[3:4], (8, 128))
            r1 = jnp.broadcast_to(rstd[7:8], (8, 128))
            ts = slice(t * 128, (t + 1) * 128)
            r = 2 * (s0 % NQ)
            xns[r * CH:(r + 1) * CH, ts] = _pack(jnp.concatenate([c * r0 for c in c0], axis=0))
            xns[(r + 1) * CH:(r + 2) * CH, ts] = _pack(jnp.concatenate([c * r1 for c in c1], axis=0))

        for cp in grp_head() + grp(0, 0):
            cp.start()
        setup()
        xb1[1, 0, :, 0:8, :] = jnp.zeros((G, 8, W), bf16)
        for cp in grp_head():
            cp.wait()
        for k in range(NQ):
            build(1, k)
        for s0 in range(2):
            for t in range(NT):
                norm(conv_var(s0, t))

        def dma1(i, slot):
            @pl.when(i < NI - 1)
            def _():
                for cp in grp(i, slot):
                    cp.wait()

            @pl.when(i == NI - 1)
            def _():
                for cp in grp_last():
                    cp.wait()
                xb1[(NI - 1) % 2, PB - 4, :, 8:16, :] = jnp.zeros((G, 8, W), bf16)

            @pl.when(i + 1 < NI - 1)
            def _():
                for cp in grp(i + 1, 1 - slot):
                    cp.start()

            @pl.when(i + 1 == NI - 1)
            def _():
                for cp in grp_last():
                    cp.start()

        def block1(b, slot, u, pend):
            def mm1(r, c):
                n = E // NCH
                y = jnp.dot(w1t(c * n, n), _unp(xns[r * CH:(r + 1) * CH, :]), preferred_element_type=f32)
                h = _gelu2(y)
                h2 = h * h
                acc[c * n:(c + 1) * n, :] += (h2[:, 0:128] + h2[:, 128:256]) + (h2[:, 256:384] + h2[:, 384:512])
                if r in STO:
                    row0 = pl.multiple_of((b * NSTO + STO.index(r)) * EH + c * (n // 2), 8)
                    hbuf[pl.ds(row0, n // 2), :] = _pack(h)
                return y

            for k in range(NQ):
                tiles = list(range(NT))
                for o in range(2):
                    for c in range(NCH):
                        y = mm1(2 * k + o, c)
                        if pend is not None:
                            norm(pend, y[TIE:TIE + 8, 0:128])
                        pend = conv_var(k + 2, tiles.pop(0))
                build(slot, u * NQ + k)
            return pend

        def pass1(i, carry):
            slot = i & 1
            dma1(i, slot)
            pend = None
            for u in range(U1):
                pend = block1(i * U1 + u, slot, u, pend)
            norm(pend)
            return carry

        lax.fori_loop(0, NB // U1, pass1, 0)

    pl.run_scoped(scope1,
                  pltpu.VMEM((2, PB, G, 16, W), bf16),
                  pltpu.VMEM((NQ * SROWS, W), u32),
                  pltpu.VMEM((TB * CH, W), u32),
                  pltpu.SemaphoreType.DMA((2, 2)))

    def scope2(xb2, ob, hre, cbuf, sem2, semo):
        def in2(b, slot, half):
            return pltpu.make_async_copy(x_hbm.at[pl.ds(NQ * b + 2 * half, 2)],
                                         xb2.at[slot, pl.ds(2 * half, 2)], sem2.at[slot, half])

        def out2(b, slot, half):
            return pltpu.make_async_copy(ob.at[slot, pl.ds(2 * half, 2)],
                                         o_hbm.at[pl.ds(NQ * b + 2 * half, 2)], semo.at[slot, half])

        def conv_rec(slot, groups=range(G)):
            lane = lax.broadcasted_iota(jnp.int32, (8, 128), 1)
            for g in (groups if CV2 else ()):
                need = sorted({r + d for r in REC for d in (-1, 0, 1)})
                xs = {q: xb2[slot, q // 2, q % 2, g].astype(f32) for q in need}
                wt = [dwb[tap, 8 * g:8 * g + 8, :] for tap in range(9)]
                a0p, a2p, part = {}, {}, {}
                for t in range(NT + 1):
                    ts = slice(t * 128, (t + 1) * 128)
                    for k, r in enumerate(REC):
                        def col(j):
                            return (xs[r - 1][:, ts] * wt[j] + xs[r][:, ts] * wt[3 + j]) + xs[r + 1][:, ts] * wt[6 + j]
                        if t < NT:
                            a2 = col(2)
                        if t > 0:
                            m2 = jnp.where(lane == 0, a2 if t < NT else jnp.zeros((8, 128), f32), a2p[k])
                            cbuf[(k + 1) * C + 8 * g:(k + 1) * C + 8 * g + 8, (t - 1) * 128:t * 128] = (
                                part[k] + pltpu.roll(m2, 127, 1))
                        if t < NT:
                            a0 = col(0)
                            m0 = jnp.where(lane == 127, a0p[k] if t > 0 else jnp.zeros((8, 128), f32), a0)
                            part[k] = pltpu.roll(m0, 1, 1) + col(1)
                            a0p[k], a2p[k] = a0, a2
            for g in (() if CV2 else groups):
                need = sorted({r + d for r in REC for d in (-1, 0, 1)})
                xs = {q: xb2[slot, q // 2, q % 2, g].astype(f32) for q in need}
                wt = [_tile4(dwb[tap, 8 * g:8 * g + 8, :]) for tap in range(9)]
                for k, r in enumerate(REC):
                    a = []
                    for j in range(3):
                        t = xs[r - 1] * wt[j]
                        t = t + xs[r] * wt[3 + j]
                        t = t + xs[r + 1] * wt[6 + j]
                        a.append(t)
                    cbuf[(k + 1) * C + 8 * g:(k + 1) * C + 8 * g + 8, :] = _shift_r(a[0]) + a[1] + _shift_l(a[2])

        def ln_rec(k):
            cols = []
            for t in range(NT):
                c = [cbuf[(k + 1) * C + 8 * g:(k + 1) * C + 8 * g + 8, t * 128:(t + 1) * 128] for g in range(G)]
                r = _rstd1(c)
                cols.append(jnp.concatenate([v * r for v in c], axis=0))
            return jnp.concatenate(cols, axis=1).astype(bf16)

        for b0 in range(3):
            for hf in range(2):
                in2(b0, b0, hf).start()
        ssq = jnp.sum(acc[...].T, axis=0, keepdims=True) * (1.0 / (4.0 * GA * GA))
        gx = jnp.sqrt(ssq + 1e-6)
        nx = gx / (jnp.sum(gx, axis=1, keepdims=True) * (1.0 / E) + 1e-6)
        gam = gam_ref[...].astype(f32).reshape(1, E)
        bet = bet_ref[...].astype(f32).reshape(1, E)
        scale = (gam * nx + 1.0) * (1.0 / (2.0 * GA))
        w2f = w2t_ref[...].astype(f32)
        w2s[...] = _pack(w2f * scale)
        cbuf[0:C, :] = jnp.broadcast_to(jnp.sum(w2f * bet, axis=1, keepdims=True), (C, W))
        for hf in range(2):
            in2(0, 0, hf).wait()
        conv_rec(0)

        def block2(b, slot, oslot, dma=3):
            nslot = jnp.where(slot == 2, 0, slot + 1)

            def wait_in():
                @pl.when(b + 1 < NB)
                def _():
                    for hf in range(2):
                        in2(b + 1, nslot, hf).wait()

            def start_in(half):
                @pl.when(b + 3 < NB)
                def _():
                    in2(b + 3, slot, half).start()

            def wait_out(half):
                @pl.when(b >= 2)
                def _():
                    out2(b - 2, oslot, half).wait()

            def mm2(hp):
                return jnp.dot(_unp(w2s[...]), _unp(hp), preferred_element_type=f32)

            first = [k for k in range(NSTO) if STO[k] < NQ][0]
            pending = list(range(G))
            r_first = STO[first]

            def finish(r, o, ngroups=0, deadline=False):
                for g in range(G):
                    xr = xb2[slot, r // 2, r % 2, g].astype(f32)
                    if deadline:
                        bg = cbuf[pl.ds(pl.multiple_of(zs[0] + 8 * g, 8), 8), 0:128]
                    else:
                        bg = cbuf[8 * g:8 * g + 8, 0:128]
                    v = o[8 * g:8 * g + 8, :] + (xr + _tile4(bg))
                    ob[oslot, r // 2, r % 2, g] = v.astype(bf16)
                for j in range(ngroups):
                    t = j * NT // ngroups
                    xb2[slot, r_first // 2, r_first % 2, 0, :, 0:128] = o[0:8, t * 128:(t + 1) * 128].astype(bf16)
                    conv_rec(nslot, [pending.pop(0)])

            def rec(k):
                y = jnp.dot(w1t(), ln_rec(k), preferred_element_type=f32)
                hre[k * EH:(k + 1) * EH, :] = _pack(_gelu2(y))

            def sto_mm(k):
                row0 = pl.multiple_of((b * NSTO + k) * EH, 8)
                return mm2(hbuf[pl.ds(row0, EH), :])

            def sto(k, *a):
                finish(STO[k], sto_mm(k), *a)

            def fin(k, *a):
                finish(REC[k], mm2(hre[pl.ds(pl.multiple_of(zs[0] + k * EH, 8), EH), :]), *a)

            rec_hi = [k for k in range(NREC) if REC[k] >= NQ]
            rec_lo = [k for k in range(NREC) if REC[k] < NQ]
            sto_hi = [k for k in range(NSTO) if STO[k] >= NQ]
            sto_lo = [k for k in range(NSTO) if STO[k] < NQ]
            first = sto_lo.pop(0)
            tail = ([f"s{k}" for k in sto_hi] + [f"f{k}" for k in rec_hi] + ["o", "I"]
                    + [f"s{k}" for k in sto_lo] + [f"f{k}" for k in rec_lo])
            mixed = tail
            plan = [int(ch) for ch in PLAN]
            seq = " ".join(["W0 W1 J A B"] + [f"r{k}" for k in rec_hi + rec_lo] + mixed)
            for tok in seq.split():
                if tok in "IJ" and not dma & 1 or tok[0] in "Wo" and not dma & 2:
                    continue
                if tok[0] == "c":
                    conv_rec(nslot, range(int(tok[1], 16), int(tok[2], 16)))
                elif tok == "o":
                    out2(b, oslot, 1).start()
                elif tok == "I":
                    start_in(1)
                elif tok == "J":
                    wait_in()
                elif tok[0] == "W":
                    wait_out(int(tok[1]))
                elif tok == "A":
                    o_first = sto_mm(first)
                elif tok == "B":
                    finish(STO[first], o_first)
                elif tok[0] == "r":
                    rec(int(tok[1]))
                else:
                    ng = plan.pop(0)
                    {"s": sto, "f": fin}[tok[0]](int(tok[1]), ng, DEADL and not plan)
            if dma & 2:
                out2(b, oslot, 0).start()
            if dma & 1:
                start_in(0)
            return nslot

        def pass2(i, slot, dma=3):
            for u in range(U2):
                b = i * U2 + u
                oslot = (u % 2) if U2 % 2 == 0 else (b & 1)
                slot = block2(b, slot, oslot, dma)
            return slot

        lax.fori_loop(0, NB // U2, pass2, jnp.int32(0))
        for hf in range(2):
            out2(NB - 2, 0, hf).wait()
            out2(NB - 1, 1, hf).wait()
        x2 = 9
        if x2 < 9:
            if x2 & 1:
                for b0 in range(1, 3):
                    for hf in range(2):
                        in2(b0, b0, hf).start()
            lax.fori_loop(0, NB // U2, functools.partial(pass2, dma=x2), jnp.int32(0))
            if x2 & 2:
                for hf in range(2):
                    out2(NB - 2, 0, hf).wait()
                    out2(NB - 1, 1, hf).wait()

    pl.run_scoped(scope2,
                  pltpu.VMEM((3, NQ, 2, G, 8, W), bf16),
                  pltpu.VMEM((2, NQ, 2, G, 8, W), bf16),
                  pltpu.VMEM((NREC * EH, W), u32),
                  pltpu.VMEM(((NREC + 1) * C, W), f32),
                  pltpu.SemaphoreType.DMA((3, 2)),
                  pltpu.SemaphoreType.DMA((2, 2)))


@jax.jit
def pallas_standalone__modern_conv_block_convnext_v2__vision_kernel(x, dw, w1, w2, grn_gamma, grn_beta):
    xt = jnp.transpose(x, (0, 1, 3, 2)).reshape(H // 2, 2, G, 8, W)
    w2t = w2.T
    vm = pl.BlockSpec(memory_space=pltpu.VMEM)
    o = pl.pallas_call(
        kernel,
        out_shape=jax.ShapeDtypeStruct((H // 2, 2, G, 8, W), bf16),
        in_specs=[pl.BlockSpec(memory_space=pl.ANY), vm, vm, vm, vm, vm],
        out_specs=pl.BlockSpec(memory_space=pl.ANY),
        scratch_shapes=[
            pltpu.VMEM((NB * NSTO * EH, W), u32),
            pltpu.VMEM((9, C, 128), f32),
            pltpu.VMEM((C, 128), u32),
            pltpu.VMEM((EH, 128), u32),
            pltpu.VMEM((E, 128), f32),
            pltpu.VMEM((CH, E), u32),
            pltpu.VMEM((PADV, 3, C), bf16),
            pltpu.SMEM((1,), jnp.int32),
        ],
        compiler_params=pltpu.CompilerParams(vmem_limit_bytes=128 * 1024 * 1024,
                                             disable_bounds_checks=NOBC),
        name="convnext",
    )(xt, dw, w1, w2t, grn_gamma, grn_beta)
    return jnp.transpose(o.reshape(1, H, C, W), (0, 1, 3, 2))
```

```python
import math
import jax
import jax.numpy as jnp
from jax import lax
from jax.experimental import pallas as pl
from jax.experimental.pallas import tpu as pltpu

H = 512
W = 512
C = 96
E = 384
G = C // 8
NT = W // 128
TB = 8
NB = H // TB
NQ = TB // 2
REC = (1, 2, 3)
STO = tuple(r for r in range(TB) if r not in REC)
NSTO = len(STO)
NREC = len(REC)
EH = E // 2
CH = C // 2
SROWS = G * 24
NCH = 2
U1 = 2
R1 = TB * U1
NI = NB // U1
NX = 2 * U1
TIE = 16
PLAN = "2222220"
AR = 0
PADV = 15

C0 = math.sqrt(2.0 / math.pi)
C1 = 0.044715
GA = (C0 * C1) ** (1.0 / 3.0)
GK = C0 / GA
LN_EPS = 1e-5

f32 = jnp.float32
bf16 = jnp.bfloat16
u32 = jnp.uint32


def _pack(v):
    return pltpu.bitcast(v.astype(bf16), u32)


def _unp(v):
    return pltpu.bitcast(v, bf16)


def _zero_lane(a, l):
    lane = lax.broadcasted_iota(jnp.int32, a.shape, 1)
    return jnp.where(lane == l, jnp.zeros_like(a), a)


def _shift_r(a, edge=True):
    lane = lax.broadcasted_iota(jnp.int32, (a.shape[0], 128), 1)
    v = [a[:, t * 128:(t + 1) * 128] for t in range(NT)]
    m = [_zero_lane(v[0], 127) if edge else v[0]] + [jnp.where(lane == 127, v[t - 1], v[t]) for t in range(1, NT)]
    return jnp.concatenate([pltpu.roll(u, 1, 1) for u in m], axis=1)


def _shift_l(a, edge=True):
    lane = lax.broadcasted_iota(jnp.int32, (a.shape[0], 128), 1)
    v = [a[:, t * 128:(t + 1) * 128] for t in range(NT)]
    m = ([jnp.where(lane == 0, v[t + 1], v[t]) for t in range(NT - 1)]
         + [_zero_lane(v[NT - 1], 0) if edge else v[NT - 1]])
    return jnp.concatenate([pltpu.roll(u, 127, 1) for u in m], axis=1)


def _tile4(v):
    return jnp.concatenate([v] * NT, axis=1)


def _sums(c):
    s1 = c[0]
    s2 = c[0] * c[0]
    for g in range(1, G):
        s1 = s1 + c[g]
        s2 = s2 + c[g] * c[g]
    return s1, s2


def _merge4(a, b):
    lo = lax.broadcasted_iota(jnp.int32, (8, 128), 0) < 4
    return jnp.where(lo, a, b) + pltpu.roll(jnp.where(lo, b, a), 4, 0)


def _var_from(n, shift):
    eps = LN_EPS / (GA * GA)
    mean = n * (1.0 / (C * GA))
    msq = pltpu.roll(mean * mean, shift, 0)
    return jnp.maximum(n * (1.0 / (C * GA * GA)) + eps - msq, eps)


def _var2(c0, c1):
    a1, a2 = _sums(c0)
    b1, b2 = _sums(c1)
    m1 = _merge4(a1, b1)
    m2 = _merge4(a2, b2)
    sub = lax.broadcasted_iota(jnp.int32, (8, 128), 0)
    n = jnp.where((sub & 2) == 0, m1 + pltpu.roll(m1, 6, 0), m2 + pltpu.roll(m2, 2, 0))
    n = n + pltpu.roll(n, 1, 0)
    return _var_from(n, 2)


def _var1(c):
    s1, s2 = _sums(c)
    n = _merge4(s1, s2)
    n = n + pltpu.roll(n, 2, 0)
    n = n + pltpu.roll(n, 1, 0)
    return _var_from(n, 4)


def _rsqrt(v):
    return jnp.exp2(jnp.log(v) * (-0.5 / math.log(2.0)))


def _gelu2(y):
    u = y * (y * y + GK)
    return y * (jnp.tanh(u) + 1.0)


def kernel(x_hbm, dw_hbm, w1_hbm, w2t_hbm, gam_hbm, bet_hbm, o_hbm,
           hbuf, xb, dmat, w1s, acc, w2s, w1_ref, w2t_ref, dw_ref, gam_ref, bet_ref, pad0,
           zs, semx, semp):
    def xcopy(r0, n, d0, sem):
        return pltpu.make_async_copy(x_hbm.at[pl.ds(r0, n)], xb.at[pl.ds(d0, n)], sem)

    def grp_head():
        return xcopy(0, TB - 1, R1 + 1, semx.at[2])

    def grp(i, slot):
        return xcopy(R1 * i + TB - 1, R1, R1 * slot, semx.at[2 * slot])

    def grp_last():
        return xcopy(R1 * (NI - 1) + TB - 1, R1 - TB + 1, R1 * ((NI - 1) % 2), semx.at[2 * ((NI - 1) % 2)])

    def in2(b, slot):
        return xcopy(TB * b, TB, TB * slot, semx.at[slot])

    params = [pltpu.make_async_copy(src, dst, semp.at[j]) for j, (src, dst) in enumerate(
        [(dw_hbm, dw_ref), (w1_hbm, w1_ref), (w2t_hbm, w2t_ref), (gam_hbm, gam_ref), (bet_hbm, bet_ref)])]
    for cp in params[:2] + [grp_head()] + params[2:] + [grp(0, 0)]:
        cp.start()
    zs[0] = 0
    pad0[...] = jnp.zeros_like(pad0)

    def w1t(c0=0, n=E):
        return _unp(w1s[c0 // 2:(c0 + n) // 2, :])[:, :C]

    def tap_columns():
        sub = lax.broadcasted_iota(jnp.int32, (C, C), 0)
        lan = lax.broadcasted_iota(jnp.int32, (C, C), 1)
        eye = sub == lan
        cols = []
        for i in range(3):
            for j in range(3):
                row = dw_ref[i, j:j + 1, :].astype(f32)
                col = jnp.sum(jnp.where(eye, jnp.broadcast_to(row, (C, C)), 0.0), axis=1, keepdims=True)
                cols.append(jnp.broadcast_to(col, (C, 128)))
        return cols

    def setup():
        cols = tap_columns()
        c_ = lax.broadcasted_iota(jnp.int32, (8, 128), 0)
        k_ = lax.broadcasted_iota(jnp.int32, (8, 128), 1)
        for g in range(G):
            halves = []
            for o in range(2):
                d = jnp.zeros((8, 128), f32)
                for i in range(3):
                    ri = i + o
                    for j in range(3):
                        kpos = (ri // 2) * 48 + j * 16 + (ri % 2) * 8
                        d = jnp.where(k_ == c_ + kpos, cols[i * 3 + j][8 * g:8 * g + 8], d)
                halves.append(d)
            dmat[8 * g:8 * g + 8, :] = _pack(jnp.concatenate(halves, axis=0))
        w1f = w1_ref[...].astype(f32)
        w1c = w1f - jnp.sum(w1f, axis=0, keepdims=True) * (1.0 / C)
        w1p = jnp.concatenate([w1c, jnp.zeros((128 - C, E), f32)], axis=0)
        w1s[...] = _pack(w1p.T)

    def scope1(sbuf, xns):
        def build(row0, k):
            for g in range(G):
                v = pltpu.bitcast(xb[pl.ds(row0 + 2 * k, 2), g].reshape(16, W), u32)
                base = (k % NQ) * SROWS + g * 24
                sbuf[base:base + 8, :] = _shift_r(v, False)
                sbuf[base + 8:base + 16, :] = v
                sbuf[base + 16:base + 24, :] = _shift_l(v, False)

        def conv_var(s0, t):
            ts = slice(t * 128, (t + 1) * 128)
            cv = []
            for g in range(G):
                parts = []
                for sl in (s0, s0 + 1):
                    bb = (sl % NQ) * SROWS + g * 24
                    lft, mid, rgt = (sbuf[bb + 8 * j:bb + 8 * j + 8, ts] for j in range(3))
                    parts += [_zero_lane(lft, 0) if t == 0 else lft, mid,
                              _zero_lane(rgt, 127) if t == NT - 1 else rgt]
                s = _unp(jnp.concatenate(parts, axis=0))
                d = _unp(dmat[8 * g:8 * g + 8, :])[:, :C]
                cv.append(jnp.dot(d, s, preferred_element_type=f32))
            c0 = [v[0:8] for v in cv]
            c1 = [v[8:16] for v in cv]
            return (s0, t, c0, c1, _var2(c0, c1))

        def norm(st, tie=None):
            s0, t, c0, c1, var = st
            if tie is not None:
                never = lax.broadcasted_iota(jnp.int32, (8, 128), 0) < zs[0]
                var = jnp.where(never, tie, var)
            rstd = _rsqrt(var)
            r0 = jnp.broadcast_to(rstd[3:4], (8, 128))
            r1 = jnp.broadcast_to(rstd[7:8], (8, 128))
            ts = slice(t * 128, (t + 1) * 128)
            r = 2 * (s0 % NQ)
            xns[r * CH:(r + 1) * CH, ts] = _pack(jnp.concatenate([c * r0 for c in c0], axis=0))
            xns[(r + 1) * CH:(r + 2) * CH, ts] = _pack(jnp.concatenate([c * r1 for c in c1], axis=0))

        acc[...] = jnp.zeros_like(acc)
        xb[R1] = jnp.zeros((G, 8, W), bf16)
        params[0].wait()
        params[1].wait()
        setup()
        grp_head().wait()
        for k in range(NQ):
            build(R1, k)
        for s0 in range(2):
            for t in range(NT):
                norm(conv_var(s0, t))

        def dma1(i, slot):
            @pl.when(i < NI - 1)
            def _():
                grp(i, slot).wait()

            @pl.when(i == NI - 1)
            def _():
                grp_last().wait()
                xb[R1 * ((NI - 1) % 2) + R1 - TB + 1] = jnp.zeros((G, 8, W), bf16)
                for b0 in range(2):
                    in2(b0, (NI % 2) * U1 + b0).start()

            @pl.when(i + 1 < NI - 1)
            def _():
                grp(i + 1, 1 - slot).start()

            @pl.when(i + 1 == NI - 1)
            def _():
                grp_last().start()

        def block1(b, row0, u, pend):
            n = E // NCH
            for k in range(NQ):
                for t in range(NT):
                    r, c = 2 * k + t // NCH, t % NCH
                    y = jnp.dot(w1t(c * n, n), _unp(xns[r * CH:(r + 1) * CH, :]), preferred_element_type=f32)
                    h = _gelu2(y)
                    h2 = h * h
                    acc[c * n:(c + 1) * n, :] += (h2[:, 0:128] + h2[:, 128:256]) + (h2[:, 256:384] + h2[:, 384:512])
                    if r in STO:
                        row = pl.multiple_of((b * NSTO + STO.index(r)) * EH + c * (n // 2), 8)
                        hbuf[pl.ds(row, n // 2), :] = _pack(h)
                    if pend is not None:
                        norm(pend, y[TIE:TIE + 8, 0:128])
                    pend = conv_var(k + 2, t)
                build(row0, u * NQ + k)
            return pend

        def pass1(i, carry):
            slot = i & 1
            dma1(i, slot)
            pend = None
            for u in range(U1):
                pend = block1(i * U1 + u, slot * R1, u, pend)
            norm(pend)
            return carry

        lax.fori_loop(0, NI, pass1, 0)

    pl.run_scoped(scope1,
                  pltpu.VMEM((NQ * SROWS, W), u32),
                  pltpu.VMEM((TB * CH, W), u32))

    assert NI % 2 == 0 and NX == 4

    def scope2(ob, hre, cbuf, dwb, semo):
        def out2(b, slot, half):
            return pltpu.make_async_copy(ob.at[pl.ds(TB * slot + NQ * half, NQ)],
                                         o_hbm.at[pl.ds(TB * b + NQ * half, NQ)], semo.at[slot, half])

        def conv_rec(row0, groups=range(G)):
            for g in groups:
                need = sorted({r + d for r in REC for d in (-1, 0, 1)})
                xs = {q: xb[row0 + q, g].astype(f32) for q in need}
                wt = [_tile4(dwb[tap, 8 * g:8 * g + 8, :]) for tap in range(9)]
                for k, r in enumerate(REC):
                    a = []
                    for j in range(3):
                        t = xs[r - 1] * wt[j]
                        t = t + xs[r] * wt[3 + j]
                        t = t + xs[r + 1] * wt[6 + j]
                        a.append(t)
                    cbuf[(k + 1) * C + 8 * g:(k + 1) * C + 8 * g + 8, :] = _shift_r(a[0]) + a[1] + _shift_l(a[2])

        def ln_rec(k):
            cols = []
            for t in range(NT):
                c = [cbuf[(k + 1) * C + 8 * g:(k + 1) * C + 8 * g + 8, t * 128:(t + 1) * 128] for g in range(G)]
                r = jnp.broadcast_to(lax.rsqrt(_var1(c))[7:8], (8, 128))
                cols.append(jnp.concatenate([v * r for v in c], axis=0))
            return jnp.concatenate(cols, axis=1).astype(bf16)

        in2(2, 2).start()
        for cp in params[2:]:
            cp.wait()
        in2(0, 0).wait()
        for tap, col in enumerate(tap_columns()):
            dwb[tap] = col
        ssq = jnp.sum(acc[...].T, axis=0, keepdims=True) * (1.0 / (4.0 * GA * GA))
        gx = jnp.sqrt(ssq + 1e-6)
        nx = gx / (jnp.sum(gx, axis=1, keepdims=True) * (1.0 / E) + 1e-6)
        gam = gam_ref[...].astype(f32).reshape(1, E)
        bet = bet_ref[...].astype(f32).reshape(1, E)
        scale = (gam * nx + 1.0) * (1.0 / (2.0 * GA))
        w2f = w2t_ref[...].astype(f32)
        w2s[...] = _pack(w2f * scale)
        cbuf[0:C, 0:128] = jnp.broadcast_to(jnp.sum(w2f * bet, axis=1, keepdims=True), (C, 128))
        conv_rec(0)

        def pass2(b, carry):
            row0 = (b & 3) * TB
            nrow0 = ((b + 1) & 3) * TB
            oslot = b & 1

            @pl.when(b + 3 < NB)
            def _():
                in2(b + 3, (b + 3) & 3).start()

            @pl.when(b >= 2)
            def _():
                for hf in range(2):
                    out2(b - 2, oslot, hf).wait()

            @pl.when(b + 1 < NB)
            def _():
                in2(b + 1, (b + 1) & 3).wait()

            pending = list(range(G))
            plan = [int(ch) for ch in PLAN]

            def finish(r, hp, ngroups):
                o = jnp.dot(_unp(w2s[...]), _unp(hp), preferred_element_type=f32)
                for hf in range(2):
                    ls = slice(hf * 256, hf * 256 + 256)
                    for j in range((ngroups + 1 - hf) // 2):
                        t = 2 * hf + j
                        xb[row0 + STO[0], zs[0]] = _tile4(o[AR:AR + 8, t * 128:(t + 1) * 128]).astype(bf16)
                        conv_rec(nrow0, [pending.pop(0)])
                    for g in range(G):
                        xr = xb[row0 + r, g, :, ls].astype(f32)
                        bg = cbuf[8 * g:8 * g + 8, 0:128]
                        v = o[8 * g:8 * g + 8, ls] + (xr + jnp.concatenate([bg, bg], axis=1))
                        ob[oslot * TB + r, g, :, ls] = v.astype(bf16)

            def sto(k, ngroups):
                finish(STO[k], hbuf[pl.ds(pl.multiple_of((b * NSTO + k) * EH, 8), EH), :], ngroups)

            sto(0, 0)
            for k in range(NREC):
                y = jnp.dot(w1t(), ln_rec(k), preferred_element_type=f32)
                hre[k * EH:(k + 1) * EH, :] = _pack(_gelu2(y))
            for k in range(1, NSTO):
                sto(k, plan.pop(0))
            out2(b, oslot, 1).start()
            for k in range(NREC):
                finish(REC[k], hre[pl.ds(pl.multiple_of(zs[0] + k * EH, 8), EH), :], plan.pop(0))
            out2(b, oslot, 0).start()
            return carry

        lax.fori_loop(0, NB, pass2, 0)
        for hf in range(2):
            out2(NB - 2, 0, hf).wait()
            out2(NB - 1, 1, hf).wait()

    pl.run_scoped(scope2,
                  pltpu.VMEM((2 * TB, G, 8, W), bf16),
                  pltpu.VMEM((NREC * EH, W), u32),
                  pltpu.VMEM(((NREC + 1) * C, W), f32),
                  pltpu.VMEM((9, C, 128), f32),
                  pltpu.SemaphoreType.DMA((2, 2)))


@jax.jit
def pallas_standalone__modern_conv_block_convnext_v2__vision_kernel(x, dw, w1, w2, grn_gamma, grn_beta):
    xt = jnp.transpose(x, (0, 1, 3, 2)).reshape(H, G, 8, W)
    w2t = w2.T
    hbm = pl.BlockSpec(memory_space=pl.ANY)
    o = pl.pallas_call(
        kernel,
        out_shape=jax.ShapeDtypeStruct((H, G, 8, W), bf16),
        in_specs=[hbm] * 6,
        out_specs=hbm,
        scratch_shapes=[
            pltpu.VMEM((NB * NSTO * EH, W), u32),
            pltpu.VMEM((NX * TB, G, 8, W), bf16),
            pltpu.VMEM((C, 128), u32),
            pltpu.VMEM((EH, 128), u32),
            pltpu.VMEM((E, 128), f32),
            pltpu.VMEM((CH, E), u32),
            pltpu.VMEM((C, E), bf16),
            pltpu.VMEM((C, E), bf16),
            pltpu.VMEM((3, 3, C), bf16),
            pltpu.VMEM((E,), bf16),
            pltpu.VMEM((E,), bf16),
            pltpu.VMEM((PADV, 3, C), bf16),
            pltpu.SMEM((1,), jnp.int32),
            pltpu.SemaphoreType.DMA((NX,)),
            pltpu.SemaphoreType.DMA((5,)),
        ],
        compiler_params=pltpu.CompilerParams(vmem_limit_bytes=128 * 1024 * 1024,
                                             disable_bounds_checks=True),
        name="convnext",
    )(xt, dw, w1, w2t, grn_gamma, grn_beta)
    return jnp.transpose(o.reshape(1, H, C, W), (0, 1, 3, 2))
```

```python
import math
import jax
import jax.numpy as jnp
from jax import lax
from jax.experimental import pallas as pl
from jax.experimental.pallas import tpu as pltpu

H = 512
W = 512
C = 96
E = 384
G = C // 8
NT = W // 128
TB = 8
NB = H // TB
NQ = TB // 2
REC = (1, 2, 3)
STO = tuple(r for r in range(TB) if r not in REC)
NSTO = len(STO)
NREC = len(REC)
EH = E // 2
CH = C // 2
SROWS = G * 24
NCH = 2
U1 = 2
R1 = TB * U1
NI = NB // U1
NX = 2 * U1
TIE = 16
PLAN = "2222220"
AR = 0
PADV = 15

C0 = math.sqrt(2.0 / math.pi)
C1 = 0.044715
GA = (C0 * C1) ** (1.0 / 3.0)
GK = C0 / GA
LN_EPS = 1e-5

f32 = jnp.float32
bf16 = jnp.bfloat16
u32 = jnp.uint32


def _pack(v):
    return pltpu.bitcast(v.astype(bf16), u32)


def _unp(v):
    return pltpu.bitcast(v, bf16)


def _zero_lane(a, l):
    lane = lax.broadcasted_iota(jnp.int32, a.shape, 1)
    return jnp.where(lane == l, jnp.zeros_like(a), a)


def _shift_r(a, edge=True):
    lane = lax.broadcasted_iota(jnp.int32, (a.shape[0], 128), 1)
    v = [a[:, t * 128:(t + 1) * 128] for t in range(NT)]
    m = [_zero_lane(v[0], 127) if edge else v[0]] + [jnp.where(lane == 127, v[t - 1], v[t]) for t in range(1, NT)]
    return jnp.concatenate([pltpu.roll(u, 1, 1) for u in m], axis=1)


def _shift_l(a, edge=True):
    lane = lax.broadcasted_iota(jnp.int32, (a.shape[0], 128), 1)
    v = [a[:, t * 128:(t + 1) * 128] for t in range(NT)]
    m = ([jnp.where(lane == 0, v[t + 1], v[t]) for t in range(NT - 1)]
         + [_zero_lane(v[NT - 1], 0) if edge else v[NT - 1]])
    return jnp.concatenate([pltpu.roll(u, 127, 1) for u in m], axis=1)


def _tile4(v):
    return jnp.concatenate([v] * NT, axis=1)


def _sums(c):
    s1 = c[0]
    s2 = c[0] * c[0]
    for g in range(1, G):
        s1 = s1 + c[g]
        s2 = s2 + c[g] * c[g]
    return s1, s2


def _merge4(a, b):
    lo = lax.broadcasted_iota(jnp.int32, (8, 128), 0) < 4
    return jnp.where(lo, a, b) + pltpu.roll(jnp.where(lo, b, a), 4, 0)


def _var_from(n, shift):
    eps = LN_EPS / (GA * GA)
    mean = n * (1.0 / (C * GA))
    msq = pltpu.roll(mean * mean, shift, 0)
    return jnp.maximum(n * (1.0 / (C * GA * GA)) + eps - msq, eps)


def _var2(c0, c1):
    a1, a2 = _sums(c0)
    b1, b2 = _sums(c1)
    m1 = _merge4(a1, b1)
    m2 = _merge4(a2, b2)
    sub = lax.broadcasted_iota(jnp.int32, (8, 128), 0)
    n = jnp.where((sub & 2) == 0, m1 + pltpu.roll(m1, 6, 0), m2 + pltpu.roll(m2, 2, 0))
    n = n + pltpu.roll(n, 1, 0)
    return _var_from(n, 2)


def _var1(c):
    s1, s2 = _sums(c)
    n = _merge4(s1, s2)
    n = n + pltpu.roll(n, 2, 0)
    n = n + pltpu.roll(n, 1, 0)
    return _var_from(n, 4)


def _rsqrt(v):
    return jnp.exp2(jnp.log(v) * (-0.5 / math.log(2.0)))


def _gelu2(y):
    u = y * (y * y + GK)
    return y * (jnp.tanh(u) + 1.0)


def kernel(x_hbm, dw_hbm, w1_hbm, w2t_hbm, gam_hbm, bet_hbm, o_hbm,
           hbuf, xb, cbuf, dmat, w1s, acc, w2s, w1_ref, w2t_ref, dw_ref, gam_ref, bet_ref, pad0,
           zs, semx, semp):
    def xcopy(r0, n, d0, sem):
        return pltpu.make_async_copy(x_hbm.at[pl.ds(r0, n)], xb.at[pl.ds(d0, n)], sem)

    def grp_head():
        return xcopy(0, TB - 1, R1 + 1, semx.at[2])

    def grp(i, slot):
        return xcopy(R1 * i + TB - 1, R1, R1 * slot, semx.at[2 * slot])

    def grp_last():
        return xcopy(R1 * (NI - 1) + TB - 1, R1 - TB + 1, R1 * ((NI - 1) % 2), semx.at[2 * ((NI - 1) % 2)])

    def in2(b, slot):
        return xcopy(TB * b, TB, TB * slot, semx.at[slot])

    params = [pltpu.make_async_copy(src, dst, semp.at[j]) for j, (src, dst) in enumerate(
        [(dw_hbm, dw_ref), (w1_hbm, w1_ref), (w2t_hbm, w2t_ref), (gam_hbm, gam_ref), (bet_hbm, bet_ref)])]
    for cp in params[:2] + [grp_head()] + params[2:] + [grp(0, 0)]:
        cp.start()
    zs[0] = 0
    pad0[...] = jnp.zeros_like(pad0)

    def w1t(c0=0, n=E):
        return _unp(w1s[c0 // 2:(c0 + n) // 2, :])[:, :C]

    def tap_columns():
        sub = lax.broadcasted_iota(jnp.int32, (C, C), 0)
        lan = lax.broadcasted_iota(jnp.int32, (C, C), 1)
        eye = sub == lan
        diags = [jnp.where(eye, jnp.broadcast_to(dw_ref[i, j:j + 1, :].astype(f32), (C, C)), 0.0)
                 for i in range(3) for j in range(3)]
        ones = jnp.ones((C, 128), bf16)
        return [jnp.dot(d.astype(bf16), ones, preferred_element_type=f32) for d in diags]

    def setup():
        cols = tap_columns()
        c_ = lax.broadcasted_iota(jnp.int32, (8, 128), 0)
        k_ = lax.broadcasted_iota(jnp.int32, (8, 128), 1)
        for g in range(G):
            halves = []
            for o in range(2):
                d = jnp.zeros((8, 128), f32)
                for i in range(3):
                    ri = i + o
                    for j in range(3):
                        kpos = (ri // 2) * 48 + j * 16 + (ri % 2) * 8
                        d = jnp.where(k_ == c_ + kpos, cols[i * 3 + j][8 * g:8 * g + 8], d)
                halves.append(d)
            dmat[8 * g:8 * g + 8, :] = _pack(jnp.concatenate(halves, axis=0))
        w1f = w1_ref[...].astype(f32)
        w1c = w1f - jnp.sum(w1f, axis=0, keepdims=True) * (1.0 / C)
        w1p = jnp.concatenate([w1c, jnp.zeros((128 - C, E), f32)], axis=0)
        w1s[...] = _pack(w1p.T)

    def scope1(sbuf, xns):
        def build(row0, k):
            for g in range(G):
                v = pltpu.bitcast(xb[pl.ds(row0 + 2 * k, 2), g].reshape(16, W), u32)
                base = (k % NQ) * SROWS + g * 24
                sbuf[base:base + 8, :] = _shift_r(v, False)
                sbuf[base + 8:base + 16, :] = v
                sbuf[base + 16:base + 24, :] = _shift_l(v, False)

        def conv_var(s0, t):
            ts = slice(t * 128, (t + 1) * 128)
            cv = []
            for g in range(G):
                parts = []
                for sl in (s0, s0 + 1):
                    bb = (sl % NQ) * SROWS + g * 24
                    lft, mid, rgt = (sbuf[bb + 8 * j:bb + 8 * j + 8, ts] for j in range(3))
                    parts += [_zero_lane(lft, 0) if t == 0 else lft, mid,
                              _zero_lane(rgt, 127) if t == NT - 1 else rgt]
                s = _unp(jnp.concatenate(parts, axis=0))
                d = _unp(dmat[8 * g:8 * g + 8, :])[:, :C]
                cv.append(jnp.dot(d, s, preferred_element_type=f32))
            c0 = [v[0:8] for v in cv]
            c1 = [v[8:16] for v in cv]
            return (s0, t, c0, c1, _var2(c0, c1))

        def norm(st, tie=None):
            s0, t, c0, c1, var = st
            if tie is not None:
                never = lax.broadcasted_iota(jnp.int32, (8, 128), 0) < zs[0]
                var = jnp.where(never, tie, var)
            rstd = _rsqrt(var)
            r0 = jnp.broadcast_to(rstd[3:4], (8, 128))
            r1 = jnp.broadcast_to(rstd[7:8], (8, 128))
            ts = slice(t * 128, (t + 1) * 128)
            r = 2 * (s0 % NQ)
            xns[r * CH:(r + 1) * CH, ts] = _pack(jnp.concatenate([c * r0 for c in c0], axis=0))
            xns[(r + 1) * CH:(r + 2) * CH, ts] = _pack(jnp.concatenate([c * r1 for c in c1], axis=0))

        acc[...] = jnp.zeros_like(acc)
        xb[R1] = jnp.zeros((G, 8, W), bf16)
        params[0].wait()
        params[1].wait()
        setup()
        grp_head().wait()
        for k in range(NQ):
            build(R1, k)
        for s0 in range(2):
            for t in range(NT):
                st = conv_var(s0, t)
                norm(st)
                for o in range(2):
                    if 2 * s0 + o in REC:
                        k = REC.index(2 * s0 + o)
                        cbuf[(k + 1) * C:(k + 2) * C, t * 128:(t + 1) * 128] = jnp.concatenate(st[2 + o], axis=0)

        def dma1(i, slot):
            @pl.when(i < NI - 1)
            def _():
                grp(i, slot).wait()

            @pl.when(i == NI - 1)
            def _():
                grp_last().wait()
                xb[R1 * ((NI - 1) % 2) + R1 - TB + 1] = jnp.zeros((G, 8, W), bf16)
                for b0 in range(2):
                    in2(b0, (NI % 2) * U1 + b0).start()

            @pl.when(i + 1 < NI - 1)
            def _():
                grp(i + 1, 1 - slot).start()

            @pl.when(i + 1 == NI - 1)
            def _():
                grp_last().start()

        def block1(b, row0, u, pend):
            n = E // NCH
            for k in range(NQ):
                for t in range(NT):
                    r, c = 2 * k + t // NCH, t % NCH
                    y = jnp.dot(w1t(c * n, n), _unp(xns[r * CH:(r + 1) * CH, :]), preferred_element_type=f32)
                    h = _gelu2(y)
                    h2 = h * h
                    acc[c * n:(c + 1) * n, :] += (h2[:, 0:128] + h2[:, 128:256]) + (h2[:, 256:384] + h2[:, 384:512])
                    if r in STO:
                        row = pl.multiple_of((b * NSTO + STO.index(r)) * EH + c * (n // 2), 8)
                        hbuf[pl.ds(row, n // 2), :] = _pack(h)
                    if pend is not None:
                        norm(pend, y[TIE:TIE + 8, 0:128])
                    pend = conv_var(k + 2, t)
                build(row0, u * NQ + k)
            return pend

        def pass1(i, carry):
            slot = i & 1
            dma1(i, slot)
            pend = None
            for u in range(U1):
                pend = block1(i * U1 + u, slot * R1, u, pend)
            norm(pend)
            return carry

        lax.fori_loop(0, NI, pass1, 0)

    pl.run_scoped(scope1,
                  pltpu.VMEM((NQ * SROWS, W), u32),
                  pltpu.VMEM((TB * CH, W), u32))

    assert NI % 2 == 0 and NX == 4 and max(REC) < 4

    def scope2(ob, hre, dwb, semo):
        def out2(b, slot, half):
            return pltpu.make_async_copy(ob.at[pl.ds(TB * slot + NQ * half, NQ)],
                                         o_hbm.at[pl.ds(TB * b + NQ * half, NQ)], semo.at[slot, half])

        def conv_rec(row0, groups=range(G)):
            for g in groups:
                need = sorted({r + d for r in REC for d in (-1, 0, 1)})
                xs = {q: xb[row0 + q, g].astype(f32) for q in need}
                wt = [_tile4(dwb[tap, 8 * g:8 * g + 8, :]) for tap in range(9)]
                for k, r in enumerate(REC):
                    a = []
                    for j in range(3):
                        t = xs[r - 1] * wt[j]
                        t = t + xs[r] * wt[3 + j]
                        t = t + xs[r + 1] * wt[6 + j]
                        a.append(t)
                    cbuf[(k + 1) * C + 8 * g:(k + 1) * C + 8 * g + 8, :] = _shift_r(a[0]) + a[1] + _shift_l(a[2])

        def ln_rec(k):
            cols = []
            for t in range(NT):
                c = [cbuf[(k + 1) * C + 8 * g:(k + 1) * C + 8 * g + 8, t * 128:(t + 1) * 128] for g in range(G)]
                r = jnp.broadcast_to(lax.rsqrt(_var1(c))[7:8], (8, 128))
                cols.append(jnp.concatenate([v * r for v in c], axis=0))
            return jnp.concatenate(cols, axis=1).astype(bf16)

        in2(2, 2).start()
        for cp in params[2:]:
            cp.wait()
        for tap, col in enumerate(tap_columns()):
            dwb[tap] = col
        ssq = jnp.sum(acc[...].T, axis=0, keepdims=True) * (1.0 / (4.0 * GA * GA))
        gx = jnp.sqrt(ssq + 1e-6)
        nx = gx / (jnp.sum(gx, axis=1, keepdims=True) * (1.0 / E) + 1e-6)
        gam = gam_ref[...].astype(f32).reshape(1, E)
        bet = bet_ref[...].astype(f32).reshape(1, E)
        scale = (gam * nx + 1.0) * (1.0 / (2.0 * GA))
        w2f = w2t_ref[...].astype(f32)
        w2s[...] = _pack(w2f * scale)
        cbuf[0:C, 0:128] = jnp.broadcast_to(jnp.sum(w2f * bet, axis=1, keepdims=True), (C, 128))
        in2(0, 0).wait()

        def pass2(b, carry):
            row0 = (b & 3) * TB
            nrow0 = ((b + 1) & 3) * TB
            oslot = b & 1

            @pl.when(b + 3 < NB)
            def _():
                in2(b + 3, (b + 3) & 3).start()

            @pl.when(b >= 2)
            def _():
                for hf in range(2):
                    out2(b - 2, oslot, hf).wait()

            @pl.when(b + 1 < NB)
            def _():
                in2(b + 1, (b + 1) & 3).wait()

            pending = list(range(G))
            plan = [int(ch) for ch in PLAN]

            def finish(r, hp, ngroups):
                o = jnp.dot(_unp(w2s[...]), _unp(hp), preferred_element_type=f32)
                for hf in range(2):
                    ls = slice(hf * 256, hf * 256 + 256)
                    for j in range((ngroups + 1 - hf) // 2):
                        t = 2 * hf + j
                        xb[row0 + STO[0], zs[0]] = _tile4(o[AR:AR + 8, t * 128:(t + 1) * 128]).astype(bf16)
                        conv_rec(nrow0, [pending.pop(0)])
                    for g in range(G):
                        xr = xb[row0 + r, g, :, ls].astype(f32)
                        bg = cbuf[8 * g:8 * g + 8, 0:128]
                        v = o[8 * g:8 * g + 8, ls] + (xr + jnp.concatenate([bg, bg], axis=1))
                        ob[oslot * TB + r, g, :, ls] = v.astype(bf16)

            def sto(k, ngroups):
                finish(STO[k], hbuf[pl.ds(pl.multiple_of((b * NSTO + k) * EH, 8), EH), :], ngroups)

            sto(0, 0)
            for k in range(NREC):
                y = jnp.dot(w1t(), ln_rec(k), preferred_element_type=f32)
                hre[k * EH:(k + 1) * EH, :] = _pack(_gelu2(y))
            for k in range(1, NSTO):
                sto(k, plan.pop(0))
            out2(b, oslot, 1).start()
            for k in range(NREC):
                finish(REC[k], hre[pl.ds(pl.multiple_of(zs[0] + k * EH, 8), EH), :], plan.pop(0))
            out2(b, oslot, 0).start()
            return carry

        lax.fori_loop(0, NB, pass2, 0)
        for hf in range(2):
            out2(NB - 2, 0, hf).wait()
            out2(NB - 1, 1, hf).wait()

    pl.run_scoped(scope2,
                  pltpu.VMEM((2 * TB, G, 8, W), bf16),
                  pltpu.VMEM((NREC * EH, W), u32),
                  pltpu.VMEM((9, C, 128), f32),
                  pltpu.SemaphoreType.DMA((2, 2)))


@jax.jit
def pallas_standalone__modern_conv_block_convnext_v2__vision_kernel(x, dw, w1, w2, grn_gamma, grn_beta):
    xt = jnp.transpose(x, (0, 1, 3, 2)).reshape(H, G, 8, W)
    w2t = w2.T
    hbm = pl.BlockSpec(memory_space=pl.ANY)
    o = pl.pallas_call(
        kernel,
        out_shape=jax.ShapeDtypeStruct((H, G, 8, W), bf16),
        in_specs=[hbm] * 6,
        out_specs=hbm,
        scratch_shapes=[
            pltpu.VMEM((NB * NSTO * EH, W), u32),
            pltpu.VMEM((NX * TB, G, 8, W), bf16),
            pltpu.VMEM(((NREC + 1) * C, W), f32),
            pltpu.VMEM((C, 128), u32),
            pltpu.VMEM((EH, 128), u32),
            pltpu.VMEM((E, 128), f32),
            pltpu.VMEM((CH, E), u32),
            pltpu.VMEM((C, E), bf16),
            pltpu.VMEM((C, E), bf16),
            pltpu.VMEM((3, 3, C), bf16),
            pltpu.VMEM((E,), bf16),
            pltpu.VMEM((E,), bf16),
            pltpu.VMEM((PADV, 3, C), bf16),
            pltpu.SMEM((1,), jnp.int32),
            pltpu.SemaphoreType.DMA((NX,)),
            pltpu.SemaphoreType.DMA((5,)),
        ],
        compiler_params=pltpu.CompilerParams(vmem_limit_bytes=128 * 1024 * 1024,
                                             disable_bounds_checks=True),
        name="convnext",
    )(xt, dw, w1, w2t, grn_gamma, grn_beta)
    return jnp.transpose(o.reshape(1, H, C, W), (0, 1, 3, 2))
```

```python
import math
import jax
import jax.numpy as jnp
from jax import lax
from jax.experimental import pallas as pl
from jax.experimental.pallas import tpu as pltpu

H = 512
W = 512
C = 96
E = 384
G = C // 8
NT = W // 128
TB = 8
NB = H // TB
NQ = TB // 2
REC = (1, 2, 3)
STO = tuple(r for r in range(TB) if r not in REC)
NSTO = len(STO)
NREC = len(REC)
EH = E // 2
CH = C // 2
SROWS = G * 24
NCH = 2
U1 = 2
R1 = TB * U1
NI = NB // U1
NX = 2 * U1
TIE = 24
PLAN = "2222220"
AR = 0
NEV = "1" == "1"
FOLD = "1" == "1"
NBH = NB


def bh(b):
    return b if NBH == NB else jnp.minimum(b, NBH - 1)


PADV = 15

C0 = math.sqrt(2.0 / math.pi)
C1 = 0.044715
GA = (C0 * C1) ** (1.0 / 3.0)
GK = C0 / GA
LN_EPS = 1e-5

f32 = jnp.float32
bf16 = jnp.bfloat16
u32 = jnp.uint32


def _pack(v):
    return pltpu.bitcast(v.astype(bf16), u32)


def _unp(v):
    return pltpu.bitcast(v, bf16)


def _zero_lane(a, l):
    lane = lax.broadcasted_iota(jnp.int32, a.shape, 1)
    return jnp.where(lane == l, jnp.zeros_like(a), a)


def _shift_r(a, edge=True):
    lane = lax.broadcasted_iota(jnp.int32, (a.shape[0], 128), 1)
    v = [a[:, t * 128:(t + 1) * 128] for t in range(NT)]
    m = [_zero_lane(v[0], 127) if edge else v[0]] + [jnp.concatenate([v[t][:, :127], v[t - 1][:, 127:]], axis=1) for t in range(1, NT)]
    return jnp.concatenate([pltpu.roll(u, 1, 1) for u in m], axis=1)


def _shift_l(a, edge=True):
    lane = lax.broadcasted_iota(jnp.int32, (a.shape[0], 128), 1)
    v = [a[:, t * 128:(t + 1) * 128] for t in range(NT)]
    m = ([jnp.concatenate([v[t + 1][:, :1], v[t][:, 1:]], axis=1) for t in range(NT - 1)]
         + [_zero_lane(v[NT - 1], 0) if edge else v[NT - 1]])
    return jnp.concatenate([pltpu.roll(u, 127, 1) for u in m], axis=1)


def _tile4(v):
    return jnp.concatenate([v] * NT, axis=1)


def _sums(c):
    s1 = c[0]
    s2 = c[0] * c[0]
    for g in range(1, G):
        s1 = s1 + c[g]
        s2 = s2 + c[g] * c[g]
    return s1, s2


def _merge4(a, b):
    p = jnp.concatenate([a[:4], b[4:]], axis=0)
    q = jnp.concatenate([b[:4], a[4:]], axis=0)
    return p + pltpu.roll(q, 4, 0)


def _var_from(n, shift):
    if FOLD:
        eps = LN_EPS * C * C
        return jnp.maximum(n * float(C) + eps - pltpu.roll(n * n, shift, 0), eps)
    eps = LN_EPS / (GA * GA)
    mean = n * (1.0 / (C * GA))
    msq = pltpu.roll(mean * mean, shift, 0)
    return jnp.maximum(n * (1.0 / (C * GA * GA)) + eps - msq, eps)


def _var2(c0, c1):
    a1, a2 = _sums(c0)
    b1, b2 = _sums(c1)
    m1 = _merge4(a1, b1)
    m2 = _merge4(a2, b2)
    sub = lax.broadcasted_iota(jnp.int32, (8, 128), 0)
    n = jnp.where((sub & 2) == 0, m1 + pltpu.roll(m1, 6, 0), m2 + pltpu.roll(m2, 2, 0))
    n = n + pltpu.roll(n, 1, 0)
    return _var_from(n, 2)


def _var1(c):
    s1, s2 = _sums(c)
    n = _merge4(s1, s2)
    n = n + pltpu.roll(n, 2, 0)
    n = n + pltpu.roll(n, 1, 0)
    return _var_from(n, 4)


def _rsqrt(v):
    return jnp.exp2(jnp.log(v) * (-0.5 / math.log(2.0)))


def _gelu2(y):
    u = y * (y * y + GK)
    return y * (jnp.tanh(u) + 1.0)


def kernel(x_hbm, dw_hbm, w1_hbm, w2t_hbm, gam_hbm, bet_hbm, o_hbm,
           hbuf, xb, cbuf, dmat, w1s, acc, w2s, w1_ref, w2t_ref, dw_ref, gam_ref, bet_ref, pad0,
           zs, semx, semp):
    def xcopy(r0, n, d0, sem):
        return pltpu.make_async_copy(x_hbm.at[pl.ds(r0, n)], xb.at[pl.ds(d0, n)], sem)

    def grp_head():
        return xcopy(0, TB - 1, R1 + 1, semx.at[2])

    def grp(i, slot):
        return xcopy(R1 * i + TB - 1, R1, R1 * slot, semx.at[2 * slot])

    def grp_last():
        return xcopy(R1 * (NI - 1) + TB - 1, R1 - TB + 1, R1 * ((NI - 1) % 2), semx.at[2 * ((NI - 1) % 2)])

    def in2(b, slot):
        return xcopy(TB * b, TB, TB * slot, semx.at[slot])

    params = [pltpu.make_async_copy(src, dst, semp.at[j]) for j, (src, dst) in enumerate(
        [(dw_hbm, dw_ref), (w1_hbm, w1_ref), (w2t_hbm, w2t_ref), (gam_hbm, gam_ref), (bet_hbm, bet_ref)])]
    for cp in params[:2] + [grp_head()] + params[2:] + [grp(0, 0)]:
        cp.start()
    zs[0] = 0
    pad0[...] = jnp.zeros_like(pad0)

    def w1t(c0=0, n=E):
        return _unp(w1s[c0 // 2:(c0 + n) // 2, :])[:, :C]

    def tap_columns():
        sub = lax.broadcasted_iota(jnp.int32, (C, C), 0)
        lan = lax.broadcasted_iota(jnp.int32, (C, C), 1)
        eye = sub == lan
        diags = [jnp.where(eye, jnp.broadcast_to(dw_ref[i, j:j + 1, :].astype(f32), (C, C)), 0.0)
                 for i in range(3) for j in range(3)]
        ones = jnp.ones((C, 128), bf16)
        return [jnp.dot(d.astype(bf16), ones, preferred_element_type=f32) for d in diags]

    def setup():
        cols = tap_columns()
        c_ = lax.broadcasted_iota(jnp.int32, (8, 128), 0)
        k_ = lax.broadcasted_iota(jnp.int32, (8, 128), 1)
        for g in range(G):
            halves = []
            for o in range(2):
                d = jnp.zeros((8, 128), f32)
                for i in range(3):
                    ri = i + o
                    for j in range(3):
                        kpos = (ri // 2) * 48 + j * 16 + (ri % 2) * 8
                        d = jnp.where(k_ == c_ + kpos, cols[i * 3 + j][8 * g:8 * g + 8], d)
                halves.append(d)
            dmat[8 * g:8 * g + 8, :] = _pack(jnp.concatenate(halves, axis=0))
        w1f = w1_ref[...].astype(f32)
        w1c = w1f - jnp.sum(w1f, axis=0, keepdims=True) * (1.0 / C)
        if FOLD:
            w1c = w1c * (GA * C)
        w1p = jnp.concatenate([w1c, jnp.zeros((128 - C, E), f32)], axis=0)
        w1s[...] = _pack(w1p.T)

    def scope1(sbuf, xns):
        def build(row0, k):
            for g in range(G):
                v = pltpu.bitcast(xb[pl.ds(row0 + 2 * k, 2), g].reshape(16, W), u32)
                base = (k % NQ) * SROWS + g * 24
                sbuf[base:base + 8, :] = _shift_r(v, False)
                sbuf[base + 8:base + 16, :] = v
                sbuf[base + 16:base + 24, :] = _shift_l(v, False)

        def conv_mm(s0, t, g):
            ts = slice(t * 128, (t + 1) * 128)
            parts = []
            for sl in (s0, s0 + 1):
                bb = (sl % NQ) * SROWS + g * 24
                lft, mid, rgt = (sbuf[bb + 8 * j:bb + 8 * j + 8, ts] for j in range(3))
                parts += [_zero_lane(lft, 0) if t == 0 else lft, mid,
                          _zero_lane(rgt, 127) if t == NT - 1 else rgt]
            s = _unp(jnp.concatenate(parts, axis=0))
            d = _unp(dmat[8 * g:8 * g + 8, :])[:, :C]
            return jnp.dot(d, s, preferred_element_type=f32)

        def stats(s0, t, cv):
            c0 = [v[0:8] for v in cv]
            c1 = [v[8:16] for v in cv]
            return (s0, t, c0, c1, _var2(c0, c1))

        def conv_var(s0, t):
            return stats(s0, t, [conv_mm(s0, t, g) for g in range(G)])

        def norm(st, tie=None, never=None):
            s0, t, c0, c1, var = st
            if tie is not None:
                if never is None:
                    never = lax.broadcasted_iota(jnp.int32, (8, 128), 0) < zs[0]
                var = jnp.where(never, tie, var)
            rstd = _rsqrt(var)
            r0 = jnp.broadcast_to(rstd[3:4], (8, 128))
            r1 = jnp.broadcast_to(rstd[7:8], (8, 128))
            ts = slice(t * 128, (t + 1) * 128)
            r = 2 * (s0 % NQ)
            xns[r * CH:(r + 1) * CH, ts] = _pack(jnp.concatenate([c * r0 for c in c0], axis=0))
            xns[(r + 1) * CH:(r + 2) * CH, ts] = _pack(jnp.concatenate([c * r1 for c in c1], axis=0))

        acc[...] = jnp.zeros_like(acc)
        xb[R1] = jnp.zeros((G, 8, W), bf16)
        params[0].wait()
        params[1].wait()
        setup()
        grp_head().wait()
        for k in range(NQ):
            build(R1, k)
        for s0 in range(2):
            for t in range(NT):
                st = conv_var(s0, t)
                norm(st)
                for o in range(2):
                    if 2 * s0 + o in REC:
                        k = REC.index(2 * s0 + o)
                        cbuf[(k + 1) * C:(k + 2) * C, t * 128:(t + 1) * 128] = jnp.concatenate(st[2 + o], axis=0)

        def dma1(i, slot):
            @pl.when(i < NI - 1)
            def _():
                grp(i, slot).wait()

            @pl.when(i == NI - 1)
            def _():
                grp_last().wait()
                xb[R1 * ((NI - 1) % 2) + R1 - TB + 1] = jnp.zeros((G, 8, W), bf16)
                for b0 in range(2):
                    in2(b0, (NI % 2) * U1 + b0).start()

            @pl.when(i + 1 < NI - 1)
            def _():
                grp(i + 1, 1 - slot).start()

            @pl.when(i + 1 == NI - 1)
            def _():
                grp_last().start()

        def block1(b, row0, u, pend, never):
            n = E // NCH
            per = NT * G // (2 * NCH)
            for k in range(NQ):
                todo = [(t, g) for t in range(NT) for g in range(G)]
                cv = []
                for j in range(2 * NCH):
                    r, c = 2 * k + j // NCH, j % NCH
                    y = jnp.dot(w1t(c * n, n), _unp(xns[r * CH:(r + 1) * CH, :]), preferred_element_type=f32)
                    h = _gelu2(y)
                    h2 = h * h
                    acc[c * n:(c + 1) * n, :] += (h2[:, 0:128] + h2[:, 128:256]) + (h2[:, 256:384] + h2[:, 384:512])
                    if r in STO:
                        row = pl.multiple_of((bh(b) * NSTO + STO.index(r)) * EH + c * (n // 2), 8)
                        hbuf[pl.ds(row, n // 2), :] = _pack(h)
                    if pend is not None:
                        norm(pend, y[TIE:TIE + 8, 0:128], never)
                        pend = None
                    for _ in range(per):
                        t, g = todo.pop(0)
                        cv.append(conv_mm(k + 2, t, g))
                        if g == G - 1:
                            pend = stats(k + 2, t, cv)
                            cv = []
                build(row0, u * NQ + k)
            return pend

        def pass1(i, carry):
            slot = i & 1
            dma1(i, slot)
            pend = None
            never = (lax.broadcasted_iota(jnp.int32, (8, 128), 0) < zs[0]) if NEV else None
            for u in range(U1):
                pend = block1(i * U1 + u, slot * R1, u, pend, never)
            norm(pend)
            return carry

        lax.fori_loop(0, NI, pass1, 0)

    pl.run_scoped(scope1,
                  pltpu.VMEM((NQ * SROWS, W), u32),
                  pltpu.VMEM((TB * CH, W), u32))

    assert NI % 2 == 0 and NX == 4 and max(REC) < 4

    def scope2(ob, hre, dwb, semo):
        def out2(b, slot, half):
            return pltpu.make_async_copy(ob.at[pl.ds(TB * slot + NQ * half, NQ)],
                                         o_hbm.at[pl.ds(TB * b + NQ * half, NQ)], semo.at[slot, half])

        def conv_rec(row0, groups=range(G)):
            for g in groups:
                need = sorted({r + d for r in REC for d in (-1, 0, 1)})
                xs = {q: xb[row0 + q, g].astype(f32) for q in need}
                wt = [_tile4(dwb[tap, 8 * g:8 * g + 8, :]) for tap in range(9)]
                for k, r in enumerate(REC):
                    a = []
                    for j in range(3):
                        t = xs[r - 1] * wt[j]
                        t = t + xs[r] * wt[3 + j]
                        t = t + xs[r + 1] * wt[6 + j]
                        a.append(t)
                    cbuf[(k + 1) * C + 8 * g:(k + 1) * C + 8 * g + 8, :] = _shift_r(a[0]) + a[1] + _shift_l(a[2])

        def ln_rec(k):
            cols = []
            for t in range(NT):
                c = [cbuf[(k + 1) * C + 8 * g:(k + 1) * C + 8 * g + 8, t * 128:(t + 1) * 128] for g in range(G)]
                r = jnp.broadcast_to(lax.rsqrt(_var1(c))[7:8], (8, 128))
                cols.append(jnp.concatenate([v * r for v in c], axis=0))
            return jnp.concatenate(cols, axis=1).astype(bf16)

        in2(2, 2).start()
        for cp in params[2:]:
            cp.wait()
        for tap, col in enumerate(tap_columns()):
            dwb[tap] = col
        ssq = jnp.sum(acc[...].T, axis=0, keepdims=True) * (1.0 / (4.0 * GA * GA))
        gx = jnp.sqrt(ssq + 1e-6)
        nx = gx / (jnp.sum(gx, axis=1, keepdims=True) * (1.0 / E) + 1e-6)
        gam = gam_ref[...].astype(f32).reshape(1, E)
        bet = bet_ref[...].astype(f32).reshape(1, E)
        scale = (gam * nx + 1.0) * (1.0 / (2.0 * GA))
        w2f = w2t_ref[...].astype(f32)
        w2s[...] = _pack(w2f * scale)
        cbuf[0:C, 0:128] = jnp.broadcast_to(jnp.sum(w2f * bet, axis=1, keepdims=True), (C, 128))
        in2(0, 0).wait()

        def pass2(b, carry):
            row0 = (b & 3) * TB
            nrow0 = ((b + 1) & 3) * TB
            oslot = b & 1

            @pl.when(b + 3 < NB)
            def _():
                in2(b + 3, (b + 3) & 3).start()

            @pl.when(b >= 2)
            def _():
                for hf in range(2):
                    out2(b - 2, oslot, hf).wait()

            @pl.when(b + 1 < NB)
            def _():
                in2(b + 1, (b + 1) & 3).wait()

            pending = list(range(G))
            plan = [int(ch) for ch in PLAN]

            def finish(r, hp, ngroups):
                o = jnp.dot(_unp(w2s[...]), _unp(hp), preferred_element_type=f32)
                for hf in range(2):
                    ls = slice(hf * 256, hf * 256 + 256)
                    for j in range((ngroups + 1 - hf) // 2):
                        t = 2 * hf + j
                        xb[row0 + STO[0], zs[0]] = _tile4(o[AR:AR + 8, t * 128:(t + 1) * 128]).astype(bf16)
                        conv_rec(nrow0, [pending.pop(0)])
                    for g in range(G):
                        xr = xb[row0 + r, g, :, ls].astype(f32)
                        bg = cbuf[8 * g:8 * g + 8, 0:128]
                        v = o[8 * g:8 * g + 8, ls] + (xr + jnp.concatenate([bg, bg], axis=1))
                        ob[oslot * TB + r, g, :, ls] = v.astype(bf16)

            def sto(k, ngroups):
                finish(STO[k], hbuf[pl.ds(pl.multiple_of((bh(b) * NSTO + k) * EH, 8), EH), :], ngroups)

            sto(0, 0)
            for k in range(NREC):
                y = jnp.dot(w1t(), ln_rec(k), preferred_element_type=f32)
                hre[k * EH:(k + 1) * EH, :] = _pack(_gelu2(y))
            for k in range(1, NSTO):
                sto(k, plan.pop(0))
            out2(b, oslot, 1).start()
            for k in range(NREC):
                finish(REC[k], hre[pl.ds(pl.multiple_of(zs[0] + k * EH, 8), EH), :], plan.pop(0))
            out2(b, oslot, 0).start()
            return carry

        lax.fori_loop(0, NB, pass2, 0)
        for hf in range(2):
            out2(NB - 2, 0, hf).wait()
            out2(NB - 1, 1, hf).wait()

    pl.run_scoped(scope2,
                  pltpu.VMEM((2 * TB, G, 8, W), bf16),
                  pltpu.VMEM((NREC * EH, W), u32),
                  pltpu.VMEM((9, C, 128), f32),
                  pltpu.SemaphoreType.DMA((2, 2)))


@jax.jit
def pallas_standalone__modern_conv_block_convnext_v2__vision_kernel(x, dw, w1, w2, grn_gamma, grn_beta):
    xt = jnp.transpose(x, (0, 1, 3, 2)).reshape(H, G, 8, W)
    w2t = w2.T
    hbm = pl.BlockSpec(memory_space=pl.ANY)
    o = pl.pallas_call(
        kernel,
        out_shape=jax.ShapeDtypeStruct((H, G, 8, W), bf16),
        in_specs=[hbm] * 6,
        out_specs=hbm,
        scratch_shapes=[
            pltpu.VMEM((NBH * NSTO * EH, W), u32),
            pltpu.VMEM((NX * TB, G, 8, W), bf16),
            pltpu.VMEM(((NREC + 1) * C, W), f32),
            pltpu.VMEM((C, 128), u32),
            pltpu.VMEM((EH, 128), u32),
            pltpu.VMEM((E, 128), f32),
            pltpu.VMEM((CH, E), u32),
            pltpu.VMEM((C, E), bf16),
            pltpu.VMEM((C, E), bf16),
            pltpu.VMEM((3, 3, C), bf16),
            pltpu.VMEM((E,), bf16),
            pltpu.VMEM((E,), bf16),
            pltpu.VMEM((PADV, 3, C), bf16),
            pltpu.SMEM((1,), jnp.int32),
            pltpu.SemaphoreType.DMA((NX,)),
            pltpu.SemaphoreType.DMA((5,)),
        ],
        compiler_params=pltpu.CompilerParams(vmem_limit_bytes=128 * 1024 * 1024,
                                             disable_bounds_checks=True),
        name="convnext",
    )(xt, dw, w1, w2t, grn_gamma, grn_beta)
    return jnp.transpose(o.reshape(1, H, C, W), (0, 1, 3, 2))
```

```python
import math

import jax
import jax.numpy as jnp
from jax import lax
from jax.experimental import pallas as pl
from jax.experimental.pallas import tpu as pltpu

H = 512
W = 512
C = 96
E = 384
G = C // 8
NT = W // 128
TB = 8
NB = H // TB
NQ = TB // 2
REC = (1, 2, 3)
STO = tuple(r for r in range(TB) if r not in REC)
NSTO = len(STO)
NREC = len(REC)
EH = E // 2
CH = C // 2
SROWS = G * 24
NCH = 3
U1 = 2
R1 = TB * U1
NI = NB // U1
NX = 2 * U1
TIE = 40
PLAN = (2, 2, 2, 2, 2, 2, 0)
PADV = 15

C0 = math.sqrt(2.0 / math.pi)
C1 = 0.044715
GA = (C0 * C1) ** (1.0 / 3.0)
GK = C0 / GA
LN_EPS = 1e-5

f32 = jnp.float32
bf16 = jnp.bfloat16
u32 = jnp.uint32


def _pack(v):
    return pltpu.bitcast(v.astype(bf16), u32)


def _unp(v):
    return pltpu.bitcast(v, bf16)


def _tiles(a):
    return [a[:, t * 128:(t + 1) * 128] for t in range(NT)]


def _zero_lane(a, l):
    lane = lax.broadcasted_iota(jnp.int32, a.shape, 1)
    return jnp.where(lane == l, jnp.zeros_like(a), a)


def _shift_r(a):
    v = _tiles(a)
    m = [_zero_lane(v[0], 127)] + [jnp.concatenate([v[t][:, :127], v[t - 1][:, 127:]], axis=1)
                                   for t in range(1, NT)]
    return jnp.concatenate([pltpu.roll(u, 1, 1) for u in m], axis=1)


def _shift_l(a, edge=True):
    v = _tiles(a)
    m = ([jnp.concatenate([v[t + 1][:, :1], v[t][:, 1:]], axis=1) for t in range(NT - 1)]
         + [_zero_lane(v[NT - 1], 0) if edge else v[NT - 1]])
    return jnp.concatenate([pltpu.roll(u, 127, 1) for u in m], axis=1)


def _sums(c):
    s1 = c[0]
    s2 = c[0] * c[0]
    for g in range(1, G):
        s1 = s1 + c[g]
        s2 = s2 + c[g] * c[g]
    return s1, s2


def _merge4(a, b):
    p = jnp.concatenate([a[:4], b[4:]], axis=0)
    q = jnp.concatenate([b[:4], a[4:]], axis=0)
    return p + pltpu.roll(q, 4, 0)


def _var_from(n, shift):
    eps = LN_EPS * C * C
    return jnp.maximum(n * float(C) + eps - pltpu.roll(n * n, shift, 0), eps)


def _var2(c0, c1):
    a1, a2 = _sums(c0)
    b1, b2 = _sums(c1)
    m1 = _merge4(a1, b1)
    m2 = _merge4(a2, b2)
    sub = lax.broadcasted_iota(jnp.int32, (8, 128), 0)
    n = jnp.where((sub & 2) == 0, m1 + pltpu.roll(m1, 6, 0), m2 + pltpu.roll(m2, 2, 0))
    n = n + pltpu.roll(n, 1, 0)
    return _var_from(n, 2)


def _var1(c):
    s1, s2 = _sums(c)
    n = _merge4(s1, s2)
    n = n + pltpu.roll(n, 2, 0)
    n = n + pltpu.roll(n, 1, 0)
    return _var_from(n, 4)


def _rsqrt(v):
    return jnp.exp2(jnp.log(v) * (-0.5 / math.log(2.0)))


def _gelu2(y):
    u = y * (y * y + GK)
    return y * (jnp.tanh(u) + 1.0)


def _kernel(x_hbm, dw_hbm, w1_hbm, w2t_hbm, gam_hbm, bet_hbm, o_hbm,
            hbuf, xb, cbuf, dmat, w1s, acc, w2s, w1_ref, w2t_ref, dw_ref, gam_ref, bet_ref, pad,
            zs, semx, semp):
    def xcopy(r0, n, d0, sem):
        return pltpu.make_async_copy(x_hbm.at[pl.ds(r0, n)], xb.at[pl.ds(d0, n)], sem)

    def grp_head():
        return xcopy(0, TB - 1, R1 + 1, semx.at[2])

    def grp(i, slot):
        return xcopy(R1 * i + TB - 1, R1, R1 * slot, semx.at[2 * slot])

    def grp_last():
        return xcopy(R1 * (NI - 1) + TB - 1, R1 - TB + 1, R1 * ((NI - 1) % 2), semx.at[2 * ((NI - 1) % 2)])

    def in2(b, slot):
        return xcopy(TB * b, TB, TB * slot, semx.at[slot])

    params = [pltpu.make_async_copy(src, dst, semp.at[j]) for j, (src, dst) in enumerate(
        [(dw_hbm, dw_ref), (w1_hbm, w1_ref), (w2t_hbm, w2t_ref), (gam_hbm, gam_ref), (bet_hbm, bet_ref)])]
    for cp in params[:2] + [grp_head()] + params[2:] + [grp(0, 0)]:
        cp.start()
    zs[0] = 0
    pad[...] = jnp.zeros_like(pad)

    def w1t(c0=0, n=E):
        return _unp(w1s[c0 // 2:(c0 + n) // 2, :])[:, :C]

    def tap_columns():
        sub = lax.broadcasted_iota(jnp.int32, (C, C), 0)
        lan = lax.broadcasted_iota(jnp.int32, (C, C), 1)
        eye = sub - lan == zs[0]
        diags = [jnp.where(eye, jnp.broadcast_to(dw_ref[i, j:j + 1, :].astype(f32), (C, C)), 0.0)
                 for i in range(3) for j in range(3)]
        ones = jnp.ones((C, 128), bf16)
        return [jnp.dot(d.astype(bf16), ones, preferred_element_type=f32) for d in diags]

    def setup():
        cols = tap_columns()
        c_ = lax.broadcasted_iota(jnp.int32, (8, 128), 0)
        k_ = lax.broadcasted_iota(jnp.int32, (8, 128), 1)
        for g in range(G):
            halves = []
            for o in range(2):
                d = jnp.zeros((8, 128), f32)
                for i in range(3):
                    ri = i + o
                    for j in range(3):
                        for jj in ((0, 3) if j == 0 else (j,)):
                            kpos = (ri // 2) * 64 + jj * 16 + (ri % 2) * 8
                            d = jnp.where(k_ == c_ + kpos, cols[i * 3 + j][8 * g:8 * g + 8], d)
                halves.append(d)
            dmat[8 * g:8 * g + 8, :] = _pack(jnp.concatenate(halves, axis=0))
        w1f = w1_ref[...].astype(f32)
        w1c = w1f - jnp.sum(w1f, axis=0, keepdims=True) * (1.0 / C)
        w1c = w1c * (GA * C)
        w1p = jnp.concatenate([w1c, jnp.zeros((128 - C, E), f32)], axis=0)
        w1s[...] = _pack(w1p.T)

    def scope1(sbuf, xns):
        def build(row0, k):
            for g in range(G):
                v = pltpu.bitcast(xb[pl.ds(row0 + 2 * k, 2), g].reshape(16, W), u32)
                base = (k % NQ) * SROWS + g * 24
                sbuf[base:base + 8, :] = jnp.concatenate([pltpu.roll(u, 1, 1) for u in _tiles(v)], axis=1)
                sbuf[base + 8:base + 16, :] = v
                sbuf[base + 16:base + 24, :] = _shift_l(v, False)

        def conv_mm(s0, t, g):
            ts = slice(t * 128, (t + 1) * 128)
            parts = []
            for sl in (s0, s0 + 1):
                bb = (sl % NQ) * SROWS + g * 24
                lft, mid, rgt = (sbuf[bb + 8 * j:bb + 8 * j + 8, ts] for j in range(3))
                seam = jnp.zeros((8, 128), u32)
                if t > 0:
                    lane = lax.broadcasted_iota(jnp.int32, (8, 128), 1)
                    seam = jnp.where(lane > 0, seam, sbuf[bb:bb + 8, (t - 1) * 128:t * 128])
                parts += [_zero_lane(lft, 0), mid, _zero_lane(rgt, 127) if t == NT - 1 else rgt, seam]
            s = _unp(jnp.concatenate(parts, axis=0))
            d = _unp(dmat[8 * g:8 * g + 8, :])
            return jnp.dot(d, s, preferred_element_type=f32)

        def stats(s0, t, cv):
            c0 = [v[0:8] for v in cv]
            c1 = [v[8:16] for v in cv]
            return (s0, t, c0, c1, _var2(c0, c1))

        def norm(st, tie=None, never=None):
            s0, t, c0, c1, var = st
            if tie is not None:
                var = jnp.where(never, tie, var)
            rstd = _rsqrt(var)
            r0 = jnp.broadcast_to(rstd[3:4], (8, 128))
            r1 = jnp.broadcast_to(rstd[7:8], (8, 128))
            ts = slice(t * 128, (t + 1) * 128)
            r = 2 * (s0 % NQ)
            xns[r * CH:(r + 1) * CH, ts] = _pack(jnp.concatenate([c * r0 for c in c0], axis=0))
            xns[(r + 1) * CH:(r + 2) * CH, ts] = _pack(jnp.concatenate([c * r1 for c in c1], axis=0))

        acc[...] = jnp.zeros_like(acc)
        xb[R1] = jnp.zeros((G, 8, W), bf16)
        params[0].wait()
        params[1].wait()
        setup()
        grp_head().wait()
        for k in range(NQ):
            build(R1, k)
        for s0 in range(2):
            for t in range(NT):
                st = stats(s0, t, [conv_mm(s0, t, g) for g in range(G)])
                norm(st)
                for o in range(2):
                    if 2 * s0 + o in REC:
                        k = REC.index(2 * s0 + o)
                        cbuf[k * C:(k + 1) * C, t * 128:(t + 1) * 128] = jnp.concatenate(st[2 + o], axis=0)

        def dma1(i, slot):
            @pl.when(i < NI - 1)
            def _():
                grp(i, slot).wait()

            @pl.when(i == NI - 1)
            def _():
                grp_last().wait()
                xb[R1 * ((NI - 1) % 2) + R1 - TB + 1] = jnp.zeros((G, 8, W), bf16)
                for b0 in range(2):
                    in2(b0, (NI % 2) * U1 + b0).start()

            @pl.when(i + 1 < NI - 1)
            def _():
                grp(i + 1, 1 - slot).start()

            @pl.when(i + 1 == NI - 1)
            def _():
                grp_last().start()

        def block1(b, row0, u, pend, never):
            n = E // NCH
            per = NT * G // (2 * NCH)
            for k in range(NQ):
                todo = [(t, g) for t in range(NT) for g in range(G)]
                cv = []
                for j in range(2 * NCH):
                    r, c = 2 * k + j // NCH, j % NCH
                    y = jnp.dot(w1t(c * n, n), _unp(xns[r * CH:(r + 1) * CH, :]), preferred_element_type=f32)
                    h = _gelu2(y)
                    h2 = _tiles(h * h)
                    acc[c * n:(c + 1) * n, :] += (h2[0] + h2[1]) + (h2[2] + h2[3])
                    if r in STO:
                        row = pl.multiple_of((b * NSTO + STO.index(r)) * EH + c * (n // 2), 8)
                        hbuf[pl.ds(row, n // 2), :] = _pack(h)
                    if pend is not None:
                        norm(pend, y[TIE:TIE + 8, 0:128], never)
                        pend = None
                    for _ in range(per):
                        t, g = todo.pop(0)
                        cv.append(conv_mm(k + 2, t, g))
                        if g == G - 1:
                            pend = stats(k + 2, t, cv)
                            cv = []
                build(row0, u * NQ + k)
            return pend

        def pass1(i, carry):
            slot = i & 1
            dma1(i, slot)
            never = lax.broadcasted_iota(jnp.int32, (8, 128), 0) < zs[0]
            pend = None
            for u in range(U1):
                pend = block1(i * U1 + u, slot * R1, u, pend, never)
            norm(pend)
            return carry

        lax.fori_loop(0, NI, pass1, 0)

    pl.run_scoped(scope1,
                  pltpu.VMEM((NQ * SROWS, W), u32),
                  pltpu.VMEM((TB * CH, W), u32))

    assert NI % 2 == 0 and NX == 4 and max(REC) < NQ

    def scope2(ob, hre, dwb, semo):
        def out2(b, slot, half):
            return pltpu.make_async_copy(ob.at[pl.ds(TB * slot + NQ * half, NQ)],
                                         o_hbm.at[pl.ds(TB * b + NQ * half, NQ)], semo.at[slot, half])

        def conv_rec(row0, g):
            need = sorted({r + d for r in REC for d in (-1, 0, 1)})
            xs = {q: xb[row0 + q, g].astype(f32) for q in need}
            wt = [jnp.concatenate([dwb[tap, 8 * g:8 * g + 8, :]] * NT, axis=1) for tap in range(9)]
            for k, r in enumerate(REC):
                a = []
                for j in range(3):
                    t = xs[r - 1] * wt[j]
                    t = t + xs[r] * wt[3 + j]
                    t = t + xs[r + 1] * wt[6 + j]
                    a.append(t)
                cbuf[k * C + 8 * g:k * C + 8 * g + 8, :] = _shift_r(a[0]) + a[1] + _shift_l(a[2])

        def ln_rec(k):
            cols = []
            for t in range(NT):
                c = [cbuf[k * C + 8 * g:k * C + 8 * g + 8, t * 128:(t + 1) * 128] for g in range(G)]
                r = jnp.broadcast_to(lax.rsqrt(_var1(c))[7:8], (8, 128))
                cols.append(jnp.concatenate([v * r for v in c], axis=0))
            return jnp.concatenate(cols, axis=1).astype(bf16)

        in2(2, 2).start()
        for cp in params[2:]:
            cp.wait()
        for tap, col in enumerate(tap_columns()):
            dwb[tap] = col
        ssq = jnp.sum(acc[...].T, axis=0, keepdims=True) * (1.0 / (4.0 * GA * GA))
        gx = jnp.sqrt(ssq + 1e-6)
        nx = gx / (jnp.sum(gx, axis=1, keepdims=True) * (1.0 / E) + 1e-6)
        gam = gam_ref[...].astype(f32).reshape(1, E)
        bet = bet_ref[...].astype(f32).reshape(1, E)
        scale = (gam * nx + 1.0) * (1.0 / (2.0 * GA))
        w2f = w2t_ref[...].astype(f32)
        w2s[...] = _pack(w2f * scale)
        dwb[9] = jnp.broadcast_to(jnp.sum(w2f * bet, axis=1, keepdims=True), (C, 128))
        in2(0, 0).wait()

        def pass2(b, carry):
            row0 = (b & 3) * TB
            nrow0 = ((b + 1) & 3) * TB
            oslot = b & 1

            @pl.when(b + 3 < NB)
            def _():
                in2(b + 3, (b + 3) & 3).start()

            @pl.when(b >= 2)
            def _():
                for hf in range(2):
                    out2(b - 2, oslot, hf).wait()

            @pl.when(b + 1 < NB)
            def _():
                in2(b + 1, (b + 1) & 3).wait()

            pending = list(range(G))
            plan = list(PLAN)

            def finish(r, hp, ngroups):
                o = jnp.dot(_unp(w2s[...]), _unp(hp), preferred_element_type=f32)
                for hf in range(2):
                    ls = slice(hf * 256, hf * 256 + 256)
                    for j in range((ngroups + 1 - hf) // 2):
                        t = 2 * hf + j
                        mark = o[0:8, t * 128:(t + 1) * 128]
                        xb[row0 + STO[0], zs[0]] = jnp.concatenate([mark] * NT, axis=1).astype(bf16)
                        conv_rec(nrow0, pending.pop(0))
                    for g in range(G):
                        xr = xb[row0 + r, g, :, ls].astype(f32)
                        bg = dwb[9, 8 * g:8 * g + 8, :]
                        v = o[8 * g:8 * g + 8, ls] + (xr + jnp.concatenate([bg, bg], axis=1))
                        ob[oslot * TB + r, g, :, ls] = v.astype(bf16)

            def sto(k, ngroups):
                finish(STO[k], hbuf[pl.ds(pl.multiple_of((b * NSTO + k) * EH, 8), EH), :], ngroups)

            sto(0, 0)
            for k in range(NREC):
                y = jnp.dot(w1t(), ln_rec(k), preferred_element_type=f32)
                hre[k * EH:(k + 1) * EH, :] = _pack(_gelu2(y))
            for k in range(1, NSTO):
                sto(k, plan.pop(0))
            out2(b, oslot, 1).start()
            for k in range(NREC):
                finish(REC[k], hre[pl.ds(pl.multiple_of(zs[0] + k * EH, 8), EH), :], plan.pop(0))
            out2(b, oslot, 0).start()
            return carry

        lax.fori_loop(0, NB, pass2, 0)
        for hf in range(2):
            out2(NB - 2, 0, hf).wait()
            out2(NB - 1, 1, hf).wait()

    pl.run_scoped(scope2,
                  pltpu.VMEM((2 * TB, G, 8, W), bf16),
                  pltpu.VMEM((NREC * EH, W), u32),
                  pltpu.VMEM((10, C, 128), f32),
                  pltpu.SemaphoreType.DMA((2, 2)))


@jax.jit
def pallas_standalone__modern_conv_block_convnext_v2__vision_kernel(
    x: jax.Array,
    dw: jax.Array,
    w1: jax.Array,
    w2: jax.Array,
    grn_gamma: jax.Array,
    grn_beta: jax.Array,
):
    xt = jnp.transpose(x, (0, 1, 3, 2)).reshape(H, G, 8, W)
    hbm = pl.BlockSpec(memory_space=pl.ANY)
    o = pl.pallas_call(
        _kernel,
        out_shape=jax.ShapeDtypeStruct((H, G, 8, W), bf16),
        in_specs=[hbm] * 6,
        out_specs=hbm,
        scratch_shapes=[
            pltpu.VMEM((NB * NSTO * EH, W), u32),
            pltpu.VMEM((NX * TB, G, 8, W), bf16),
            pltpu.VMEM((NREC * C, W), f32),
            pltpu.VMEM((C, 128), u32),
            pltpu.VMEM((EH, 128), u32),
            pltpu.VMEM((E, 128), f32),
            pltpu.VMEM((CH, E), u32),
            pltpu.VMEM((C, E), bf16),
            pltpu.VMEM((C, E), bf16),
            pltpu.VMEM((3, 3, C), bf16),
            pltpu.VMEM((E,), bf16),
            pltpu.VMEM((E,), bf16),
            pltpu.VMEM((PADV, 3, C), bf16),
            pltpu.SMEM((1,), jnp.int32),
            pltpu.SemaphoreType.DMA((NX,)),
            pltpu.SemaphoreType.DMA((5,)),
        ],
        compiler_params=pltpu.CompilerParams(vmem_limit_bytes=128 * 1024 * 1024,
                                             disable_bounds_checks=True),
        name="convnext",
    )(xt, dw, w1, w2.T, grn_gamma, grn_beta)
    return jnp.transpose(o.reshape(1, H, C, W), (0, 1, 3, 2))
```

```python
import math

import jax
import jax.numpy as jnp
from jax import lax
from jax.experimental import pallas as pl
from jax.experimental.pallas import tpu as pltpu

H = 512
W = 512
C = 96
E = 384
G = C // 8
NT = W // 128
TB = 8
NB = H // TB
NQ = TB // 2
REC = (1, 2, 3)
STO = tuple(r for r in range(TB) if r not in REC)
NSTO = len(STO)
NREC = len(REC)
EH = E // 2
CH = C // 2
SROWS = G * 24
NCH = 3
U1 = 2
R1 = TB * U1
NI = NB // U1
NX = 2 * U1
TIE = 40
PLAN = (2, 2, 2, 2, 2, 2, 0)
PADV = 7

C0 = math.sqrt(2.0 / math.pi)
C1 = 0.044715
GA = (C0 * C1) ** (1.0 / 3.0)
GK = C0 / GA
LN_EPS = 1e-5

f32 = jnp.float32
bf16 = jnp.bfloat16
u32 = jnp.uint32


def _pack(v):
    return pltpu.bitcast(v.astype(bf16), u32)


def _unp(v):
    return pltpu.bitcast(v, bf16)


def _tiles(a):
    return [a[:, t * 128:(t + 1) * 128] for t in range(NT)]


def _zero_lane(a, l):
    lane = lax.broadcasted_iota(jnp.int32, a.shape, 1)
    return jnp.where(lane == l, jnp.zeros_like(a), a)


def _shift_r(a):
    v = _tiles(a)
    m = [_zero_lane(v[0], 127)] + [jnp.concatenate([v[t][:, :127], v[t - 1][:, 127:]], axis=1)
                                   for t in range(1, NT)]
    return jnp.concatenate([pltpu.roll(u, 1, 1) for u in m], axis=1)


def _shift_l(a, edge=True):
    v = _tiles(a)
    m = ([jnp.concatenate([v[t + 1][:, :1], v[t][:, 1:]], axis=1) for t in range(NT - 1)]
         + [_zero_lane(v[NT - 1], 0) if edge else v[NT - 1]])
    return jnp.concatenate([pltpu.roll(u, 127, 1) for u in m], axis=1)


def _sums(c):
    s1 = c[0]
    s2 = c[0] * c[0]
    for g in range(1, G):
        s1 = s1 + c[g]
        s2 = s2 + c[g] * c[g]
    return s1, s2


def _merge4(a, b):
    p = jnp.concatenate([a[:4], b[4:]], axis=0)
    q = jnp.concatenate([b[:4], a[4:]], axis=0)
    return p + pltpu.roll(q, 4, 0)


def _var_from(n, shift):
    eps = LN_EPS * C * C
    return jnp.maximum(n * float(C) + eps - pltpu.roll(n * n, shift, 0), eps)


def _var2(c0, c1):
    a1, a2 = _sums(c0)
    b1, b2 = _sums(c1)
    m1 = _merge4(a1, b1)
    m2 = _merge4(a2, b2)
    sub = lax.broadcasted_iota(jnp.int32, (8, 128), 0)
    n = jnp.where((sub & 2) == 0, m1 + pltpu.roll(m1, 6, 0), m2 + pltpu.roll(m2, 2, 0))
    n = n + pltpu.roll(n, 1, 0)
    return _var_from(n, 2)


def _var1(c):
    s1, s2 = _sums(c)
    n = _merge4(s1, s2)
    n = n + pltpu.roll(n, 2, 0)
    n = n + pltpu.roll(n, 1, 0)
    return _var_from(n, 4)


def _rsqrt(v):
    return jnp.exp2(jnp.log(v) * (-0.5 / math.log(2.0)))


def _gelu2(y):
    u = y * (y * y + GK)
    return y * (jnp.tanh(u) + 1.0)


def _kernel(x_hbm, dw_hbm, w1_hbm, w2t_hbm, gam_hbm, bet_hbm, o_hbm,
            hbuf, xb, cbuf, dmat, w1s, acc, w2s, w_ref, dw_ref, gam_ref, bet_ref, pad,
            zs, semx, semp):
    def xcopy(r0, n, d0, sem):
        return pltpu.make_async_copy(x_hbm.at[pl.ds(r0, n)], xb.at[pl.ds(d0, n)], sem)

    def grp_head():
        return xcopy(0, TB - 1, R1 + 1, semx.at[2])

    def grp(i, slot):
        return xcopy(R1 * i + TB - 1, R1, R1 * slot, semx.at[2 * slot])

    def grp_last():
        return xcopy(R1 * (NI - 1) + TB - 1, R1 - TB + 1, R1 * ((NI - 1) % 2), semx.at[2 * ((NI - 1) % 2)])

    def in2(b, slot):
        return xcopy(TB * b, TB, TB * slot, semx.at[slot])

    params = [pltpu.make_async_copy(src, dst, semp.at[j]) for j, (src, dst) in enumerate(
        [(dw_hbm, dw_ref), (w1_hbm, w_ref), (gam_hbm, gam_ref), (bet_hbm, bet_ref), (w2t_hbm, w_ref)])]
    for cp in params[:2] + [grp_head()] + params[2:4] + [grp(0, 0)]:
        cp.start()
    zs[0] = 0
    pad[...] = jnp.zeros_like(pad)

    def w1t(c0=0, n=E):
        return _unp(w1s[c0 // 2:(c0 + n) // 2, :])[:, :C]

    def tap_columns():
        sub = lax.broadcasted_iota(jnp.int32, (C, C), 0)
        lan = lax.broadcasted_iota(jnp.int32, (C, C), 1)
        eye = sub - lan == zs[0]
        diags = [jnp.where(eye, jnp.broadcast_to(dw_ref[i, j:j + 1, :].astype(f32), (C, C)), 0.0)
                 for i in range(3) for j in range(3)]
        ones = jnp.ones((C, 128), bf16)
        return [jnp.dot(d.astype(bf16), ones, preferred_element_type=f32) for d in diags]

    def setup():
        cols = tap_columns()
        c_ = lax.broadcasted_iota(jnp.int32, (8, 128), 0)
        k_ = lax.broadcasted_iota(jnp.int32, (8, 128), 1)
        for g in range(G):
            halves = []
            for o in range(2):
                d = jnp.zeros((8, 128), f32)
                for i in range(3):
                    ri = i + o
                    for j in range(3):
                        for jj in ((0, 3) if j == 0 else (j,)):
                            kpos = (ri // 2) * 64 + jj * 16 + (ri % 2) * 8
                            d = jnp.where(k_ == c_ + kpos, cols[i * 3 + j][8 * g:8 * g + 8], d)
                halves.append(d)
            dmat[8 * g:8 * g + 8, :] = _pack(jnp.concatenate(halves, axis=0))
        w1f = w_ref[...].astype(f32)
        w1c = w1f - jnp.sum(w1f, axis=0, keepdims=True) * (1.0 / C)
        w1c = w1c * (GA * C)
        w1p = jnp.concatenate([w1c, jnp.zeros((128 - C, E), f32)], axis=0)
        w1s[...] = _pack(w1p.T)

    def scope1(sbuf, xns):
        def build(row0, k):
            for g in range(G):
                v = pltpu.bitcast(xb[pl.ds(row0 + 2 * k, 2), g].reshape(16, W), u32)
                base = (k % NQ) * SROWS + g * 24
                sbuf[base:base + 8, :] = jnp.concatenate([pltpu.roll(u, 1, 1) for u in _tiles(v)], axis=1)
                sbuf[base + 8:base + 16, :] = v
                sbuf[base + 16:base + 24, :] = _shift_l(v, False)

        def conv_mm(s0, t, g):
            ts = slice(t * 128, (t + 1) * 128)
            parts = []
            for sl in (s0, s0 + 1):
                bb = (sl % NQ) * SROWS + g * 24
                lft, mid, rgt = (sbuf[bb + 8 * j:bb + 8 * j + 8, ts] for j in range(3))
                seam = jnp.zeros((8, 128), u32)
                if t > 0:
                    lane = lax.broadcasted_iota(jnp.int32, (8, 128), 1)
                    seam = jnp.where(lane > 0, seam, sbuf[bb:bb + 8, (t - 1) * 128:t * 128])
                parts += [_zero_lane(lft, 0), mid, _zero_lane(rgt, 127) if t == NT - 1 else rgt, seam]
            s = _unp(jnp.concatenate(parts, axis=0))
            d = _unp(dmat[8 * g:8 * g + 8, :])
            return jnp.dot(d, s, preferred_element_type=f32)

        def stats(s0, t, cv):
            c0 = [v[0:8] for v in cv]
            c1 = [v[8:16] for v in cv]
            return (s0, t, c0, c1, _var2(c0, c1))

        def norm(st, tie=None, never=None):
            s0, t, c0, c1, var = st
            if tie is not None:
                var = jnp.where(never, tie, var)
            rstd = _rsqrt(var)
            r0 = jnp.broadcast_to(rstd[3:4], (8, 128))
            r1 = jnp.broadcast_to(rstd[7:8], (8, 128))
            ts = slice(t * 128, (t + 1) * 128)
            r = 2 * (s0 % NQ)
            xns[r * CH:(r + 1) * CH, ts] = _pack(jnp.concatenate([c * r0 for c in c0], axis=0))
            xns[(r + 1) * CH:(r + 2) * CH, ts] = _pack(jnp.concatenate([c * r1 for c in c1], axis=0))

        acc[...] = jnp.zeros_like(acc)
        xb[R1] = jnp.zeros((G, 8, W), bf16)
        params[0].wait()
        params[1].wait()
        setup()
        params[4].start()
        grp_head().wait()
        for k in range(NQ):
            build(R1, k)
        for s0 in range(2):
            for t in range(NT):
                st = stats(s0, t, [conv_mm(s0, t, g) for g in range(G)])
                norm(st)
                for o in range(2):
                    if 2 * s0 + o in REC:
                        k = REC.index(2 * s0 + o)
                        cbuf[k * C:(k + 1) * C, t * 128:(t + 1) * 128] = jnp.concatenate(st[2 + o], axis=0)

        def dma1(i, slot):
            @pl.when(i < NI - 1)
            def _():
                grp(i, slot).wait()

            @pl.when(i == NI - 1)
            def _():
                grp_last().wait()
                xb[R1 * ((NI - 1) % 2) + R1 - TB + 1] = jnp.zeros((G, 8, W), bf16)
                for b0 in range(2):
                    in2(b0, (NI % 2) * U1 + b0).start()

            @pl.when(i + 1 < NI - 1)
            def _():
                grp(i + 1, 1 - slot).start()

            @pl.when(i + 1 == NI - 1)
            def _():
                grp_last().start()

        def block1(b, row0, u, never):
            n = E // NCH
            per = NT * G // (2 * NCH)
            for k in range(NQ):
                todo = [(t, g) for t in range(NT) for g in range(G)]
                cv = []
                pend = None
                for j in range(2 * NCH):
                    for _ in range(per):
                        t, g = todo.pop(0)
                        cv.append(conv_mm(k + 2, t, g))
                        if g == G - 1:
                            pend = stats(k + 2, t, cv)
                            cv = []
                    r, c = 2 * k + j // NCH, j % NCH
                    y = jnp.dot(w1t(c * n, n), _unp(xns[r * CH:(r + 1) * CH, :]), preferred_element_type=f32)
                    h = _gelu2(y)
                    h2 = _tiles(h * h)
                    acc[c * n:(c + 1) * n, :] = ((acc[c * n:(c + 1) * n, :] + h2[0]) + h2[1]) + (h2[2] + h2[3])
                    if r in STO:
                        row = pl.multiple_of((b * NSTO + STO.index(r)) * EH + c * (n // 2), 8)
                        hbuf[pl.ds(row, n // 2), :] = _pack(h)
                    if pend is not None:
                        norm(pend, y[TIE:TIE + 8, 0:128], never)
                        pend = None
                build(row0, u * NQ + k)

        def pass1(i, carry):
            slot = i & 1
            dma1(i, slot)
            never = lax.broadcasted_iota(jnp.int32, (8, 128), 0) < zs[0]
            for u in range(U1):
                block1(i * U1 + u, slot * R1, u, never)
            return carry

        lax.fori_loop(0, NI, pass1, 0)

    pl.run_scoped(scope1,
                  pltpu.VMEM((NQ * SROWS, W), u32),
                  pltpu.VMEM((TB * CH, W), u32))

    assert NI % 2 == 0 and NX == 4 and max(REC) < NQ

    def scope2(ob, hre, dwb, semo):
        def out2(b, slot, half):
            return pltpu.make_async_copy(ob.at[pl.ds(TB * slot + NQ * half, NQ)],
                                         o_hbm.at[pl.ds(TB * b + NQ * half, NQ)], semo.at[slot, half])

        def conv_rec(row0, g):
            need = sorted({r + d for r in REC for d in (-1, 0, 1)})
            xs = {q: xb[row0 + q, g].astype(f32) for q in need}
            wt = [jnp.concatenate([dwb[tap, 8 * g:8 * g + 8, :]] * NT, axis=1) for tap in range(9)]
            for k, r in enumerate(REC):
                a = []
                for j in range(3):
                    t = xs[r - 1] * wt[j]
                    t = t + xs[r] * wt[3 + j]
                    t = t + xs[r + 1] * wt[6 + j]
                    a.append(t)
                cbuf[k * C + 8 * g:k * C + 8 * g + 8, :] = _shift_r(a[0]) + a[1] + _shift_l(a[2])

        def ln_rec(k):
            cols = []
            for t in range(NT):
                c = [cbuf[k * C + 8 * g:k * C + 8 * g + 8, t * 128:(t + 1) * 128] for g in range(G)]
                r = jnp.broadcast_to(lax.rsqrt(_var1(c))[7:8], (8, 128))
                cols.append(jnp.concatenate([v * r for v in c], axis=0))
            return jnp.concatenate(cols, axis=1).astype(bf16)

        in2(2, 2).start()
        for cp in params[2:]:
            cp.wait()
        for tap, col in enumerate(tap_columns()):
            dwb[tap] = col
        ssq = jnp.sum(acc[...].T, axis=0, keepdims=True) * (1.0 / (4.0 * GA * GA))
        gx = jnp.sqrt(ssq + 1e-6)
        nx = gx / (jnp.sum(gx, axis=1, keepdims=True) * (1.0 / E) + 1e-6)
        gam = gam_ref[...].astype(f32).reshape(1, E)
        bet = bet_ref[...].astype(f32).reshape(1, E)
        scale = (gam * nx + 1.0) * (1.0 / (2.0 * GA))
        w2f = w_ref[...].astype(f32)
        w2s[...] = _pack(w2f * scale)
        dwb[9] = jnp.broadcast_to(jnp.sum(w2f * bet, axis=1, keepdims=True), (C, 128))
        in2(0, 0).wait()

        def pass2(b, carry):
            row0 = (b & 3) * TB
            nrow0 = ((b + 1) & 3) * TB
            oslot = b & 1

            @pl.when(b + 3 < NB)
            def _():
                in2(b + 3, (b + 3) & 3).start()

            @pl.when(b >= 2)
            def _():
                for hf in range(2):
                    out2(b - 2, oslot, hf).wait()

            @pl.when(b + 1 < NB)
            def _():
                in2(b + 1, (b + 1) & 3).wait()

            pending = list(range(G))
            plan = list(PLAN)

            def finish(r, hp, ngroups):
                o = jnp.dot(_unp(w2s[...]), _unp(hp), preferred_element_type=f32)
                for hf in range(2):
                    ls = slice(hf * 256, hf * 256 + 256)
                    for j in range((ngroups + 1 - hf) // 2):
                        t = 2 * hf + j
                        mark = o[0:8, t * 128:(t + 1) * 128]
                        xb[row0 + STO[0], zs[0]] = jnp.concatenate([mark] * NT, axis=1).astype(bf16)
                        conv_rec(nrow0, pending.pop(0))
                    for g in range(G):
                        xr = xb[row0 + r, g, :, ls].astype(f32)
                        bg = dwb[9, 8 * g:8 * g + 8, :]
                        v = o[8 * g:8 * g + 8, ls] + (xr + jnp.concatenate([bg, bg], axis=1))
                        ob[oslot * TB + r, g, :, ls] = v.astype(bf16)

            def sto(k, ngroups):
                finish(STO[k], hbuf[pl.ds(pl.multiple_of((b * NSTO + k) * EH, 8), EH), :], ngroups)

            sto(0, 0)
            for k in range(NREC):
                y = jnp.dot(w1t(), ln_rec(k), preferred_element_type=f32)
                hre[k * EH:(k + 1) * EH, :] = _pack(_gelu2(y))
            for k in range(1, NSTO):
                sto(k, plan.pop(0))
            out2(b, oslot, 1).start()
            for k in range(NREC):
                finish(REC[k], hre[pl.ds(pl.multiple_of(zs[0] + k * EH, 8), EH), :], plan.pop(0))
            out2(b, oslot, 0).start()
            return carry

        lax.fori_loop(0, NB, pass2, 0)
        for hf in range(2):
            out2(NB - 2, 0, hf).wait()
            out2(NB - 1, 1, hf).wait()

    pl.run_scoped(scope2,
                  pltpu.VMEM((2 * TB, G, 8, W), bf16),
                  pltpu.VMEM((NREC * EH, W), u32),
                  pltpu.VMEM((10, C, 128), f32),
                  pltpu.SemaphoreType.DMA((2, 2)))


@jax.jit
def pallas_standalone__modern_conv_block_convnext_v2__vision_kernel(
    x: jax.Array,
    dw: jax.Array,
    w1: jax.Array,
    w2: jax.Array,
    grn_gamma: jax.Array,
    grn_beta: jax.Array,
):
    xt = jnp.transpose(x, (0, 1, 3, 2)).reshape(H, G, 8, W)
    hbm = pl.BlockSpec(memory_space=pl.ANY)
    o = pl.pallas_call(
        _kernel,
        out_shape=jax.ShapeDtypeStruct((H, G, 8, W), bf16),
        in_specs=[hbm] * 6,
        out_specs=hbm,
        scratch_shapes=[
            pltpu.VMEM((NB * NSTO * EH, W), u32),
            pltpu.VMEM((NX * TB, G, 8, W), bf16),
            pltpu.VMEM((NREC * C, W), f32),
            pltpu.VMEM((C, 128), u32),
            pltpu.VMEM((EH, 128), u32),
            pltpu.VMEM((E, 128), f32),
            pltpu.VMEM((CH, E), u32),
            pltpu.VMEM((C, E), bf16),
            pltpu.VMEM((3, 3, C), bf16),
            pltpu.VMEM((E,), bf16),
            pltpu.VMEM((E,), bf16),
            pltpu.VMEM((PADV, 3, C), bf16),
            pltpu.SMEM((1,), jnp.int32),
            pltpu.SemaphoreType.DMA((NX,)),
            pltpu.SemaphoreType.DMA((5,)),
        ],
        compiler_params=pltpu.CompilerParams(vmem_limit_bytes=128 * 1024 * 1024,
                                             disable_bounds_checks=True),
        name="convnext",
    )(xt, dw, w1, w2.T, grn_gamma, grn_beta)
    return jnp.transpose(o.reshape(1, H, C, W), (0, 1, 3, 2))
```

```python
import math

import jax
import jax.numpy as jnp
from jax import lax
from jax.experimental import pallas as pl
from jax.experimental.pallas import tpu as pltpu

H = 512
W = 512
C = 96
E = 384
G = C // 8
NT = W // 128
TB = 8
NB = H // TB
NQ = TB // 2
REC = (1, 2, 3)
STO = tuple(r for r in range(TB) if r not in REC)
NSTO = len(STO)
NREC = len(REC)
EH = E // 2
CH = C // 2
SROWS = G * 24
NCH = 3
U1 = 2
R1 = TB * U1
NI = NB // U1
NX = 2 * U1
TIE = 40
PLAN = (2, 2, 2, 2, 2, 2, 0)
PADV = 7

C0 = math.sqrt(2.0 / math.pi)
C1 = 0.044715
GA = (C0 * C1) ** (1.0 / 3.0)
GK = C0 / GA
LN_EPS = 1e-5

f32 = jnp.float32
bf16 = jnp.bfloat16
u32 = jnp.uint32


def _pack(v):
    return pltpu.bitcast(v.astype(bf16), u32)


def _unp(v):
    return pltpu.bitcast(v, bf16)


def _tiles(a):
    return [a[:, t * 128:(t + 1) * 128] for t in range(NT)]


def _zero_lane(a, l):
    lane = lax.broadcasted_iota(jnp.int32, a.shape, 1)
    return jnp.where(lane == l, jnp.zeros_like(a), a)


def _shift_r(a):
    v = _tiles(a)
    m = [_zero_lane(v[0], 127)] + [jnp.concatenate([v[t][:, :127], v[t - 1][:, 127:]], axis=1)
                                   for t in range(1, NT)]
    return jnp.concatenate([pltpu.roll(u, 1, 1) for u in m], axis=1)


def _shift_l(a, edge=True):
    v = _tiles(a)
    m = ([jnp.concatenate([v[t + 1][:, :1], v[t][:, 1:]], axis=1) for t in range(NT - 1)]
         + [_zero_lane(v[NT - 1], 0) if edge else v[NT - 1]])
    return jnp.concatenate([pltpu.roll(u, 127, 1) for u in m], axis=1)


def _sums(c):
    s1 = c[0]
    s2 = c[0] * c[0]
    for g in range(1, G):
        s1 = s1 + c[g]
        s2 = s2 + c[g] * c[g]
    return s1, s2


def _merge4(a, b):
    p = jnp.concatenate([a[:4], b[4:]], axis=0)
    q = jnp.concatenate([b[:4], a[4:]], axis=0)
    return p + pltpu.roll(q, 4, 0)


def _var_from(n, shift):
    eps = LN_EPS * C * C
    return jnp.maximum(n * float(C) + eps - pltpu.roll(n * n, shift, 0), eps)


def _var2(c0, c1):
    a1, a2 = _sums(c0)
    b1, b2 = _sums(c1)
    m1 = _merge4(a1, b1)
    m2 = _merge4(a2, b2)
    sub = lax.broadcasted_iota(jnp.int32, (8, 128), 0)
    n = jnp.where((sub & 2) == 0, m1 + pltpu.roll(m1, 6, 0), m2 + pltpu.roll(m2, 2, 0))
    n = n + pltpu.roll(n, 1, 0)
    return _var_from(n, 2)


def _var1(c):
    s1, s2 = _sums(c)
    n = _merge4(s1, s2)
    n = n + pltpu.roll(n, 2, 0)
    n = n + pltpu.roll(n, 1, 0)
    return _var_from(n, 4)


def _rsqrt(v):
    return jnp.exp2(jnp.log(v) * (-0.5 / math.log(2.0)))


def _gelu2(y):
    u = y * (y * y + GK)
    return y * (jnp.tanh(u) + 1.0)


def _kernel(x_hbm, dw_hbm, w1_hbm, w2t_hbm, gam_hbm, bet_hbm, o_hbm,
            hbuf, xb, cbuf, dmat, w1s, acc, w2s, w_ref, dw_ref, gam_ref, bet_ref, pad,
            zs, semx, semp):
    def xcopy(r0, n, d0, sem):
        return pltpu.make_async_copy(x_hbm.at[pl.ds(r0, n)], xb.at[pl.ds(d0, n)], sem)

    def grp_head():
        return xcopy(0, TB - 1, R1 + 1, semx.at[2])

    def grp(i, slot):
        return xcopy(R1 * i + TB - 1, R1, R1 * slot, semx.at[2 * slot])

    def grp_last():
        return xcopy(R1 * (NI - 1) + TB - 1, R1 - TB + 1, R1 * ((NI - 1) % 2), semx.at[2 * ((NI - 1) % 2)])

    def in2(b, slot):
        return xcopy(TB * b, TB, TB * slot, semx.at[slot])

    params = [pltpu.make_async_copy(src, dst, semp.at[j]) for j, (src, dst) in enumerate(
        [(dw_hbm, dw_ref), (w1_hbm, w_ref), (gam_hbm, gam_ref), (bet_hbm, bet_ref), (w2t_hbm, w_ref)])]
    for cp in params[:2] + [grp_head()] + params[2:4] + [grp(0, 0)]:
        cp.start()
    zs[0] = 0
    pad[...] = jnp.zeros_like(pad)

    def w1t(c0=0, n=E):
        return _unp(w1s[c0 // 2:(c0 + n) // 2, :])[:, :C]

    def tap_columns():
        sub = lax.broadcasted_iota(jnp.int32, (C, C), 0)
        lan = lax.broadcasted_iota(jnp.int32, (C, C), 1)
        eye = sub - lan == zs[0]
        diags = [jnp.where(eye, jnp.broadcast_to(dw_ref[i, j:j + 1, :].astype(f32), (C, C)), 0.0)
                 for i in range(3) for j in range(3)]
        ones = jnp.ones((C, 128), bf16)
        return [jnp.dot(d.astype(bf16), ones, preferred_element_type=f32) for d in diags]

    def setup():
        cols = tap_columns()
        c_ = lax.broadcasted_iota(jnp.int32, (8, 128), 0)
        k_ = lax.broadcasted_iota(jnp.int32, (8, 128), 1)
        for g in range(G):
            halves = []
            for o in range(2):
                d = jnp.zeros((8, 128), f32)
                for i in range(3):
                    ri = i + o
                    for j in range(3):
                        for jj in ((0, 3) if j == 0 else (j,)):
                            kpos = (ri // 2) * 64 + jj * 16 + (ri % 2) * 8
                            d = jnp.where(k_ == c_ + kpos, cols[i * 3 + j][8 * g:8 * g + 8], d)
                halves.append(d)
            dmat[8 * g:8 * g + 8, :] = _pack(jnp.concatenate(halves, axis=0))
        w1f = w_ref[...].astype(f32)
        w1c = w1f - jnp.sum(w1f, axis=0, keepdims=True) * (1.0 / C)
        w1c = w1c * (GA * C)
        w1p = jnp.concatenate([w1c, jnp.zeros((128 - C, E), f32)], axis=0)
        w1s[...] = _pack(w1p.T)

    def scope1(sbuf, xns):
        def build(row0, k):
            for g in range(G):
                v = pltpu.bitcast(xb[pl.ds(row0 + 2 * k, 2), g].reshape(16, W), u32)
                base = (k % NQ) * SROWS + g * 24
                sbuf[base:base + 8, :] = jnp.concatenate([pltpu.roll(u, 1, 1) for u in _tiles(v)], axis=1)
                sbuf[base + 8:base + 16, :] = v
                sbuf[base + 16:base + 24, :] = _shift_l(v, False)

        def conv_mm(s0, t, g):
            ts = slice(t * 128, (t + 1) * 128)
            parts = []
            for sl in (s0, s0 + 1):
                bb = (sl % NQ) * SROWS + g * 24
                lft, mid, rgt = (sbuf[bb + 8 * j:bb + 8 * j + 8, ts] for j in range(3))
                seam = jnp.zeros((8, 128), u32)
                if t > 0:
                    lane = lax.broadcasted_iota(jnp.int32, (8, 128), 1)
                    seam = jnp.where(lane > 0, seam, sbuf[bb:bb + 8, (t - 1) * 128:t * 128])
                parts += [_zero_lane(lft, 0), mid, _zero_lane(rgt, 127) if t == NT - 1 else rgt, seam]
            s = _unp(jnp.concatenate(parts, axis=0))
            d = _unp(dmat[8 * g:8 * g + 8, :])
            return jnp.dot(d, s, preferred_element_type=f32)

        def stats(s0, t, cv):
            c0 = [v[0:8] for v in cv]
            c1 = [v[8:16] for v in cv]
            return (s0, t, c0, c1, _var2(c0, c1))

        def norm(st, tie=None, never=None):
            s0, t, c0, c1, var = st
            if tie is not None:
                var = jnp.where(never, tie, var)
            rstd = _rsqrt(var)
            r0 = jnp.broadcast_to(rstd[3:4], (8, 128))
            r1 = jnp.broadcast_to(rstd[7:8], (8, 128))
            ts = slice(t * 128, (t + 1) * 128)
            r = 2 * (s0 % NQ)
            xns[r * CH:(r + 1) * CH, ts] = _pack(jnp.concatenate([c * r0 for c in c0], axis=0))
            xns[(r + 1) * CH:(r + 2) * CH, ts] = _pack(jnp.concatenate([c * r1 for c in c1], axis=0))

        acc[...] = jnp.zeros_like(acc)
        xb[R1] = jnp.zeros((G, 8, W), bf16)
        params[0].wait()
        params[1].wait()
        setup()
        params[4].start()
        grp_head().wait()
        for k in range(NQ):
            build(R1, k)
        for s0 in range(2):
            for t in range(NT):
                st = stats(s0, t, [conv_mm(s0, t, g) for g in range(G)])
                norm(st)
                for o in range(2):
                    if 2 * s0 + o in REC:
                        k = REC.index(2 * s0 + o)
                        cbuf[k * C:(k + 1) * C, t * 128:(t + 1) * 128] = jnp.concatenate(st[2 + o], axis=0)

        def dma1(i, slot):
            @pl.when(i < NI - 1)
            def _():
                grp(i, slot).wait()

            @pl.when(i == NI - 1)
            def _():
                grp_last().wait()
                xb[R1 * ((NI - 1) % 2) + R1 - TB + 1] = jnp.zeros((G, 8, W), bf16)
                for b0 in range(2):
                    in2(b0, (NI % 2) * U1 + b0).start()

            @pl.when(i + 1 < NI - 1)
            def _():
                grp(i + 1, 1 - slot).start()

            @pl.when(i + 1 == NI - 1)
            def _():
                grp_last().start()

        def block1(b, row0, u, never):
            n = E // NCH
            per = NT * G // (2 * NCH)
            for k in range(NQ):
                todo = [(t, g) for t in range(NT) for g in range(G)]
                cv = []
                pend = None
                for j in range(2 * NCH):
                    for _ in range(per):
                        t, g = todo.pop(0)
                        cv.append(conv_mm(k + 2, t, g))
                        if g == G - 1:
                            pend = stats(k + 2, t, cv)
                            cv = []
                    r, c = 2 * k + j // NCH, j % NCH
                    y = jnp.dot(w1t(c * n, n), _unp(xns[r * CH:(r + 1) * CH, :]), preferred_element_type=f32)
                    h = _gelu2(y)
                    h2 = _tiles(h * h)
                    acc[c * n:(c + 1) * n, :] = ((acc[c * n:(c + 1) * n, :] + h2[0]) + h2[1]) + (h2[2] + h2[3])
                    if r in STO:
                        row = pl.multiple_of((b * NSTO + STO.index(r)) * EH + c * (n // 2), 8)
                        hbuf[pl.ds(row, n // 2), :] = _pack(h)
                    if pend is not None:
                        norm(pend, y[TIE:TIE + 8, 0:128], never)
                        pend = None
                build(row0, u * NQ + k)

        def pass1(i, carry):
            slot = i & 1
            dma1(i, slot)
            never = lax.broadcasted_iota(jnp.int32, (8, 128), 0) < zs[0]
            for u in range(U1):
                block1(i * U1 + u, slot * R1, u, never)
            return carry

        lax.fori_loop(0, NI, pass1, 0)

    pl.run_scoped(scope1,
                  pltpu.VMEM((NQ * SROWS, W), u32),
                  pltpu.VMEM((TB * CH, W), u32))

    assert NI % 2 == 0 and NX == 4 and max(REC) < NQ

    def scope2(ob, hre, dwb, semo):
        def out2(b, slot, half):
            return pltpu.make_async_copy(ob.at[pl.ds(TB * slot + NQ * half, NQ)],
                                         o_hbm.at[pl.ds(TB * b + NQ * half, NQ)], semo.at[slot])

        def out2_wait(b, slot):
            pltpu.make_async_copy(ob.at[pl.ds(TB * slot, TB)], o_hbm.at[pl.ds(TB * b, TB)], semo.at[slot]).wait()

        def conv_rec(row0, g):
            need = sorted({r + d for r in REC for d in (-1, 0, 1)})
            xs = {q: xb[row0 + q, g].astype(f32) for q in need}
            wt = [jnp.concatenate([dwb[tap, 8 * g:8 * g + 8, :]] * NT, axis=1) for tap in range(9)]
            for k, r in enumerate(REC):
                a = []
                for j in range(3):
                    t = xs[r - 1] * wt[j]
                    t = t + xs[r] * wt[3 + j]
                    t = t + xs[r + 1] * wt[6 + j]
                    a.append(t)
                cbuf[k * C + 8 * g:k * C + 8 * g + 8, :] = _shift_r(a[0]) + a[1] + _shift_l(a[2])

        def ln_rec(k):
            cols = []
            for t in range(NT):
                c = [cbuf[k * C + 8 * g:k * C + 8 * g + 8, t * 128:(t + 1) * 128] for g in range(G)]
                r = jnp.broadcast_to(lax.rsqrt(_var1(c))[7:8], (8, 128))
                cols.append(jnp.concatenate([v * r for v in c], axis=0))
            return jnp.concatenate(cols, axis=1).astype(bf16)

        in2(2, 2).start()
        for cp in params[2:]:
            cp.wait()
        for tap, col in enumerate(tap_columns()):
            dwb[tap] = col
        ssq = jnp.sum(acc[...].T, axis=0, keepdims=True) * (1.0 / (4.0 * GA * GA))
        gx = jnp.sqrt(ssq + 1e-6)
        nx = gx / (jnp.sum(gx, axis=1, keepdims=True) * (1.0 / E) + 1e-6)
        gam = gam_ref[...].astype(f32).reshape(1, E)
        bet = bet_ref[...].astype(f32).reshape(1, E)
        scale = (gam * nx + 1.0) * (1.0 / (2.0 * GA))
        w2f = w_ref[...].astype(f32)
        w2s[...] = _pack(w2f * scale)
        dwb[9] = jnp.broadcast_to(jnp.sum(w2f * bet, axis=1, keepdims=True), (C, 128))
        in2(0, 0).wait()

        def pass2(b, hrow):
            row0 = (b & 3) * TB
            nrow0 = ((b + 1) & 3) * TB
            oslot = b & 1

            @pl.when(b >= 2)
            def _():
                out2_wait(b - 2, oslot)

            @pl.when(b + 1 < NB)
            def _():
                in2(b + 1, (b + 1) & 3).wait()

            pending = list(range(G))
            plan = list(PLAN)

            def finish(r, hp, ngroups):
                o = jnp.dot(_unp(w2s[...]), _unp(hp), preferred_element_type=f32)
                for hf in range(2):
                    ls = slice(hf * 256, hf * 256 + 256)
                    for j in range((ngroups + 1 - hf) // 2):
                        t = 2 * hf + j
                        mark = o[0:8, t * 128:(t + 1) * 128]
                        xb[row0 + STO[0], zs[0]] = jnp.concatenate([mark] * NT, axis=1).astype(bf16)
                        conv_rec(nrow0, pending.pop(0))
                    for g in range(G):
                        xr = xb[row0 + r, g, :, ls].astype(f32)
                        bg = dwb[9, 8 * g:8 * g + 8, :]
                        v = o[8 * g:8 * g + 8, ls] + (xr + jnp.concatenate([bg, bg], axis=1))
                        ob[oslot * TB + r, g, :, ls] = v.astype(bf16)

            def sto(k, ngroups):
                finish(STO[k], hbuf[pl.ds(pl.multiple_of(hrow + k * EH, 8), EH), :], ngroups)

            sto(0, 0)

            @pl.when(b + 3 < NB)
            def _():
                in2(b + 3, (b + 3) & 3).start()

            for k in range(NREC):
                y = jnp.dot(w1t(), ln_rec(k), preferred_element_type=f32)
                hre[k * EH:(k + 1) * EH, :] = _pack(_gelu2(y))
            for k in range(1, NSTO):
                sto(k, plan.pop(0))
            out2(b, oslot, 1).start()
            for k in range(NREC):
                finish(REC[k], hre[pl.ds(pl.multiple_of(zs[0] + k * EH, 8), EH), :], plan.pop(0))
            out2(b, oslot, 0).start()
            return hrow + NSTO * EH

        lax.fori_loop(0, NB, pass2, jnp.int32(0))
        out2_wait(NB - 2, 0)
        out2_wait(NB - 1, 1)

    pl.run_scoped(scope2,
                  pltpu.VMEM((2 * TB, G, 8, W), bf16),
                  pltpu.VMEM((NREC * EH, W), u32),
                  pltpu.VMEM((10, C, 128), f32),
                  pltpu.SemaphoreType.DMA((2,)))


@jax.jit
def pallas_standalone__modern_conv_block_convnext_v2__vision_kernel(
    x: jax.Array,
    dw: jax.Array,
    w1: jax.Array,
    w2: jax.Array,
    grn_gamma: jax.Array,
    grn_beta: jax.Array,
):
    xt = jnp.transpose(x, (0, 1, 3, 2)).reshape(H, G, 8, W)
    hbm = pl.BlockSpec(memory_space=pl.ANY)
    o = pl.pallas_call(
        _kernel,
        out_shape=jax.ShapeDtypeStruct((H, G, 8, W), bf16),
        in_specs=[hbm] * 6,
        out_specs=hbm,
        scratch_shapes=[
            pltpu.VMEM((NB * NSTO * EH, W), u32),
            pltpu.VMEM((NX * TB, G, 8, W), bf16),
            pltpu.VMEM((NREC * C, W), f32),
            pltpu.VMEM((C, 128), u32),
            pltpu.VMEM((EH, 128), u32),
            pltpu.VMEM((E, 128), f32),
            pltpu.VMEM((CH, E), u32),
            pltpu.VMEM((C, E), bf16),
            pltpu.VMEM((3, 3, C), bf16),
            pltpu.VMEM((E,), bf16),
            pltpu.VMEM((E,), bf16),
            pltpu.VMEM((PADV, 3, C), bf16),
            pltpu.SMEM((1,), jnp.int32),
            pltpu.SemaphoreType.DMA((NX,)),
            pltpu.SemaphoreType.DMA((5,)),
        ],
        compiler_params=pltpu.CompilerParams(vmem_limit_bytes=128 * 1024 * 1024,
                                             disable_bounds_checks=True),
        name="convnext",
    )(xt, dw, w1, w2.T, grn_gamma, grn_beta)
    return jnp.transpose(o.reshape(1, H, C, W), (0, 1, 3, 2))
```

```python
import math

import jax
import jax.numpy as jnp
from jax import lax
from jax.experimental import pallas as pl
from jax.experimental.pallas import tpu as pltpu

H = 512
W = 512
C = 96
E = 384
G = C // 8
NT = W // 128
TB = 8
NB = H // TB
NQ = TB // 2
REC = (1, 2, 3)
STO = tuple(r for r in range(TB) if r not in REC)
NSTO = len(STO)
NREC = len(REC)
EH = E // 2
CH = C // 2
GB = 4
SROWS = G * 24
NCH = 3
U1 = 2
R1 = TB * U1
NI = NB // U1
NX = 2 * U1
TIE = 40
PLAN = (2, 2, 2, 2, 2, 2, 0)
PADV = 7

C0 = math.sqrt(2.0 / math.pi)
C1 = 0.044715
GA = (C0 * C1) ** (1.0 / 3.0)
GK = C0 / GA
LN_EPS = 1e-5

f32 = jnp.float32
bf16 = jnp.bfloat16
u32 = jnp.uint32


def _pack(v):
    return pltpu.bitcast(v.astype(bf16), u32)


def _unp(v):
    return pltpu.bitcast(v, bf16)


def _tiles(a):
    return [a[:, t * 128:(t + 1) * 128] for t in range(NT)]


def _zero_lane(a, l):
    lane = lax.broadcasted_iota(jnp.int32, a.shape, 1)
    return jnp.where(lane == l, jnp.zeros_like(a), a)


def _shift_r(a):
    v = _tiles(a)
    m = [_zero_lane(v[0], 127)] + [jnp.concatenate([v[t][:, :127], v[t - 1][:, 127:]], axis=1)
                                   for t in range(1, NT)]
    return jnp.concatenate([pltpu.roll(u, 1, 1) for u in m], axis=1)


def _shift_l(a, edge=True):
    v = _tiles(a)
    m = ([jnp.concatenate([v[t + 1][:, :1], v[t][:, 1:]], axis=1) for t in range(NT - 1)]
         + [_zero_lane(v[NT - 1], 0) if edge else v[NT - 1]])
    return jnp.concatenate([pltpu.roll(u, 127, 1) for u in m], axis=1)


def _sums(c):
    return jnp.sum(c, axis=0), jnp.sum(c * c, axis=0)


def _merge4(a, b):
    p = jnp.concatenate([a[:4], b[4:]], axis=0)
    q = jnp.concatenate([b[:4], a[4:]], axis=0)
    return p + pltpu.roll(q, 4, 0)


def _var_from(n, shift):
    eps = LN_EPS * C * C
    return jnp.maximum(n * float(C) + eps - pltpu.roll(n * n, shift, 0), eps)


def _var2(c):
    s1, s2 = _sums(c)
    m1 = _merge4(s1[:8], s1[8:])
    m2 = _merge4(s2[:8], s2[8:])
    sub = lax.broadcasted_iota(jnp.int32, (8, 128), 0)
    n = jnp.where((sub & 2) == 0, m1 + pltpu.roll(m1, 6, 0), m2 + pltpu.roll(m2, 2, 0))
    n = n + pltpu.roll(n, 1, 0)
    return _var_from(n, 2)


def _var1(c):
    s1, s2 = _sums(c)
    n = _merge4(s1, s2)
    n = n + pltpu.roll(n, 2, 0)
    n = n + pltpu.roll(n, 1, 0)
    return _var_from(n, 4)


def _rsqrt(v):
    return jnp.exp2(jnp.log(v) * (-0.5 / math.log(2.0)))


def _gelu2(y):
    u = y * (y * y + GK)
    return y * (jnp.tanh(u) + 1.0)


def _kernel(x_hbm, dw_hbm, w1_hbm, w2t_hbm, gam_hbm, bet_hbm, o_hbm,
            hbuf, xb, cbuf, dmat, w1s, acc, w2s, w_ref, dw_ref, gam_ref, bet_ref, pad,
            zs, semx, semp):
    def xcopy(r0, n, d0, sem):
        return pltpu.make_async_copy(x_hbm.at[pl.ds(r0, n)], xb.at[pl.ds(d0, n)], sem)

    def grp_head():
        return xcopy(0, TB - 1, R1 + 1, semx.at[2])

    def grp(i, slot):
        return xcopy(R1 * i + TB - 1, R1, R1 * slot, semx.at[2 * slot])

    def grp_last():
        return xcopy(R1 * (NI - 1) + TB - 1, R1 - TB + 1, R1 * ((NI - 1) % 2), semx.at[2 * ((NI - 1) % 2)])

    def in2(b, slot):
        return xcopy(TB * b, TB, TB * slot, semx.at[slot])

    params = [pltpu.make_async_copy(src, dst, semp.at[j]) for j, (src, dst) in enumerate(
        [(dw_hbm, dw_ref), (w1_hbm, w_ref), (gam_hbm, gam_ref), (bet_hbm, bet_ref), (w2t_hbm, w_ref)])]
    for cp in params[:2] + [grp_head()] + params[2:4] + [grp(0, 0)]:
        cp.start()
    zs[0] = 0
    pad[...] = jnp.zeros_like(pad)

    def w1t(c0=0, n=E):
        return _unp(w1s[c0 // 2:(c0 + n) // 2, :])[:, :C]

    def tap_columns():
        sub = lax.broadcasted_iota(jnp.int32, (C, C), 0)
        lan = lax.broadcasted_iota(jnp.int32, (C, C), 1)
        eye = sub - lan == zs[0]
        diags = [jnp.where(eye, jnp.broadcast_to(dw_ref[i, j:j + 1, :].astype(f32), (C, C)), 0.0)
                 for i in range(3) for j in range(3)]
        ones = jnp.ones((C, 128), bf16)
        return [jnp.dot(d.astype(bf16), ones, preferred_element_type=f32) for d in diags]

    def setup():
        cols = tap_columns()
        c_ = lax.broadcasted_iota(jnp.int32, (8, 128), 0)
        k_ = lax.broadcasted_iota(jnp.int32, (8, 128), 1)
        for g in range(G):
            halves = []
            for o in range(2):
                d = jnp.zeros((8, 128), f32)
                for i in range(3):
                    ri = i + o
                    for j in range(3):
                        for jj in ((0, 3) if j == 0 else (j,)):
                            kpos = (ri // 2) * 64 + jj * 16 + (ri % 2) * 8
                            d = jnp.where(k_ == c_ + kpos, cols[i * 3 + j][8 * g:8 * g + 8], d)
                halves.append(d)
            dmat[8 * g:8 * g + 8, :] = _pack(jnp.concatenate(halves, axis=0))
        w1f = w_ref[...].astype(f32)
        w1c = w1f - jnp.sum(w1f, axis=0, keepdims=True) * (1.0 / C)
        w1c = w1c * (GA * C)
        w1p = jnp.concatenate([w1c, jnp.zeros((128 - C, E), f32)], axis=0)
        w1s[...] = _pack(w1p.T)

    def scope1(sbuf, xns):
        def build(row0, k):
            for g0 in range(0, G, GB):
                v = xb[pl.ds(row0 + 2 * k, 2), g0:g0 + GB]
                v = pltpu.bitcast(jnp.swapaxes(v, 0, 1).reshape(GB * 16, W), u32)
                lft = jnp.concatenate([pltpu.roll(u, 1, 1) for u in _tiles(v)], axis=1)
                parts = [a.reshape(GB, 8, W) for a in (lft, v, _shift_l(v, False))]
                base = (k % NQ) * SROWS + g0 * 24
                sbuf[base:base + GB * 24, :] = jnp.concatenate(parts, axis=1).reshape(GB * 24, W)

        def lane_masks():
            lane = lax.broadcasted_iota(jnp.int32, (GB, 8, 128), 2)
            return lane == 0, lane > 0, lane == 127, jnp.zeros((GB, 8, 128), u32)

        def conv_mm(s0, t, g0, masks):
            first, rest, last, zero = masks
            parts = []
            for sl in (s0, s0 + 1):
                r0 = (sl % NQ) * SROWS + g0 * 24
                v = sbuf[r0:r0 + GB * 24, t * 128:(t + 1) * 128].reshape(GB, 24, 128)
                seam = zero
                if t > 0:
                    prev = sbuf[r0:r0 + GB * 24, (t - 1) * 128:t * 128].reshape(GB, 24, 128)
                    seam = lax.select(rest, zero, prev[:, 0:8])
                parts += [lax.select(first, zero, v[:, 0:8]), v[:, 8:16],
                          lax.select(last, zero, v[:, 16:24]) if t == NT - 1 else v[:, 16:24], seam]
            s = _unp(jnp.concatenate(parts, axis=1).reshape(GB * 64, 128))
            d = _unp(dmat[8 * g0:8 * (g0 + GB), :])
            return [jnp.dot(d[16 * g:16 * g + 16], s[128 * g:128 * g + 128], preferred_element_type=f32)
                    for g in range(GB)]

        def stats(s0, t, cv):
            c = jnp.concatenate(cv, axis=0).reshape(G, 16, 128)
            return (s0, t, c[:, :8].reshape(C, 128), c[:, 8:].reshape(C, 128), _var2(c))

        def norm(st, tie=None, never=None):
            s0, t, c0, c1, var = st
            if tie is not None:
                var = lax.select(never, tie, var)
            rstd = _rsqrt(var)
            r0 = rstd[3:4]
            r1 = rstd[7:8]
            ts = slice(t * 128, (t + 1) * 128)
            r = 2 * (s0 % NQ)
            xns[r * CH:(r + 1) * CH, ts] = _pack(c0 * r0)
            xns[(r + 1) * CH:(r + 2) * CH, ts] = _pack(c1 * r1)

        acc[...] = jnp.zeros_like(acc)
        xb[R1] = jnp.zeros((G, 8, W), bf16)
        params[0].wait()
        params[1].wait()
        setup()
        params[4].start()
        grp_head().wait()
        for k in range(NQ):
            build(R1, k)
        masks = lane_masks()
        for s0 in range(2):
            for t in range(NT):
                st = stats(s0, t, sum([conv_mm(s0, t, g, masks) for g in range(0, G, GB)], []))
                norm(st)
                for o in range(2):
                    if 2 * s0 + o in REC:
                        k = REC.index(2 * s0 + o)
                        for g in range(G):
                            q = 8 * (NREC * g + k)
                            cbuf[q:q + 8, t * 128:(t + 1) * 128] = st[2 + o][8 * g:8 * g + 8]

        def dma1(i, slot):
            @pl.when(i < NI - 1)
            def _():
                grp(i, slot).wait()

            @pl.when(i == NI - 1)
            def _():
                grp_last().wait()
                xb[R1 * ((NI - 1) % 2) + R1 - TB + 1] = jnp.zeros((G, 8, W), bf16)
                for b0 in range(2):
                    in2(b0, (NI % 2) * U1 + b0).start()

            @pl.when(i + 1 < NI - 1)
            def _():
                grp(i + 1, 1 - slot).start()

            @pl.when(i + 1 == NI - 1)
            def _():
                grp_last().start()

        def block1(b, row0, u, never, masks):
            n = E // NCH
            per = NT * G // (2 * NCH * GB)
            for k in range(NQ):
                todo = [(t, g) for t in range(NT) for g in range(0, G, GB)]
                cv = []
                pend = None
                for j in range(2 * NCH):
                    for _ in range(per):
                        t, g = todo.pop(0)
                        cv += conv_mm(k + 2, t, g, masks)
                        if g == G - GB:
                            pend = stats(k + 2, t, cv)
                            cv = []
                    r, c = 2 * k + j // NCH, j % NCH
                    y = jnp.dot(w1t(c * n, n), _unp(xns[r * CH:(r + 1) * CH, :]), preferred_element_type=f32)
                    h = _gelu2(y)
                    h2 = _tiles(h * h)
                    acc[c * n:(c + 1) * n, :] = ((acc[c * n:(c + 1) * n, :] + h2[0]) + h2[1]) + (h2[2] + h2[3])
                    if r in STO:
                        row = pl.multiple_of((b * NSTO + STO.index(r)) * EH + c * (n // 2), 8)
                        hbuf[pl.ds(row, n // 2), :] = _pack(h)
                    if pend is not None:
                        norm(pend, y[TIE:TIE + 8, 0:128], never)
                        pend = None
                build(row0, u * NQ + k)

        def pass1(i, carry):
            slot = i & 1
            dma1(i, slot)
            never = lax.broadcasted_iota(jnp.int32, (8, 128), 0) < zs[0]
            masks = lane_masks()
            for u in range(U1):
                block1(i * U1 + u, slot * R1, u, never, masks)
            return carry

        lax.fori_loop(0, NI, pass1, 0)

    pl.run_scoped(scope1,
                  pltpu.VMEM((NQ * SROWS, W), u32),
                  pltpu.VMEM((TB * CH, W), u32))

    assert NI % 2 == 0 and NX == 4 and REC == (1, 2, 3)

    def scope2(ob, hre, dwb, semo):
        def out2(b, slot, half):
            return pltpu.make_async_copy(ob.at[pl.ds(TB * slot + NQ * half, NQ)],
                                         o_hbm.at[pl.ds(TB * b + NQ * half, NQ)], semo.at[slot])

        def out2_wait(b, slot):
            pltpu.make_async_copy(ob.at[pl.ds(TB * slot, TB)], o_hbm.at[pl.ds(TB * b, TB)], semo.at[slot]).wait()

        def conv_rec(row0, g):
            n = 8 * NREC
            x = xb[pl.ds(row0 + REC[0] - 1, NREC + 2), g].astype(f32).reshape(n + 16, W)
            a = []
            for j in range(3):
                t = None
                for i in range(3):
                    w = dwb[3 * i + j, 8 * g:8 * g + 8, :]
                    w = jnp.concatenate([jnp.concatenate([w] * NT, axis=1)] * NREC, axis=0)
                    p = x[8 * i:8 * i + n] * w
                    t = p if t is None else t + p
                a.append(t)
            cbuf[n * g:n * (g + 1), :] = _shift_r(a[0]) + a[1] + _shift_l(a[2])

        def ln_rec(k):
            cols = []
            for t in range(NT):
                c = cbuf[:, t * 128:(t + 1) * 128].reshape(G, 8 * NREC, 128)[:, 8 * k:8 * k + 8]
                cols.append(c.reshape(C, 128) * lax.rsqrt(_var1(c))[7:8])
            return jnp.concatenate(cols, axis=1).astype(bf16)

        in2(2, 2).start()
        for cp in params[2:]:
            cp.wait()
        for tap, col in enumerate(tap_columns()):
            dwb[tap] = col
        ssq = jnp.sum(acc[...].T, axis=0, keepdims=True) * (1.0 / (4.0 * GA * GA))
        gx = jnp.sqrt(ssq + 1e-6)
        nx = gx / (jnp.sum(gx, axis=1, keepdims=True) * (1.0 / E) + 1e-6)
        gam = gam_ref[...].astype(f32).reshape(1, E)
        bet = bet_ref[...].astype(f32).reshape(1, E)
        scale = (gam * nx + 1.0) * (1.0 / (2.0 * GA))
        w2f = w_ref[...].astype(f32)
        w2s[...] = _pack(w2f * scale)
        dwb[9] = jnp.broadcast_to(jnp.sum(w2f * bet, axis=1, keepdims=True), (C, 128))
        in2(0, 0).wait()

        def pass2(b, hrow):
            row0 = (b & 3) * TB
            nrow0 = ((b + 1) & 3) * TB
            oslot = b & 1

            @pl.when(b >= 2)
            def _():
                out2_wait(b - 2, oslot)

            @pl.when(b + 1 < NB)
            def _():
                in2(b + 1, (b + 1) & 3).wait()

            pending = list(range(G))
            plan = list(PLAN)

            def finish(r, hp, ngroups):
                o = jnp.dot(_unp(w2s[...]), _unp(hp), preferred_element_type=f32)
                for hf in range(2):
                    ls = slice(hf * 256, hf * 256 + 256)
                    for j in range((ngroups + 1 - hf) // 2):
                        t = 2 * hf + j
                        mark = o[0:8, t * 128:(t + 1) * 128]
                        xb[row0 + STO[0], zs[0]] = jnp.concatenate([mark] * NT, axis=1).astype(bf16)
                        conv_rec(nrow0, pending.pop(0))
                    xr = xb[row0 + r, :, :, ls].astype(f32).reshape(C, 256)
                    v = o[:, ls] + (xr + jnp.concatenate([dwb[9]] * 2, axis=1))
                    ob[oslot * TB + r, :, :, ls] = v.reshape(G, 8, 256).astype(bf16)

            def sto(k, ngroups):
                finish(STO[k], hbuf[pl.ds(pl.multiple_of(hrow + k * EH, 8), EH), :], ngroups)

            sto(0, 0)

            @pl.when(b + 3 < NB)
            def _():
                in2(b + 3, (b + 3) & 3).start()

            for k in range(NREC):
                y = jnp.dot(w1t(), ln_rec(k), preferred_element_type=f32)
                hre[k * EH:(k + 1) * EH, :] = _pack(_gelu2(y))
            for k in range(1, NSTO):
                sto(k, plan.pop(0))
            out2(b, oslot, 1).start()
            for k in range(NREC):
                finish(REC[k], hre[pl.ds(pl.multiple_of(zs[0] + k * EH, 8), EH), :], plan.pop(0))
            out2(b, oslot, 0).start()
            return hrow + NSTO * EH

        lax.fori_loop(0, NB, pass2, jnp.int32(0))
        out2_wait(NB - 2, 0)
        out2_wait(NB - 1, 1)

    pl.run_scoped(scope2,
                  pltpu.VMEM((2 * TB, G, 8, W), bf16),
                  pltpu.VMEM((NREC * EH, W), u32),
                  pltpu.VMEM((10, C, 128), f32),
                  pltpu.SemaphoreType.DMA((2,)))


@jax.jit
def pallas_standalone__modern_conv_block_convnext_v2__vision_kernel(
    x: jax.Array,
    dw: jax.Array,
    w1: jax.Array,
    w2: jax.Array,
    grn_gamma: jax.Array,
    grn_beta: jax.Array,
):
    xt = jnp.transpose(x, (0, 1, 3, 2)).reshape(H, G, 8, W)
    hbm = pl.BlockSpec(memory_space=pl.ANY)
    o = pl.pallas_call(
        _kernel,
        out_shape=jax.ShapeDtypeStruct((H, G, 8, W), bf16),
        in_specs=[hbm] * 6,
        out_specs=hbm,
        scratch_shapes=[
            pltpu.VMEM((NB * NSTO * EH, W), u32),
            pltpu.VMEM((NX * TB, G, 8, W), bf16),
            pltpu.VMEM((NREC * C, W), f32),
            pltpu.VMEM((C, 128), u32),
            pltpu.VMEM((EH, 128), u32),
            pltpu.VMEM((E, 128), f32),
            pltpu.VMEM((CH, E), u32),
            pltpu.VMEM((C, E), bf16),
            pltpu.VMEM((3, 3, C), bf16),
            pltpu.VMEM((E,), bf16),
            pltpu.VMEM((E,), bf16),
            pltpu.VMEM((PADV, 3, C), bf16),
            pltpu.SMEM((1,), jnp.int32),
            pltpu.SemaphoreType.DMA((NX,)),
            pltpu.SemaphoreType.DMA((5,)),
        ],
        compiler_params=pltpu.CompilerParams(vmem_limit_bytes=128 * 1024 * 1024,
                                             disable_bounds_checks=True),
        name="convnext",
    )(xt, dw, w1, w2.T, grn_gamma, grn_beta)
    return jnp.transpose(o.reshape(1, H, C, W), (0, 1, 3, 2))
```

```python
import math

import jax
import jax.numpy as jnp
from jax import lax
from jax.experimental import pallas as pl
from jax.experimental.pallas import tpu as pltpu

H = 512
W = 512
C = 96
E = 384
G = C // 8
NT = W // 128
TB = 8
NB = H // TB
NQ = TB // 2
REC = (1, 2, 3)
STO = tuple(r for r in range(TB) if r not in REC)
NSTO = len(STO)
NREC = len(REC)
EH = E // 2
CH = C // 2
GB = 4
SROWS = G * 24
NCH = 3
U1 = 2
R1 = TB * U1
NI = NB // U1
NX = 2 * U1
TIE = 40
PLAN = (2, 2, 2, 2, 2, 1, 1)
PADV = 7

C0 = math.sqrt(2.0 / math.pi)
C1 = 0.044715
GA = (C0 * C1) ** (1.0 / 3.0)
GK = C0 / GA
LN_EPS = 1e-5

f32 = jnp.float32
bf16 = jnp.bfloat16
u32 = jnp.uint32


def _pack(v):
    return pltpu.bitcast(v.astype(bf16), u32)


def _unp(v):
    return pltpu.bitcast(v, bf16)


def _tiles(a):
    return [a[:, t * 128:(t + 1) * 128] for t in range(NT)]


def _zero_lane(a, l):
    lane = lax.broadcasted_iota(jnp.int32, a.shape, 1)
    return jnp.where(lane == l, jnp.zeros_like(a), a)


def _shift_r(a):
    v = _tiles(a)
    m = [_zero_lane(v[0], 127)] + [jnp.concatenate([v[t][:, :127], v[t - 1][:, 127:]], axis=1)
                                   for t in range(1, NT)]
    return jnp.concatenate([pltpu.roll(u, 1, 1) for u in m], axis=1)


def _shift_l(a, edge=True):
    v = _tiles(a)
    m = ([jnp.concatenate([v[t + 1][:, :1], v[t][:, 1:]], axis=1) for t in range(NT - 1)]
         + [_zero_lane(v[NT - 1], 0) if edge else v[NT - 1]])
    return jnp.concatenate([pltpu.roll(u, 127, 1) for u in m], axis=1)


def _sums(c):
    return jnp.sum(c, axis=0), jnp.sum(c * c, axis=0)


def _merge4(a, b):
    p = jnp.concatenate([a[:4], b[4:]], axis=0)
    q = jnp.concatenate([b[:4], a[4:]], axis=0)
    return p + pltpu.roll(q, 4, 0)


def _var_from(n, shift):
    eps = LN_EPS * C * C
    return jnp.maximum(n * float(C) + eps - pltpu.roll(n * n, shift, 0), eps)


def _var2(c):
    s1, s2 = _sums(c)
    m1 = _merge4(s1[:8], s1[8:])
    m2 = _merge4(s2[:8], s2[8:])
    sub = lax.broadcasted_iota(jnp.int32, (8, 128), 0)
    n = jnp.where((sub & 2) == 0, m1 + pltpu.roll(m1, 6, 0), m2 + pltpu.roll(m2, 2, 0))
    n = n + pltpu.roll(n, 1, 0)
    return _var_from(n, 2)


def _var1(c):
    s1, s2 = _sums(c)
    n = _merge4(s1, s2)
    n = n + pltpu.roll(n, 2, 0)
    n = n + pltpu.roll(n, 1, 0)
    return _var_from(n, 4)


def _rsqrt(v):
    return jnp.exp2(jnp.log(v) * (-0.5 / math.log(2.0)))


def _gelu2(y):
    u = y * (y * y + GK)
    return y * (jnp.tanh(u) + 1.0)


def _kernel(x_hbm, dw_hbm, w1_hbm, w2t_hbm, gam_hbm, bet_hbm, o_hbm,
            hbuf, xb, cbuf, dmat, w1s, acc, w2s, w_ref, dw_ref, gam_ref, bet_ref, pad,
            zs, semx, semp):
    def xcopy(r0, n, d0, sem):
        return pltpu.make_async_copy(x_hbm.at[pl.ds(r0, n)], xb.at[pl.ds(d0, n)], sem)

    def grp_head():
        return xcopy(0, TB - 1, R1 + 1, semx.at[2])

    def grp(i, slot):
        return xcopy(R1 * i + TB - 1, R1, R1 * slot, semx.at[2 * slot])

    def grp_last():
        return xcopy(R1 * (NI - 1) + TB - 1, R1 - TB + 1, R1 * ((NI - 1) % 2), semx.at[2 * ((NI - 1) % 2)])

    def in2(b, slot):
        return xcopy(TB * b, TB, TB * slot, semx.at[slot])

    params = [pltpu.make_async_copy(src, dst, semp.at[j]) for j, (src, dst) in enumerate(
        [(dw_hbm, dw_ref), (w1_hbm, w_ref), (gam_hbm, gam_ref), (bet_hbm, bet_ref), (w2t_hbm, w_ref)])]
    for cp in params[:2] + [grp_head()] + params[2:4] + [grp(0, 0)]:
        cp.start()
    zs[0] = 0
    pad[...] = jnp.zeros_like(pad)

    def w1t(c0=0, n=E):
        return _unp(w1s[c0 // 2:(c0 + n) // 2, :])[:, :C]

    def tap_columns():
        sub = lax.broadcasted_iota(jnp.int32, (C, C), 0)
        lan = lax.broadcasted_iota(jnp.int32, (C, C), 1)
        eye = sub - lan == zs[0]
        diags = [jnp.where(eye, jnp.broadcast_to(dw_ref[i, j:j + 1, :].astype(f32), (C, C)), 0.0)
                 for i in range(3) for j in range(3)]
        ones = jnp.ones((C, 128), bf16)
        return [jnp.dot(d.astype(bf16), ones, preferred_element_type=f32) for d in diags]

    def setup():
        cols = tap_columns()
        c_ = lax.broadcasted_iota(jnp.int32, (8, 128), 0)
        k_ = lax.broadcasted_iota(jnp.int32, (8, 128), 1)
        for g in range(G):
            halves = []
            for o in range(2):
                d = jnp.zeros((8, 128), f32)
                for i in range(3):
                    ri = i + o
                    for j in range(3):
                        for jj in ((1, 2), (0,), (3,))[j]:
                            kpos = (ri // 2) * 64 + jj * 16 + (ri % 2) * 8
                            d = jnp.where(k_ == c_ + kpos, cols[i * 3 + j][8 * g:8 * g + 8], d)
                halves.append(d)
            dmat[8 * g:8 * g + 8, :] = _pack(jnp.concatenate(halves, axis=0))
        w1f = w_ref[...].astype(f32)
        w1c = w1f - jnp.sum(w1f, axis=0, keepdims=True) * (1.0 / C)
        w1c = w1c * (GA * C)
        w1p = jnp.concatenate([w1c, jnp.zeros((128 - C, E), f32)], axis=0)
        w1s[...] = _pack(w1p.T)

    def scope1(sbuf, xns):
        def build(row0, k):
            for g0 in range(0, G, GB):
                v = xb[pl.ds(row0 + 2 * k, 2), g0:g0 + GB]
                v = pltpu.bitcast(jnp.swapaxes(v, 0, 1).reshape(GB * 16, W), u32)
                lft = jnp.concatenate([pltpu.roll(u, 1, 1) for u in _tiles(v)], axis=1)
                parts = [a.reshape(GB, 8, W) for a in (lft, v, _shift_l(v, False))]
                base = (k % NQ) * SROWS + g0 * 24
                sbuf[base:base + GB * 24, :] = jnp.concatenate(parts, axis=1).reshape(GB * 24, W)

        def lane_masks():
            lane = lax.broadcasted_iota(jnp.int32, (G, 8, 128), 2)
            return lane == 0, lane > 0, lane == 127, jnp.zeros((G, 8, 128), u32)

        def conv_rhs(s0, t, masks):
            first, rest, last, zero = masks
            parts = []
            for sl in (s0, s0 + 1):
                r0 = (sl % NQ) * SROWS
                v = sbuf[r0:r0 + SROWS, t * 128:(t + 1) * 128].reshape(G, 24, 128)
                seam = zero
                if t > 0:
                    prev = sbuf[r0:r0 + SROWS, (t - 1) * 128:t * 128].reshape(G, 24, 128)
                    seam = lax.select(rest, zero, prev[:, 0:8])
                parts += [v[:, 8:16], lax.select(first, zero, v[:, 0:8]), seam,
                          lax.select(last, zero, v[:, 16:24]) if t == NT - 1 else v[:, 16:24]]
            return _unp(jnp.concatenate(parts, axis=1).reshape(G * 64, 128))

        def conv_mm(d, s, g):
            return jnp.dot(d[16 * g:16 * g + 16], s[128 * g:128 * g + 128], preferred_element_type=f32)

        def stats(s0, t, cv):
            c = jnp.concatenate(cv, axis=0).reshape(G, 16, 128)
            return (s0, t, c[:, :8].reshape(C, 128), c[:, 8:].reshape(C, 128), _var2(c))

        def norm(st, tie=None, never=None):
            s0, t, c0, c1, var = st
            if tie is not None:
                var = lax.select(never, tie, var)
            rstd = _rsqrt(var)
            r0 = rstd[3:4]
            r1 = rstd[7:8]
            ts = slice(t * 128, (t + 1) * 128)
            r = 2 * (s0 % NQ)
            xns[r * CH:(r + 1) * CH, ts] = _pack(c0 * r0)
            xns[(r + 1) * CH:(r + 2) * CH, ts] = _pack(c1 * r1)

        acc[...] = jnp.zeros_like(acc)
        xb[R1] = jnp.zeros((G, 8, W), bf16)
        params[0].wait()
        params[1].wait()
        setup()
        params[4].start()
        grp_head().wait()
        for k in range(NQ):
            build(R1, k)
        masks = lane_masks()
        d = _unp(dmat[...])
        for s0 in range(2):
            for t in range(NT):
                s = conv_rhs(s0, t, masks)
                st = stats(s0, t, [conv_mm(d, s, g) for g in range(G)])
                norm(st)
                for o in range(2):
                    if 2 * s0 + o in REC:
                        k = REC.index(2 * s0 + o)
                        for g in range(G):
                            q = 8 * (NREC * g + k)
                            cbuf[q:q + 8, t * 128:(t + 1) * 128] = st[2 + o][8 * g:8 * g + 8]

        def dma1(i, slot):
            @pl.when(i < NI - 1)
            def _():
                grp(i, slot).wait()

            @pl.when(i == NI - 1)
            def _():
                grp_last().wait()
                xb[R1 * ((NI - 1) % 2) + R1 - TB + 1] = jnp.zeros((G, 8, W), bf16)
                for b0 in range(2):
                    in2(b0, (NI % 2) * U1 + b0).start()

            @pl.when(i + 1 < NI - 1)
            def _():
                grp(i + 1, 1 - slot).start()

            @pl.when(i + 1 == NI - 1)
            def _():
                grp_last().start()

        def block1(b, row0, u, never, masks):
            n = E // NCH
            per = NT * G // (2 * NCH)
            for k in range(NQ):
                todo = [(t, g) for t in range(NT) for g in range(G)]
                d = _unp(dmat[...])
                cv = []
                pend = None
                for j in range(2 * NCH):
                    for _ in range(per):
                        t, g = todo.pop(0)
                        if g == 0:
                            s = conv_rhs(k + 2, t, masks)
                        cv.append(conv_mm(d, s, g))
                        if g == G - 1:
                            pend = stats(k + 2, t, cv)
                            cv = []
                    r, c = 2 * k + j // NCH, j % NCH
                    y = jnp.dot(w1t(c * n, n), _unp(xns[r * CH:(r + 1) * CH, :]), preferred_element_type=f32)
                    h = _gelu2(y)
                    h2 = _tiles(h * h)
                    acc[c * n:(c + 1) * n, :] = ((acc[c * n:(c + 1) * n, :] + h2[0]) + h2[1]) + (h2[2] + h2[3])
                    if r in STO:
                        row = pl.multiple_of((b * NSTO + STO.index(r)) * EH + c * (n // 2), 8)
                        hbuf[pl.ds(row, n // 2), :] = _pack(h)
                    if pend is not None:
                        norm(pend, y[TIE:TIE + 8, 0:128], never)
                        pend = None
                build(row0, u * NQ + k)

        def pass1(i, carry):
            slot = i & 1
            dma1(i, slot)
            never = lax.broadcasted_iota(jnp.int32, (8, 128), 0) < zs[0]
            masks = lane_masks()
            for u in range(U1):
                block1(i * U1 + u, slot * R1, u, never, masks)
            return carry

        lax.fori_loop(0, NI, pass1, 0)

    pl.run_scoped(scope1,
                  pltpu.VMEM((NQ * SROWS, W), u32),
                  pltpu.VMEM((TB * CH, W), u32))

    assert NI % 2 == 0 and NX == 4 and REC == (1, 2, 3)

    def scope2(ob, hre, dwb, semo):
        def out2(b, slot, half):
            return pltpu.make_async_copy(ob.at[pl.ds(TB * slot + NQ * half, NQ)],
                                         o_hbm.at[pl.ds(TB * b + NQ * half, NQ)], semo.at[slot])

        def out2_wait(b, slot):
            pltpu.make_async_copy(ob.at[pl.ds(TB * slot, TB)], o_hbm.at[pl.ds(TB * b, TB)], semo.at[slot]).wait()

        def conv_rec(row0, g):
            n = 8 * NREC
            x = xb[pl.ds(row0 + REC[0] - 1, NREC + 2), g].astype(f32).reshape(n + 16, W)
            wt = dwb[0:9, 8 * g:8 * g + 8, :].reshape(72, 128)
            a = []
            for j in range(3):
                t = None
                for i in range(3):
                    w = wt[8 * (3 * i + j):8 * (3 * i + j) + 8]
                    w = jnp.concatenate([jnp.concatenate([w] * NT, axis=1)] * NREC, axis=0)
                    p = x[8 * i:8 * i + n] * w
                    t = p if t is None else t + p
                a.append(t)
            cbuf[n * g:n * (g + 1), :] = _shift_r(a[0]) + a[1] + _shift_l(a[2])

        def ln_rec(k):
            cols = []
            for t in range(NT):
                c = cbuf[:, t * 128:(t + 1) * 128].reshape(G, 8 * NREC, 128)[:, 8 * k:8 * k + 8]
                cols.append(c.reshape(C, 128) * _rsqrt(_var1(c))[7:8])
            return jnp.concatenate(cols, axis=1).astype(bf16)

        in2(2, 2).start()
        for cp in params[2:]:
            cp.wait()
        for tap, col in enumerate(tap_columns()):
            dwb[tap] = col
        ssq = jnp.sum(acc[...].T, axis=0, keepdims=True) * (1.0 / (4.0 * GA * GA))
        gx = jnp.sqrt(ssq + 1e-6)
        nx = gx / (jnp.sum(gx, axis=1, keepdims=True) * (1.0 / E) + 1e-6)
        gam = gam_ref[...].astype(f32).reshape(1, E)
        bet = bet_ref[...].astype(f32).reshape(1, E)
        scale = (gam * nx + 1.0) * (1.0 / (2.0 * GA))
        w2f = w_ref[...].astype(f32)
        w2s[...] = _pack(w2f * scale)
        dwb[9] = jnp.broadcast_to(jnp.sum(w2f * bet, axis=1, keepdims=True), (C, 128))
        in2(0, 0).wait()

        def pass2(b, hrow):
            row0 = (b & 3) * TB
            nrow0 = ((b + 1) & 3) * TB
            oslot = b & 1

            @pl.when(b >= 2)
            def _():
                out2_wait(b - 2, oslot)

            @pl.when(b + 1 < NB)
            def _():
                in2(b + 1, (b + 1) & 3).wait()

            pending = list(range(G))
            plan = list(PLAN)

            def finish(r, hp, ngroups):
                o = jnp.dot(_unp(w2s[...]), _unp(hp), preferred_element_type=f32)
                for hf in range(2):
                    ls = slice(hf * 256, hf * 256 + 256)
                    for j in range((ngroups + 1 - hf) // 2):
                        t = 2 * hf + j
                        mark = o[0:8, t * 128:(t + 1) * 128]
                        xb[row0 + STO[0], zs[0]] = jnp.concatenate([mark] * NT, axis=1).astype(bf16)
                        conv_rec(nrow0, pending.pop(0))
                    xr = xb[row0 + r, :, :, ls].astype(f32).reshape(C, 256)
                    v = o[:, ls] + (xr + jnp.concatenate([dwb[9]] * 2, axis=1))
                    ob[oslot * TB + r, :, :, ls] = v.reshape(G, 8, 256).astype(bf16)

            def sto(k, ngroups):
                finish(STO[k], hbuf[pl.ds(pl.multiple_of(hrow + k * EH, 8), EH), :], ngroups)

            sto(0, 0)

            @pl.when(b + 3 < NB)
            def _():
                in2(b + 3, (b + 3) & 3).start()

            for k in range(NREC):
                y = jnp.dot(w1t(), ln_rec(k), preferred_element_type=f32)
                hre[k * EH:(k + 1) * EH, :] = _pack(_gelu2(y))
            for k in range(1, NSTO):
                sto(k, plan.pop(0))
            out2(b, oslot, 1).start()
            for k in range(NREC):
                finish(REC[k], hre[pl.ds(pl.multiple_of(zs[0] + k * EH, 8), EH), :], plan.pop(0))
            out2(b, oslot, 0).start()
            return hrow + NSTO * EH

        lax.fori_loop(0, NB, pass2, jnp.int32(0))
        out2_wait(NB - 2, 0)
        out2_wait(NB - 1, 1)

    pl.run_scoped(scope2,
                  pltpu.VMEM((2 * TB, G, 8, W), bf16),
                  pltpu.VMEM((NREC * EH, W), u32),
                  pltpu.VMEM((10, C, 128), f32),
                  pltpu.SemaphoreType.DMA((2,)))


@jax.jit
def pallas_standalone__modern_conv_block_convnext_v2__vision_kernel(
    x: jax.Array,
    dw: jax.Array,
    w1: jax.Array,
    w2: jax.Array,
    grn_gamma: jax.Array,
    grn_beta: jax.Array,
):
    xt = jnp.transpose(x, (0, 1, 3, 2)).reshape(H, G, 8, W)
    hbm = pl.BlockSpec(memory_space=pl.ANY)
    o = pl.pallas_call(
        _kernel,
        out_shape=jax.ShapeDtypeStruct((H, G, 8, W), bf16),
        in_specs=[hbm] * 6,
        out_specs=hbm,
        scratch_shapes=[
            pltpu.VMEM((NB * NSTO * EH, W), u32),
            pltpu.VMEM((NX * TB, G, 8, W), bf16),
            pltpu.VMEM((NREC * C, W), f32),
            pltpu.VMEM((C, 128), u32),
            pltpu.VMEM((EH, 128), u32),
            pltpu.VMEM((E, 128), f32),
            pltpu.VMEM((CH, E), u32),
            pltpu.VMEM((C, E), bf16),
            pltpu.VMEM((3, 3, C), bf16),
            pltpu.VMEM((E,), bf16),
            pltpu.VMEM((E,), bf16),
            pltpu.VMEM((PADV, 3, C), bf16),
            pltpu.SMEM((1,), jnp.int32),
            pltpu.SemaphoreType.DMA((NX,)),
            pltpu.SemaphoreType.DMA((5,)),
        ],
        compiler_params=pltpu.CompilerParams(vmem_limit_bytes=128 * 1024 * 1024,
                                             disable_bounds_checks=True),
        name="convnext",
    )(xt, dw, w1, w2.T, grn_gamma, grn_beta)
    return jnp.transpose(o.reshape(1, H, C, W), (0, 1, 3, 2))
```

```python
import math

import jax
import jax.numpy as jnp
from jax import lax
from jax.experimental import pallas as pl
from jax.experimental.pallas import tpu as pltpu

H = 512
W = 512
C = 96
E = 384
G = C // 8
NT = W // 128
TB = 8
NB = H // TB
NQ = TB // 2
REC = (1, 2, 3)
STO = tuple(r for r in range(TB) if r not in REC)
NSTO = len(STO)
NREC = len(REC)
EH = E // 2
CH = C // 2
GB = 4
SROWS = G * 24
U1 = 2
R1 = TB * U1
NI = NB // U1
NX = 2 * U1
TIE = 16
PLAN = (2, 2, 2, 2, 2, 1, 1)
SEQ1 = ((None, None, 128, None, None, 128, None, None, 128),
        (64, None, None, 128, None, None, 128, None, None, 64))
PADV = 7

C0 = math.sqrt(2.0 / math.pi)
C1 = 0.044715
GA = (C0 * C1) ** (1.0 / 3.0)
GK = C0 / GA
LN_EPS = 1e-5

f32 = jnp.float32
bf16 = jnp.bfloat16
u32 = jnp.uint32


def _row_schedule():
    events = []
    for half, seq in enumerate(SEQ1):
        start = e0 = 0
        for n in seq:
            events.append((start, half, e0, n))
            start += n or 16
            e0 += n or 0
    return [ev[1:] for ev in sorted(events, key=lambda ev: ev[:2])]


def _pack(v):
    return pltpu.bitcast(v.astype(bf16), u32)


def _unp(v):
    return pltpu.bitcast(v, bf16)


def _tiles(a):
    return [a[:, t * 128:(t + 1) * 128] for t in range(NT)]


def _zero_lane(a, l):
    lane = lax.broadcasted_iota(jnp.int32, a.shape, 1)
    return jnp.where(lane == l, jnp.zeros_like(a), a)


def _shift_r(a):
    v = _tiles(a)
    m = [_zero_lane(v[0], 127)] + [jnp.concatenate([v[t][:, :127], v[t - 1][:, 127:]], axis=1)
                                   for t in range(1, NT)]
    return jnp.concatenate([pltpu.roll(u, 1, 1) for u in m], axis=1)


def _shift_l(a, edge=True):
    v = _tiles(a)
    m = ([jnp.concatenate([v[t + 1][:, :1], v[t][:, 1:]], axis=1) for t in range(NT - 1)]
         + [_zero_lane(v[NT - 1], 0) if edge else v[NT - 1]])
    return jnp.concatenate([pltpu.roll(u, 127, 1) for u in m], axis=1)


def _sums(c):
    return jnp.sum(c, axis=0), jnp.sum(c * c, axis=0)


def _merge4(a, b):
    p = jnp.concatenate([a[:4], b[4:]], axis=0)
    q = jnp.concatenate([b[:4], a[4:]], axis=0)
    return p + pltpu.roll(q, 4, 0)


def _var_from(n, shift):
    eps = LN_EPS * C * C
    return jnp.maximum(n * float(C) + eps - pltpu.roll(n * n, shift, 0), eps)


def _var2(c):
    s1, s2 = _sums(c)
    m1 = _merge4(s1[:8], s1[8:])
    m2 = _merge4(s2[:8], s2[8:])
    sub = lax.broadcasted_iota(jnp.int32, (8, 128), 0)
    n = jnp.where((sub & 2) == 0, m1 + pltpu.roll(m1, 6, 0), m2 + pltpu.roll(m2, 2, 0))
    n = n + pltpu.roll(n, 1, 0)
    return _var_from(n, 2)


def _var1(c):
    s1, s2 = _sums(c)
    n = _merge4(s1, s2)
    n = n + pltpu.roll(n, 2, 0)
    n = n + pltpu.roll(n, 1, 0)
    return _var_from(n, 4)


def _rsqrt(v):
    return jnp.exp2(jnp.log(v) * (-0.5 / math.log(2.0)))


def _gelu2(y):
    u = y * (y * y + GK)
    return y * (jnp.tanh(u) + 1.0)


def _kernel(x_hbm, dw_hbm, w1_hbm, w2t_hbm, gam_hbm, bet_hbm, o_hbm,
            hbuf, xb, cbuf, dmat, w1s, acc, w2s, w_ref, dw_ref, gam_ref, bet_ref, pad,
            zs, semx, semp):
    def xcopy(r0, n, d0, sem):
        return pltpu.make_async_copy(x_hbm.at[pl.ds(r0, n)], xb.at[pl.ds(d0, n)], sem)

    def grp_head():
        return xcopy(0, TB - 1, R1 + 1, semx.at[2])

    def grp(i, slot):
        return xcopy(R1 * i + TB - 1, R1, R1 * slot, semx.at[2 * slot])

    def grp_last():
        return xcopy(R1 * (NI - 1) + TB - 1, R1 - TB + 1, R1 * ((NI - 1) % 2), semx.at[2 * ((NI - 1) % 2)])

    def in2(b, slot):
        return xcopy(TB * b, TB, TB * slot, semx.at[slot])

    params = [pltpu.make_async_copy(src, dst, semp.at[j]) for j, (src, dst) in enumerate(
        [(dw_hbm, dw_ref), (w1_hbm, w_ref), (gam_hbm, gam_ref), (bet_hbm, bet_ref), (w2t_hbm, w_ref)])]
    for cp in params[:2] + [grp_head()] + params[2:4] + [grp(0, 0)]:
        cp.start()
    zs[0] = 0
    pad[...] = jnp.zeros_like(pad)

    def w1t(c0=0, n=E):
        return _unp(w1s[c0 // 2:(c0 + n) // 2, :])[:, :C]

    def tap_columns():
        sub = lax.broadcasted_iota(jnp.int32, (C, C), 0)
        lan = lax.broadcasted_iota(jnp.int32, (C, C), 1)
        eye = sub - lan == zs[0]
        diags = [jnp.where(eye, jnp.broadcast_to(dw_ref[i, j:j + 1, :].astype(f32), (C, C)), 0.0)
                 for i in range(3) for j in range(3)]
        ones = jnp.ones((C, 128), bf16)
        return [jnp.dot(d.astype(bf16), ones, preferred_element_type=f32) for d in diags]

    def setup():
        cols = tap_columns()
        c_ = lax.broadcasted_iota(jnp.int32, (8, 128), 0)
        k_ = lax.broadcasted_iota(jnp.int32, (8, 128), 1)
        for g in range(G):
            halves = []
            for o in range(2):
                d = jnp.zeros((8, 128), f32)
                for i in range(3):
                    ri = i + o
                    for j in range(3):
                        for jj in ((1, 2), (0,), (3,))[j]:
                            kpos = (ri // 2) * 64 + jj * 16 + (ri % 2) * 8
                            d = jnp.where(k_ == c_ + kpos, cols[i * 3 + j][8 * g:8 * g + 8], d)
                halves.append(d)
            dmat[8 * g:8 * g + 8, :] = _pack(jnp.concatenate(halves, axis=0))
        w1f = w_ref[...].astype(f32)
        w1c = w1f - jnp.sum(w1f, axis=0, keepdims=True) * (1.0 / C)
        w1c = w1c * (GA * C)
        w1p = jnp.concatenate([w1c, jnp.zeros((128 - C, E), f32)], axis=0)
        w1s[...] = _pack(w1p.T)

    def scope1(sbuf, *xns):
        def build(row0, k):
            for g0 in range(0, G, GB):
                v = xb[pl.ds(row0 + 2 * k, 2), g0:g0 + GB]
                v = pltpu.bitcast(jnp.swapaxes(v, 0, 1).reshape(GB * 16, W), u32)
                lft = jnp.concatenate([pltpu.roll(u, 1, 1) for u in _tiles(v)], axis=1)
                parts = [a.reshape(GB, 8, W) for a in (lft, v, _shift_l(v, False))]
                base = (k % NQ) * SROWS + g0 * 24
                sbuf[base:base + GB * 24, :] = jnp.concatenate(parts, axis=1).reshape(GB * 24, W)

        def lane_masks():
            lane = lax.broadcasted_iota(jnp.int32, (G, 8, 128), 2)
            return lane == 0, lane > 0, lane == 127, jnp.zeros((G, 8, 128), u32)

        def conv_rhs(s0, t, masks):
            first, rest, last, zero = masks
            parts = []
            for sl in (s0, s0 + 1):
                r0 = (sl % NQ) * SROWS
                v = sbuf[r0:r0 + SROWS, t * 128:(t + 1) * 128].reshape(G, 24, 128)
                seam = zero
                if t > 0:
                    prev = sbuf[r0:r0 + SROWS, (t - 1) * 128:t * 128].reshape(G, 24, 128)
                    seam = lax.select(rest, zero, prev[:, 0:8])
                parts += [v[:, 8:16], lax.select(first, zero, v[:, 0:8]), seam,
                          lax.select(last, zero, v[:, 16:24]) if t == NT - 1 else v[:, 16:24]]
            return _unp(jnp.concatenate(parts, axis=1).reshape(G * 64, 128))

        def conv_mm(d, s, g):
            return jnp.dot(d[16 * g:16 * g + 16], s[128 * g:128 * g + 128], preferred_element_type=f32)

        def stats(s0, t, cv):
            c = jnp.concatenate(cv, axis=0).reshape(G, 16, 128)
            return (s0, t, c[:, :8].reshape(C, 128), c[:, 8:].reshape(C, 128), _var2(c))

        def norm(st, tie=None, never=None):
            s0, t, c0, c1, var = st
            if tie is not None:
                var = lax.select(never, tie, var)
            rstd = _rsqrt(var)
            r0 = rstd[3:4]
            r1 = rstd[7:8]
            ts = slice(t * 128, (t + 1) * 128)
            xns[s0 % NQ][0:CH, ts] = _pack(c0 * r0)
            xns[s0 % NQ][CH:2 * CH, ts] = _pack(c1 * r1)

        acc[...] = jnp.zeros_like(acc)
        xb[R1] = jnp.zeros((G, 8, W), bf16)
        params[0].wait()
        params[1].wait()
        setup()
        params[4].start()
        grp_head().wait()
        for k in range(NQ):
            build(R1, k)
        masks = lane_masks()
        d = _unp(dmat[...])
        for s0 in range(2):
            for t in range(NT):
                s = conv_rhs(s0, t, masks)
                st = stats(s0, t, [conv_mm(d, s, g) for g in range(G)])
                norm(st)
                for o in range(2):
                    if 2 * s0 + o in REC:
                        k = REC.index(2 * s0 + o)
                        for g in range(G):
                            q = 8 * (NREC * g + k)
                            cbuf[q:q + 8, t * 128:(t + 1) * 128] = st[2 + o][8 * g:8 * g + 8]

        def dma1(i, slot):
            @pl.when(i < NI - 1)
            def _():
                grp(i, slot).wait()

            @pl.when(i == NI - 1)
            def _():
                grp_last().wait()
                xb[R1 * ((NI - 1) % 2) + R1 - TB + 1] = jnp.zeros((G, 8, W), bf16)
                for b0 in range(2):
                    in2(b0, (NI % 2) * U1 + b0).start()

            @pl.when(i + 1 < NI - 1)
            def _():
                grp(i + 1, 1 - slot).start()

            @pl.when(i + 1 == NI - 1)
            def _():
                grp_last().start()

        def block1(b, row0, u, never, masks):
            for k in range(NQ):
                todo = [(t, g) for t in range(NT) for g in range(G)]
                d = _unp(dmat[...])
                cv = []
                pend = None
                for r in (2 * k, 2 * k + 1):
                    for half, e0, n in _row_schedule():
                        if n is None:
                            for _ in range(2):
                                t, g = todo.pop(0)
                                if g == 0:
                                    s = conv_rhs(k + 2, t, masks)
                                cv.append(conv_mm(d, s, g))
                                if g == G - 1:
                                    pend = stats(k + 2, t, cv)
                                    cv = []
                            continue
                        ls = slice(half * 256, half * 256 + 256)
                        xn = xns[k][pl.ds(pl.multiple_of(zs[0] + (r % 2) * CH, 8), CH), ls]
                        y = jnp.dot(w1t(e0, n), _unp(xn), preferred_element_type=f32)
                        h = _gelu2(y)
                        h2 = h * h
                        acc[e0:e0 + n, :] = (acc[e0:e0 + n, :] + h2[:, :128]) + h2[:, 128:]
                        if r in STO:
                            row = pl.multiple_of((b * NSTO + STO.index(r)) * EH + e0 // 2, 8)
                            hbuf[pl.ds(row, n // 2), ls] = _pack(h)
                        if pend is not None:
                            norm(pend, y[TIE:TIE + 8, 0:128], never)
                            pend = None
                assert pend is None and not todo
                build(row0, u * NQ + k)

        def pass1(i, carry):
            slot = i & 1
            dma1(i, slot)
            never = lax.broadcasted_iota(jnp.int32, (8, 128), 0) < zs[0]
            masks = lane_masks()
            for u in range(U1):
                block1(i * U1 + u, slot * R1, u, never, masks)
            return carry

        lax.fori_loop(0, NI, pass1, 0)

    pl.run_scoped(scope1,
                  pltpu.VMEM((NQ * SROWS, W), u32),
                  *[pltpu.VMEM((2 * CH, W), u32)] * NQ)

    assert NI % 2 == 0 and NX == 4 and REC == (1, 2, 3)

    def scope2(ob, hre, dwb, semo):
        def out2(b, slot, half):
            return pltpu.make_async_copy(ob.at[pl.ds(TB * slot + NQ * half, NQ)],
                                         o_hbm.at[pl.ds(TB * b + NQ * half, NQ)], semo.at[slot])

        def out2_wait(b, slot):
            pltpu.make_async_copy(ob.at[pl.ds(TB * slot, TB)], o_hbm.at[pl.ds(TB * b, TB)], semo.at[slot]).wait()

        def conv_rec(row0, g):
            n = 8 * NREC
            x = xb[pl.ds(row0 + REC[0] - 1, NREC + 2), g].astype(f32).reshape(n + 16, W)
            wt = dwb[0:9, 8 * g:8 * g + 8, :].reshape(72, 128)
            a = []
            for j in range(3):
                t = None
                for i in range(3):
                    w = wt[8 * (3 * i + j):8 * (3 * i + j) + 8]
                    w = jnp.concatenate([jnp.concatenate([w] * NT, axis=1)] * NREC, axis=0)
                    p = x[8 * i:8 * i + n] * w
                    t = p if t is None else t + p
                a.append(t)
            cbuf[n * g:n * (g + 1), :] = _shift_r(a[0]) + a[1] + _shift_l(a[2])

        def ln_rec(k):
            cols = []
            for t in range(NT):
                c = cbuf[:, t * 128:(t + 1) * 128].reshape(G, 8 * NREC, 128)[:, 8 * k:8 * k + 8]
                cols.append(c.reshape(C, 128) * _rsqrt(_var1(c))[7:8])
            return jnp.concatenate(cols, axis=1).astype(bf16)

        in2(2, 2).start()
        for cp in params[2:]:
            cp.wait()
        for tap, col in enumerate(tap_columns()):
            dwb[tap] = col
        ssq = jnp.sum(acc[...].T, axis=0, keepdims=True) * (1.0 / (4.0 * GA * GA))
        gx = jnp.sqrt(ssq + 1e-6)
        nx = gx / (jnp.sum(gx, axis=1, keepdims=True) * (1.0 / E) + 1e-6)
        gam = gam_ref[...].astype(f32).reshape(1, E)
        bet = bet_ref[...].astype(f32).reshape(1, E)
        scale = (gam * nx + 1.0) * (1.0 / (2.0 * GA))
        w2f = w_ref[...].astype(f32)
        w2s[...] = _pack(w2f * scale)
        dwb[9] = jnp.broadcast_to(jnp.sum(w2f * bet, axis=1, keepdims=True), (C, 128))
        in2(0, 0).wait()

        def pass2(b, hrow):
            row0 = (b & 3) * TB
            nrow0 = ((b + 1) & 3) * TB
            oslot = b & 1

            @pl.when(b >= 2)
            def _():
                out2_wait(b - 2, oslot)

            @pl.when(b + 1 < NB)
            def _():
                in2(b + 1, (b + 1) & 3).wait()

            pending = list(range(G))
            plan = list(PLAN)

            def finish(r, hp, ngroups):
                o = jnp.dot(_unp(w2s[...]), _unp(hp), preferred_element_type=f32)
                for hf in range(2):
                    ls = slice(hf * 256, hf * 256 + 256)
                    for j in range((ngroups + 1 - hf) // 2):
                        t = 2 * hf + j
                        mark = o[0:8, t * 128:(t + 1) * 128]
                        xb[row0 + STO[0], zs[0]] = jnp.concatenate([mark] * NT, axis=1).astype(bf16)
                        conv_rec(nrow0, pending.pop(0))
                    xr = xb[row0 + r, :, :, ls].astype(f32).reshape(C, 256)
                    v = o[:, ls] + (xr + jnp.concatenate([dwb[9]] * 2, axis=1))
                    ob[oslot * TB + r, :, :, ls] = v.reshape(G, 8, 256).astype(bf16)

            def sto(k, ngroups):
                finish(STO[k], hbuf[pl.ds(pl.multiple_of(hrow + k * EH, 8), EH), :], ngroups)

            sto(0, 0)

            @pl.when(b + 3 < NB)
            def _():
                in2(b + 3, (b + 3) & 3).start()

            for k in range(NREC):
                y = jnp.dot(w1t(), ln_rec(k), preferred_element_type=f32)
                hre[k * EH:(k + 1) * EH, :] = _pack(_gelu2(y))
            for k in range(1, NSTO):
                sto(k, plan.pop(0))
            out2(b, oslot, 1).start()
            for k in range(NREC):
                finish(REC[k], hre[pl.ds(pl.multiple_of(zs[0] + k * EH, 8), EH), :], plan.pop(0))
            out2(b, oslot, 0).start()
            return hrow + NSTO * EH

        lax.fori_loop(0, NB, pass2, jnp.int32(0))
        out2_wait(NB - 2, 0)
        out2_wait(NB - 1, 1)

    pl.run_scoped(scope2,
                  pltpu.VMEM((2 * TB, G, 8, W), bf16),
                  pltpu.VMEM((NREC * EH, W), u32),
                  pltpu.VMEM((10, C, 128), f32),
                  pltpu.SemaphoreType.DMA((2,)))


@jax.jit
def pallas_standalone__modern_conv_block_convnext_v2__vision_kernel(
    x: jax.Array,
    dw: jax.Array,
    w1: jax.Array,
    w2: jax.Array,
    grn_gamma: jax.Array,
    grn_beta: jax.Array,
):
    xt = jnp.transpose(x, (0, 1, 3, 2)).reshape(H, G, 8, W)
    hbm = pl.BlockSpec(memory_space=pl.ANY)
    o = pl.pallas_call(
        _kernel,
        out_shape=jax.ShapeDtypeStruct((H, G, 8, W), bf16),
        in_specs=[hbm] * 6,
        out_specs=hbm,
        scratch_shapes=[
            pltpu.VMEM((NB * NSTO * EH, W), u32),
            pltpu.VMEM((NX * TB, G, 8, W), bf16),
            pltpu.VMEM((NREC * C, W), f32),
            pltpu.VMEM((C, 128), u32),
            pltpu.VMEM((EH, 128), u32),
            pltpu.VMEM((E, 128), f32),
            pltpu.VMEM((CH, E), u32),
            pltpu.VMEM((C, E), bf16),
            pltpu.VMEM((3, 3, C), bf16),
            pltpu.VMEM((E,), bf16),
            pltpu.VMEM((E,), bf16),
            pltpu.VMEM((PADV, 3, C), bf16),
            pltpu.SMEM((1,), jnp.int32),
            pltpu.SemaphoreType.DMA((NX,)),
            pltpu.SemaphoreType.DMA((5,)),
        ],
        compiler_params=pltpu.CompilerParams(vmem_limit_bytes=128 * 1024 * 1024,
                                             disable_bounds_checks=True),
        name="convnext",
    )(xt, dw, w1, w2.T, grn_gamma, grn_beta)
    return jnp.transpose(o.reshape(1, H, C, W), (0, 1, 3, 2))
```

```python
import math

import jax
import jax.numpy as jnp
from jax import lax
from jax.experimental import pallas as pl
from jax.experimental.pallas import tpu as pltpu

H = 512
W = 512
C = 96
E = 384
G = C // 8
NT = W // 128
TB = 8
NB = H // TB
NQ = TB // 2
REC = (1, 2, 3)
STO = tuple(r for r in range(TB) if r not in REC)
NSTO = len(STO)
NREC = len(REC)
EH = E // 2
CH = C // 2
SROWS = G * 24
U1 = 2
R1 = TB * U1
NI = NB // U1
NX = 2 * U1
TIE = 16
PLAN = (2, 2, 2, 2, 2, 1, 1)
SEQ1 = ((None, None, 128, None, None, 128, None, None, 128),
        (64, None, None, 128, None, None, 128, None, None, 64))
NDEF = 12
PADV = 7

C0 = math.sqrt(2.0 / math.pi)
C1 = 0.044715
GA = (C0 * C1) ** (1.0 / 3.0)
GK = C0 / GA
LN_EPS = 1e-5

f32 = jnp.float32
bf16 = jnp.bfloat16
u32 = jnp.uint32


def _row_schedule():
    events = []
    for half, seq in enumerate(SEQ1):
        start = e0 = 0
        for n in seq:
            events.append((start, half, e0, n))
            start += n or 16
            e0 += n or 0
    return [ev[1:] for ev in sorted(events, key=lambda ev: ev[:2])]


def _pack(v):
    return pltpu.bitcast(v.astype(bf16), u32)


def _unp(v):
    return pltpu.bitcast(v, bf16)


def _tiles(a):
    return [a[:, t * 128:(t + 1) * 128] for t in range(NT)]


def _zero_lane(a, l):
    lane = lax.broadcasted_iota(jnp.int32, a.shape, 1)
    return jnp.where(lane == l, jnp.zeros_like(a), a)


def _shift_r(a):
    v = _tiles(a)
    m = [_zero_lane(v[0], 127)] + [jnp.concatenate([v[t][:, :127], v[t - 1][:, 127:]], axis=1)
                                   for t in range(1, NT)]
    return jnp.concatenate([pltpu.roll(u, 1, 1) for u in m], axis=1)


def _shift_l(a, edge=True):
    v = _tiles(a)
    m = ([jnp.concatenate([v[t + 1][:, :1], v[t][:, 1:]], axis=1) for t in range(NT - 1)]
         + [_zero_lane(v[NT - 1], 0) if edge else v[NT - 1]])
    return jnp.concatenate([pltpu.roll(u, 127, 1) for u in m], axis=1)


def _sums(c):
    return jnp.sum(c, axis=0), jnp.sum(c * c, axis=0)


def _merge4(a, b):
    p = jnp.concatenate([a[:4], b[4:]], axis=0)
    q = jnp.concatenate([b[:4], a[4:]], axis=0)
    return p + pltpu.roll(q, 4, 0)


def _var_from(n, shift):
    eps = LN_EPS * C * C
    return jnp.maximum(n * float(C) + eps - pltpu.roll(n * n, shift, 0), eps)


def _var2(c):
    s1, s2 = _sums(c)
    m1 = _merge4(s1[:8], s1[8:])
    m2 = _merge4(s2[:8], s2[8:])
    sub = lax.broadcasted_iota(jnp.int32, (8, 128), 0)
    n = jnp.where((sub & 2) == 0, m1 + pltpu.roll(m1, 6, 0), m2 + pltpu.roll(m2, 2, 0))
    n = n + pltpu.roll(n, 1, 0)
    return _var_from(n, 2)


def _var1(c):
    s1, s2 = _sums(c)
    n = _merge4(s1, s2)
    n = n + pltpu.roll(n, 2, 0)
    n = n + pltpu.roll(n, 1, 0)
    return _var_from(n, 4)


def _rsqrt(v):
    return jnp.exp2(jnp.log(v) * (-0.5 / math.log(2.0)))


def _gelu2(y):
    u = y * (y * y + GK)
    return y * (jnp.tanh(u) + 1.0)


def _kernel(x_hbm, dw_hbm, w1_hbm, w2t_hbm, gam_hbm, bet_hbm, o_hbm,
            hbuf, xb, cbuf, dmat, w1s, acc, w2s, w_ref, dw_ref, gam_ref, bet_ref, pad,
            zs, semx, semp):
    def xcopy(r0, n, d0, sem):
        return pltpu.make_async_copy(x_hbm.at[pl.ds(r0, n)], xb.at[pl.ds(d0, n)], sem)

    def grp_head():
        return xcopy(0, TB - 1, R1 + 1, semx.at[2])

    def grp(i, slot):
        return xcopy(R1 * i + TB - 1, R1, R1 * slot, semx.at[2 * slot])

    def grp_last():
        return xcopy(R1 * (NI - 1) + TB - 1, R1 - TB + 1, R1 * ((NI - 1) % 2), semx.at[2 * ((NI - 1) % 2)])

    def in2(b, slot):
        return xcopy(TB * b, TB, TB * slot, semx.at[slot])

    params = [pltpu.make_async_copy(src, dst, semp.at[j]) for j, (src, dst) in enumerate(
        [(dw_hbm, dw_ref), (w1_hbm, w_ref), (gam_hbm, gam_ref), (bet_hbm, bet_ref), (w2t_hbm, w_ref)])]
    for cp in params[:2] + [grp_head()] + params[2:4] + [grp(0, 0)]:
        cp.start()
    zs[0] = 0
    pad[...] = jnp.zeros_like(pad)

    def w1t(c0=0, n=E):
        return _unp(w1s[c0 // 2:(c0 + n) // 2, :])[:, :C]

    def tap_columns():
        sub = lax.broadcasted_iota(jnp.int32, (C, C), 0)
        lan = lax.broadcasted_iota(jnp.int32, (C, C), 1)
        eye = sub - lan == zs[0]
        diags = [jnp.where(eye, jnp.broadcast_to(dw_ref[i, j:j + 1, :].astype(f32), (C, C)), 0.0)
                 for i in range(3) for j in range(3)]
        ones = jnp.ones((C, 128), bf16)
        return [jnp.dot(d.astype(bf16), ones, preferred_element_type=f32) for d in diags]

    def setup():
        cols = tap_columns()
        c_ = lax.broadcasted_iota(jnp.int32, (8, 128), 0)
        k_ = lax.broadcasted_iota(jnp.int32, (8, 128), 1)
        for g in range(G):
            halves = []
            for o in range(2):
                d = jnp.zeros((8, 128), f32)
                for i in range(3):
                    ri = i + o
                    for j in range(3):
                        for jj in ((1, 2), (0,), (3,))[j]:
                            kpos = (ri // 2) * 64 + jj * 16 + (ri % 2) * 8
                            d = jnp.where(k_ == c_ + kpos, cols[i * 3 + j][8 * g:8 * g + 8], d)
                halves.append(d)
            dmat[8 * g:8 * g + 8, :] = _pack(jnp.concatenate(halves, axis=0))
        w1f = w_ref[...].astype(f32)
        w1c = w1f - jnp.sum(w1f, axis=0, keepdims=True) * (1.0 / C)
        w1c = w1c * (GA * C)
        w1p = jnp.concatenate([w1c, jnp.zeros((128 - C, E), f32)], axis=0)
        w1s[...] = _pack(w1p.T)

    def scope1(sbuf, ybuf, *xns):
        def build(row0, k):
            v = xb[pl.ds(row0 + 2 * k, 2)]
            v = pltpu.bitcast(jnp.swapaxes(v, 0, 1).reshape(G * 16, W), u32)
            lft = jnp.concatenate([pltpu.roll(u, 1, 1) for u in _tiles(v)], axis=1)
            parts = [a.reshape(G, 8, W) for a in (lft, v, _shift_l(v, False))]
            base = (k % NQ) * SROWS
            sbuf[base:base + SROWS, :] = jnp.concatenate(parts, axis=1).reshape(SROWS, W)

        def lane_masks():
            lane = lax.broadcasted_iota(jnp.int32, (G, 8, 128), 2)
            return lane == 0, lane > 0, lane == 127, jnp.zeros((G, 8, 128), u32)

        def conv_rhs(s0, t, masks):
            first, rest, last, zero = masks
            parts = []
            for sl in (s0, s0 + 1):
                r0 = (sl % NQ) * SROWS
                v = sbuf[r0:r0 + SROWS, t * 128:(t + 1) * 128].reshape(G, 24, 128)
                seam = zero
                if t > 0:
                    prev = sbuf[r0:r0 + SROWS, (t - 1) * 128:t * 128].reshape(G, 24, 128)
                    seam = lax.select(rest, zero, prev[:, 0:8])
                parts += [v[:, 8:16], lax.select(first, zero, v[:, 0:8]), seam,
                          lax.select(last, zero, v[:, 16:24]) if t == NT - 1 else v[:, 16:24]]
            return _unp(jnp.concatenate(parts, axis=1).reshape(G * 64, 128))

        def conv_mm(d, s, g):
            return jnp.dot(d[16 * g:16 * g + 16], s[128 * g:128 * g + 128], preferred_element_type=f32)

        def stats(s0, t, cv):
            c = jnp.concatenate(cv, axis=0).reshape(G, 16, 128)
            return (s0, t, c[:, :8].reshape(C, 128), c[:, 8:].reshape(C, 128), _var2(c))

        def norm(st, tie=None, never=None):
            s0, t, c0, c1, var = st
            if tie is not None:
                var = lax.select(never, tie, var)
            rstd = _rsqrt(var)
            r0 = rstd[3:4]
            r1 = rstd[7:8]
            ts = slice(t * 128, (t + 1) * 128)
            xns[s0 % NQ][0:CH, ts] = _pack(c0 * r0)
            xns[s0 % NQ][CH:2 * CH, ts] = _pack(c1 * r1)

        acc[...] = jnp.zeros_like(acc)
        xb[R1] = jnp.zeros((G, 8, W), bf16)
        params[0].wait()
        params[1].wait()
        setup()
        params[4].start()
        grp_head().wait()
        for k in range(NQ):
            build(R1, k)
        masks = lane_masks()
        d = _unp(dmat[...])
        for s0 in range(2):
            for t in range(NT):
                s = conv_rhs(s0, t, masks)
                st = stats(s0, t, [conv_mm(d, s, g) for g in range(G)])
                norm(st)
                for o in range(2):
                    if 2 * s0 + o in REC:
                        k = REC.index(2 * s0 + o)
                        for g in range(G):
                            q = 8 * (NREC * g + k)
                            cbuf[q:q + 8, t * 128:(t + 1) * 128] = st[2 + o][8 * g:8 * g + 8]

        def dma1(i, slot):
            @pl.when(i < NI - 1)
            def _():
                grp(i, slot).wait()

            @pl.when(i == NI - 1)
            def _():
                grp_last().wait()
                xb[R1 * ((NI - 1) % 2) + R1 - TB + 1] = jnp.zeros((G, 8, W), bf16)
                for b0 in range(2):
                    in2(b0, (NI % 2) * U1 + b0).start()

            @pl.when(i + 1 < NI - 1)
            def _():
                grp(i + 1, 1 - slot).start()

            @pl.when(i + 1 == NI - 1)
            def _():
                grp_last().start()

        def post(y, b, r, e0, half):
            n = y.shape[0]
            h = _gelu2(y)
            h2 = h * h
            a = (acc[e0:e0 + n, :] + h2[:, :128]) + h2[:, 128:]
            acc[e0:e0 + n, :] = a
            if r in STO:
                row = pl.multiple_of((b * NSTO + STO.index(r)) * EH + e0 // 2, 8)
                hbuf[pl.ds(row, n // 2), half * 256:half * 256 + 256] = _pack(h)
            return a

        cand = sorted((u, r, e0, half) for u in range(U1) for r in STO
                      for half, e0, n in _row_schedule() if n == 128)[5:]
        defer = [cand[j * len(cand) // NDEF] for j in range(NDEF)]

        def yslot(p):
            return ybuf.at[16 * (p // 2):16 * (p // 2) + 16, (p % 2) * 256:(p % 2) * 256 + 256]

        def deferred(p, i):
            u, r, e0, half = defer[p]
            return post(yslot(p)[...], i * U1 + u, r, e0 + 112, half)

        def block1(i, row0, u, never, masks, heads):
            b = i * U1 + u
            for k in range(NQ):
                todo = [(t, g) for t in range(NT) for g in range(G)]
                d = _unp(dmat[...])
                cv = []
                pend = None
                for r in (2 * k, 2 * k + 1):
                    for half, e0, n in _row_schedule():
                        if n is None:
                            for _ in range(2):
                                t, g = todo.pop(0)
                                if g == 0:
                                    s = conv_rhs(k + 2, t, masks)
                                cv.append(conv_mm(d, s, g))
                                if g == G - 1:
                                    pend = stats(k + 2, t, cv)
                                    cv = []
                            continue
                        lhs = w1s[e0 // 2:(e0 + n) // 2, :]
                        if heads:
                            q0, ties = heads.pop(0)
                            rows = [lhs[8 * q:8 * q + 8] for q in range(n // 16)]
                            for j, (nv, tie) in enumerate(ties):
                                q = q0 + j * (len(rows) - q0) // len(ties)
                                rows[q] = lax.select(nv, tie, rows[q])
                            lhs = jnp.concatenate(rows, axis=0)
                        xn = xns[k][pl.ds(pl.multiple_of(zs[0] + (r % 2) * CH, 8), CH), half * 256:half * 256 + 256]
                        y = jnp.dot(_unp(lhs)[:, :C], _unp(xn), preferred_element_type=f32)
                        if (u, r, e0, half) in defer:
                            post(y[:n - 16], b, r, e0, half)
                            yslot(defer.index((u, r, e0, half)))[...] = y[n - 16:]
                        else:
                            post(y, b, r, e0, half)
                        if pend is not None:
                            norm(pend, y[TIE:TIE + 8, 0:128], never)
                            pend = None
                assert pend is None and not todo
                build(row0, u * NQ + k)

        def pass1(i, carry):
            slot = i & 1
            dma1(i, slot)
            sub = lax.broadcasted_iota(jnp.int32, (8, 128), 0)
            masks = lane_masks()
            ties = []
            for p in range(NDEF):
                a = deferred(p, jnp.maximum(i - 1, 0))
                probe = hbuf[pl.ds(pl.multiple_of(zs[0], 8), 8), 0:128]
                ties.append((sub + p < zs[0], pltpu.bitcast(a[0:8] + a[8:16], u32) | probe))
            heads = [(1, ties[:NDEF // 4]), (0, ties[NDEF // 4:])]
            for u in range(U1):
                block1(i, slot * R1, u, sub < zs[0], masks, heads)
            return carry

        ybuf[...] = jnp.zeros_like(ybuf)
        hbuf[0:8, :] = jnp.zeros((8, W), u32)
        lax.fori_loop(0, NI, pass1, 0)
        for p in range(NDEF):
            deferred(p, NI - 1)

    pl.run_scoped(scope1,
                  pltpu.VMEM((NQ * SROWS, W), u32),
                  pltpu.VMEM((8 * NDEF, W), f32),
                  *[pltpu.VMEM((2 * CH, W), u32)] * NQ)

    assert NI % 2 == 0 and NX == 4 and REC == (1, 2, 3)

    def scope2(ob, hre, dwb, semo):
        def out2(b, slot, half):
            return pltpu.make_async_copy(ob.at[pl.ds(TB * slot + NQ * half, NQ)],
                                         o_hbm.at[pl.ds(TB * b + NQ * half, NQ)], semo.at[slot])

        def out2_wait(b, slot):
            pltpu.make_async_copy(ob.at[pl.ds(TB * slot, TB)], o_hbm.at[pl.ds(TB * b, TB)], semo.at[slot]).wait()

        def conv_rec(row0, g):
            n = 8 * NREC
            x = xb[pl.ds(row0 + REC[0] - 1, NREC + 2), g].astype(f32).reshape(n + 16, W)
            wt = dwb[0:9, 8 * g:8 * g + 8, :].reshape(72, 128)
            a = []
            for j in range(3):
                t = None
                for i in range(3):
                    w = wt[8 * (3 * i + j):8 * (3 * i + j) + 8]
                    w = jnp.concatenate([jnp.concatenate([w] * NT, axis=1)] * NREC, axis=0)
                    p = x[8 * i:8 * i + n] * w
                    t = p if t is None else t + p
                a.append(t)
            cbuf[n * g:n * (g + 1), :] = _shift_r(a[0]) + a[1] + _shift_l(a[2])

        def ln_rec(k):
            cols = []
            for t in range(NT):
                c = cbuf[:, t * 128:(t + 1) * 128].reshape(G, 8 * NREC, 128)[:, 8 * k:8 * k + 8]
                cols.append(c.reshape(C, 128) * _rsqrt(_var1(c))[7:8])
            return jnp.concatenate(cols, axis=1).astype(bf16)

        in2(2, 2).start()
        for cp in params[2:]:
            cp.wait()
        for tap, col in enumerate(tap_columns()):
            dwb[tap] = col
        ssq = jnp.sum(acc[...].T, axis=0, keepdims=True) * (1.0 / (4.0 * GA * GA))
        gx = jnp.sqrt(ssq + 1e-6)
        nx = gx / (jnp.sum(gx, axis=1, keepdims=True) * (1.0 / E) + 1e-6)
        gam = gam_ref[...].astype(f32).reshape(1, E)
        bet = bet_ref[...].astype(f32).reshape(1, E)
        scale = (gam * nx + 1.0) * (1.0 / (2.0 * GA))
        w2f = w_ref[...].astype(f32)
        w2s[...] = _pack(w2f * scale)
        dwb[9] = jnp.broadcast_to(jnp.sum(w2f * bet, axis=1, keepdims=True), (C, 128))
        in2(0, 0).wait()

        def pass2(b, hrow):
            row0 = (b & 3) * TB
            nrow0 = ((b + 1) & 3) * TB
            oslot = b & 1

            @pl.when(b >= 2)
            def _():
                out2_wait(b - 2, oslot)

            @pl.when(b + 1 < NB)
            def _():
                in2(b + 1, (b + 1) & 3).wait()

            pending = list(range(G))
            plan = list(PLAN)

            def finish(r, hp, ngroups):
                o = jnp.dot(_unp(w2s[...]), _unp(hp), preferred_element_type=f32)
                for hf in range(2):
                    ls = slice(hf * 256, hf * 256 + 256)
                    for j in range((ngroups + 1 - hf) // 2):
                        t = 2 * hf + j
                        mark = o[0:8, t * 128:(t + 1) * 128]
                        xb[row0 + STO[0], zs[0]] = jnp.concatenate([mark] * NT, axis=1).astype(bf16)
                        conv_rec(nrow0, pending.pop(0))
                    xr = xb[row0 + r, :, :, ls].astype(f32).reshape(C, 256)
                    v = o[:, ls] + (xr + jnp.concatenate([dwb[9]] * 2, axis=1))
                    ob[oslot * TB + r, :, :, ls] = v.reshape(G, 8, 256).astype(bf16)

            def sto(k, ngroups):
                finish(STO[k], hbuf[pl.ds(pl.multiple_of(hrow + k * EH, 8), EH), :], ngroups)

            sto(0, 0)

            @pl.when(b + 3 < NB)
            def _():
                in2(b + 3, (b + 3) & 3).start()

            for k in range(NREC):
                y = jnp.dot(w1t(), ln_rec(k), preferred_element_type=f32)
                hre[k * EH:(k + 1) * EH, :] = _pack(_gelu2(y))
            for k in range(1, NSTO):
                sto(k, plan.pop(0))
            out2(b, oslot, 1).start()
            for k in range(NREC):
                finish(REC[k], hre[pl.ds(pl.multiple_of(zs[0] + k * EH, 8), EH), :], plan.pop(0))
            out2(b, oslot, 0).start()
            return hrow + NSTO * EH

        lax.fori_loop(0, NB, pass2, jnp.int32(0))
        out2_wait(NB - 2, 0)
        out2_wait(NB - 1, 1)

    pl.run_scoped(scope2,
                  pltpu.VMEM((2 * TB, G, 8, W), bf16),
                  pltpu.VMEM((NREC * EH, W), u32),
                  pltpu.VMEM((10, C, 128), f32),
                  pltpu.SemaphoreType.DMA((2,)))


@jax.jit
def pallas_standalone__modern_conv_block_convnext_v2__vision_kernel(
    x: jax.Array,
    dw: jax.Array,
    w1: jax.Array,
    w2: jax.Array,
    grn_gamma: jax.Array,
    grn_beta: jax.Array,
):
    xt = jnp.transpose(x, (0, 1, 3, 2)).reshape(H, G, 8, W)
    hbm = pl.BlockSpec(memory_space=pl.ANY)
    o = pl.pallas_call(
        _kernel,
        out_shape=jax.ShapeDtypeStruct((H, G, 8, W), bf16),
        in_specs=[hbm] * 6,
        out_specs=hbm,
        scratch_shapes=[
            pltpu.VMEM((NB * NSTO * EH, W), u32),
            pltpu.VMEM((NX * TB, G, 8, W), bf16),
            pltpu.VMEM((NREC * C, W), f32),
            pltpu.VMEM((C, 128), u32),
            pltpu.VMEM((EH, 128), u32),
            pltpu.VMEM((E, 128), f32),
            pltpu.VMEM((CH, E), u32),
            pltpu.VMEM((C, E), bf16),
            pltpu.VMEM((3, 3, C), bf16),
            pltpu.VMEM((E,), bf16),
            pltpu.VMEM((E,), bf16),
            pltpu.VMEM((PADV, 3, C), bf16),
            pltpu.SMEM((1,), jnp.int32),
            pltpu.SemaphoreType.DMA((NX,)),
            pltpu.SemaphoreType.DMA((5,)),
        ],
        compiler_params=pltpu.CompilerParams(vmem_limit_bytes=128 * 1024 * 1024,
                                             disable_bounds_checks=True),
        name="convnext",
    )(xt, dw, w1, w2.T, grn_gamma, grn_beta)
    return jnp.transpose(o.reshape(1, H, C, W), (0, 1, 3, 2))
```

```python
import math

import jax
import jax.numpy as jnp
from jax import lax
from jax.experimental import pallas as pl
from jax.experimental.pallas import tpu as pltpu

H = 512
W = 512
C = 96
E = 384
G = C // 8
NT = W // 128
TB = 8
NB = H // TB
NQ = TB // 2
REC = (1, 2, 3)
STO = tuple(r for r in range(TB) if r not in REC)
NSTO = len(STO)
NREC = len(REC)
EH = E // 2
CH = C // 2
SROWS = G * 24
U1 = 2
R1 = TB * U1
NI = NB // U1
NX = 2 * U1
TIE = 16
PLAN = (2, 2, 2, 2, 2, 1, 1)
SEQ1 = ((None, None, 128, None, None, 128, None, None, 128),
        (64, None, None, 128, None, None, 128, None, None, 64))
NDEF = 16
PADV = 7

C0 = math.sqrt(2.0 / math.pi)
C1 = 0.044715
GA = (C0 * C1) ** (1.0 / 3.0)
GK = C0 / GA
LN_EPS = 1e-5

f32 = jnp.float32
bf16 = jnp.bfloat16
u32 = jnp.uint32


def _row_schedule():
    events = []
    for half, seq in enumerate(SEQ1):
        start = e0 = 0
        for n in seq:
            events.append((start, half, e0, n))
            start += n or 16
            e0 += n or 0
    return [ev[1:] for ev in sorted(events, key=lambda ev: ev[:2])]


def _pack(v):
    return pltpu.bitcast(v.astype(bf16), u32)


def _unp(v):
    return pltpu.bitcast(v, bf16)


def _tiles(a):
    return [a[:, t * 128:(t + 1) * 128] for t in range(NT)]


def _zero_lane(a, l):
    lane = lax.broadcasted_iota(jnp.int32, a.shape, 1)
    return jnp.where(lane == l, jnp.zeros_like(a), a)


def _shift_r(a):
    v = _tiles(a)
    m = [_zero_lane(v[0], 127)] + [jnp.concatenate([v[t][:, :127], v[t - 1][:, 127:]], axis=1)
                                   for t in range(1, NT)]
    return jnp.concatenate([pltpu.roll(u, 1, 1) for u in m], axis=1)


def _shift_l(a, edge=True):
    v = _tiles(a)
    m = ([jnp.concatenate([v[t + 1][:, :1], v[t][:, 1:]], axis=1) for t in range(NT - 1)]
         + [_zero_lane(v[NT - 1], 0) if edge else v[NT - 1]])
    return jnp.concatenate([pltpu.roll(u, 127, 1) for u in m], axis=1)


def _sums(c):
    return jnp.sum(c, axis=0), jnp.sum(c * c, axis=0)


def _merge4(a, b):
    p = jnp.concatenate([a[:4], b[4:]], axis=0)
    q = jnp.concatenate([b[:4], a[4:]], axis=0)
    return p + pltpu.roll(q, 4, 0)


def _var_from(n, shift):
    eps = LN_EPS * C * C
    return jnp.maximum(n * float(C) + eps - pltpu.roll(n * n, shift, 0), eps)


def _var2(c):
    s1, s2 = _sums(c)
    m1 = _merge4(s1[:8], s1[8:])
    m2 = _merge4(s2[:8], s2[8:])
    sub = lax.broadcasted_iota(jnp.int32, (8, 128), 0)
    n = jnp.where((sub & 2) == 0, m1 + pltpu.roll(m1, 6, 0), m2 + pltpu.roll(m2, 2, 0))
    n = n + pltpu.roll(n, 1, 0)
    return _var_from(n, 2)


def _var1(c):
    s1, s2 = _sums(c)
    n = _merge4(s1, s2)
    n = n + pltpu.roll(n, 2, 0)
    n = n + pltpu.roll(n, 1, 0)
    return _var_from(n, 4)


def _rsqrt(v):
    return jnp.exp2(jnp.log(v) * (-0.5 / math.log(2.0)))


def _gelu2(y):
    u = y * (y * y + GK)
    return y * (jnp.tanh(u) + 1.0)


def _kernel(x_hbm, dw_hbm, w1_hbm, w2t_hbm, gam_hbm, bet_hbm, o_hbm,
            hbuf, xb, cbuf, dmat, w1s, acc, w2s, w_ref, dw_ref, gam_ref, bet_ref, pad,
            zs, semx, semp):
    def xcopy(r0, n, d0, sem):
        return pltpu.make_async_copy(x_hbm.at[pl.ds(r0, n)], xb.at[pl.ds(d0, n)], sem)

    def grp_head():
        return xcopy(0, TB - 1, R1 + 1, semx.at[2])

    def grp(i, slot):
        return xcopy(R1 * i + TB - 1, R1, R1 * slot, semx.at[2 * slot])

    def grp_last():
        return xcopy(R1 * (NI - 1) + TB - 1, R1 - TB + 1, R1 * ((NI - 1) % 2), semx.at[2 * ((NI - 1) % 2)])

    def in2(b, slot):
        return xcopy(TB * b, TB, TB * slot, semx.at[slot])

    params = [pltpu.make_async_copy(src, dst, semp.at[j]) for j, (src, dst) in enumerate(
        [(dw_hbm, dw_ref), (w1_hbm, w_ref), (gam_hbm, gam_ref), (bet_hbm, bet_ref), (w2t_hbm, w_ref)])]
    for cp in params[:2] + [grp_head()] + params[2:4] + [grp(0, 0)]:
        cp.start()
    zs[0] = 0
    pad[...] = jnp.zeros_like(pad)

    def w1t(c0=0, n=E):
        return _unp(w1s[c0 // 2:(c0 + n) // 2, :])[:, :C]

    def tap_columns():
        sub = lax.broadcasted_iota(jnp.int32, (C, C), 0)
        lan = lax.broadcasted_iota(jnp.int32, (C, C), 1)
        eye = sub - lan == zs[0]
        diags = [jnp.where(eye, jnp.broadcast_to(dw_ref[i, j:j + 1, :].astype(f32), (C, C)), 0.0)
                 for i in range(3) for j in range(3)]
        ones = jnp.ones((C, 128), bf16)
        return [jnp.dot(d.astype(bf16), ones, preferred_element_type=f32) for d in diags]

    def setup():
        cols = tap_columns()
        c_ = lax.broadcasted_iota(jnp.int32, (8, 128), 0)
        k_ = lax.broadcasted_iota(jnp.int32, (8, 128), 1)
        for g in range(G):
            halves = []
            for o in range(2):
                d = jnp.zeros((8, 128), f32)
                for i in range(3):
                    ri = i + o
                    for j in range(3):
                        for jj in ((1, 2), (0,), (3,))[j]:
                            kpos = (ri // 2) * 64 + jj * 16 + (ri % 2) * 8
                            d = jnp.where(k_ == c_ + kpos, cols[i * 3 + j][8 * g:8 * g + 8], d)
                halves.append(d)
            dmat[8 * g:8 * g + 8, :] = _pack(jnp.concatenate(halves, axis=0))
        w1f = w_ref[...].astype(f32)
        w1c = w1f - jnp.sum(w1f, axis=0, keepdims=True) * (1.0 / C)
        w1c = w1c * (GA * C)
        w1p = jnp.concatenate([w1c, jnp.zeros((128 - C, E), f32)], axis=0)
        w1s[...] = _pack(w1p.T)

    def scope1(sbuf, ybuf, *xns):
        def build(row0, k):
            v = xb[pl.ds(row0 + 2 * k, 2)]
            v = pltpu.bitcast(jnp.swapaxes(v, 0, 1).reshape(G * 16, W), u32)
            lft = jnp.concatenate([pltpu.roll(u, 1, 1) for u in _tiles(v)], axis=1)
            parts = [a.reshape(G, 8, W) for a in (lft, v, _shift_l(v, False))]
            base = (k % NQ) * SROWS
            sbuf[base:base + SROWS, :] = jnp.concatenate(parts, axis=1).reshape(SROWS, W)

        def lane_masks():
            lane = lax.broadcasted_iota(jnp.int32, (G, 8, 128), 2)
            return lane == 0, lane > 0, lane == 127, jnp.zeros((G, 8, 128), u32)

        def conv_rhs(s0, t, masks):
            first, rest, last, zero = masks
            parts = []
            for sl in (s0, s0 + 1):
                r0 = (sl % NQ) * SROWS
                v = sbuf[r0:r0 + SROWS, t * 128:(t + 1) * 128].reshape(G, 24, 128)
                seam = zero
                if t > 0:
                    prev = sbuf[r0:r0 + SROWS, (t - 1) * 128:t * 128].reshape(G, 24, 128)
                    seam = lax.select(rest, zero, prev[:, 0:8])
                parts += [v[:, 8:16], lax.select(first, zero, v[:, 0:8]), seam,
                          lax.select(last, zero, v[:, 16:24]) if t == NT - 1 else v[:, 16:24]]
            return _unp(jnp.concatenate(parts, axis=1).reshape(G * 64, 128))

        def conv_mm(d, s, g):
            return jnp.dot(d[16 * g:16 * g + 16], s[128 * g:128 * g + 128], preferred_element_type=f32)

        def stats(s0, t, cv):
            c = jnp.concatenate(cv, axis=0).reshape(G, 16, 128)
            return (s0, t, c[:, :8].reshape(C, 128), c[:, 8:].reshape(C, 128), _var2(c))

        def norm(st, tie=None, never=None):
            s0, t, c0, c1, var = st
            if tie is not None:
                var = lax.select(never, tie, var)
            rstd = _rsqrt(var)
            r0 = rstd[3:4]
            r1 = rstd[7:8]
            ts = slice(t * 128, (t + 1) * 128)
            xns[s0 % NQ][0:CH, ts] = _pack(c0 * r0)
            xns[s0 % NQ][CH:2 * CH, ts] = _pack(c1 * r1)

        acc[...] = jnp.zeros_like(acc)
        xb[R1] = jnp.zeros((G, 8, W), bf16)
        params[0].wait()
        params[1].wait()
        setup()
        params[4].start()
        grp_head().wait()
        for k in range(NQ):
            build(R1, k)
        masks = lane_masks()
        d = _unp(dmat[...])
        for s0 in range(2):
            for t in range(NT):
                s = conv_rhs(s0, t, masks)
                st = stats(s0, t, [conv_mm(d, s, g) for g in range(G)])
                norm(st)
                for o in range(2):
                    if 2 * s0 + o in REC:
                        k = REC.index(2 * s0 + o)
                        for g in range(G):
                            q = 8 * (NREC * g + k)
                            cbuf[q:q + 8, t * 128:(t + 1) * 128] = st[2 + o][8 * g:8 * g + 8]

        def dma1(i, slot):
            @pl.when(i < NI - 1)
            def _():
                grp(i, slot).wait()

            @pl.when(i == NI - 1)
            def _():
                grp_last().wait()
                xb[R1 * ((NI - 1) % 2) + R1 - TB + 1] = jnp.zeros((G, 8, W), bf16)
                for b0 in range(2):
                    in2(b0, (NI % 2) * U1 + b0).start()

            @pl.when(i + 1 < NI - 1)
            def _():
                grp(i + 1, 1 - slot).start()

            @pl.when(i + 1 == NI - 1)
            def _():
                grp_last().start()

        def post(y, b, r, e0, half):
            n = y.shape[0]
            h = _gelu2(y)
            h2 = h * h
            a = (acc[e0:e0 + n, :] + h2[:, :128]) + h2[:, 128:]
            acc[e0:e0 + n, :] = a
            if r in STO:
                row = pl.multiple_of((b * NSTO + STO.index(r)) * EH + e0 // 2, 8)
                hbuf[pl.ds(row, n // 2), half * 256:half * 256 + 256] = _pack(h)
            return a

        cand = sorted((u, r, e0, half) for u in range(U1) for r in STO
                      for half, e0, n in _row_schedule() if n == 128)[5:]
        defer = [cand[j * len(cand) // (NDEF - 4)] + (112,) for j in range(NDEF - 4)]
        final = {half: (e0, n) for half, e0, n in _row_schedule() if n}
        defer += [(U1 - 1, TB - 1, final[half][0], half, final[half][1] - back)
                  for back in (16, 32) for half in range(2)]

        def yslot(p):
            return ybuf.at[16 * (p // 2):16 * (p // 2) + 16, (p % 2) * 256:(p % 2) * 256 + 256]

        def deferred(p, i):
            u, r, e0, half, off = defer[p]
            return post(yslot(p)[...], i * U1 + u, r, e0 + off, half)

        def block1(i, row0, u, never, masks, heads):
            b = i * U1 + u
            for k in range(NQ):
                todo = [(t, g) for t in range(NT) for g in range(G)]
                d = _unp(dmat[...])
                cv = []
                pend = None
                for r in (2 * k, 2 * k + 1):
                    for half, e0, n in _row_schedule():
                        if n is None:
                            for _ in range(2):
                                t, g = todo.pop(0)
                                if g == 0:
                                    s = conv_rhs(k + 2, t, masks)
                                cv.append(conv_mm(d, s, g))
                                if g == G - 1:
                                    pend = stats(k + 2, t, cv)
                                    cv = []
                            continue
                        lhs = w1s[e0 // 2:(e0 + n) // 2, :]
                        if heads:
                            q0, ties = heads.pop(0)
                            rows = [lhs[8 * q:8 * q + 8] for q in range(n // 16)]
                            for j, (nv, tie) in enumerate(ties):
                                q = q0 + j * (len(rows) - q0) // len(ties)
                                rows[q] = lax.select(nv, tie, rows[q])
                            lhs = jnp.concatenate(rows, axis=0)
                        xn = xns[k][pl.ds(pl.multiple_of(zs[0] + (r % 2) * CH, 8), CH), half * 256:half * 256 + 256]
                        y = jnp.dot(_unp(lhs)[:, :C], _unp(xn), preferred_element_type=f32)
                        later = [p for p in range(NDEF) if defer[p][:4] == (u, r, e0, half)]
                        post(y[:n - 16 * len(later)], b, r, e0, half)
                        for p in later:
                            yslot(p)[...] = y[defer[p][4]:defer[p][4] + 16]
                        if pend is not None:
                            norm(pend, y[TIE:TIE + 8, 0:128], never)
                            pend = None
                assert pend is None and not todo
                build(row0, u * NQ + k)

        def pass1(i, carry):
            slot = i & 1
            dma1(i, slot)
            sub = lax.broadcasted_iota(jnp.int32, (8, 128), 0)
            masks = lane_masks()
            ties = []
            for p in range(NDEF):
                a = deferred(p, jnp.maximum(i - 1, 0))
                probe = hbuf[pl.ds(pl.multiple_of(zs[0], 8), 8), 0:128]
                ties.append((sub + p < zs[0], pltpu.bitcast(a[0:8] + a[8:16], u32) | probe))
            heads = [(1, ties[:3]), (0, ties[3:])]
            for u in range(U1):
                block1(i, slot * R1, u, sub < zs[0], masks, heads)
            return carry

        ybuf[...] = jnp.zeros_like(ybuf)
        hbuf[0:8, :] = jnp.zeros((8, W), u32)
        lax.fori_loop(0, NI, pass1, 0)
        for p in range(NDEF):
            deferred(p, NI - 1)

    pl.run_scoped(scope1,
                  pltpu.VMEM((NQ * SROWS, W), u32),
                  pltpu.VMEM((8 * NDEF, W), f32),
                  *[pltpu.VMEM((2 * CH, W), u32)] * NQ)

    assert NI % 2 == 0 and NX == 4 and REC == (1, 2, 3)

    def scope2(ob, hre, dwb, semo):
        def out2(b, slot, half):
            return pltpu.make_async_copy(ob.at[pl.ds(TB * slot + NQ * half, NQ)],
                                         o_hbm.at[pl.ds(TB * b + NQ * half, NQ)], semo.at[slot])

        def out2_wait(b, slot):
            pltpu.make_async_copy(ob.at[pl.ds(TB * slot, TB)], o_hbm.at[pl.ds(TB * b, TB)], semo.at[slot]).wait()

        def conv_rec(row0, g):
            n = 8 * NREC
            x = xb[pl.ds(row0 + REC[0] - 1, NREC + 2), g].astype(f32).reshape(n + 16, W)
            wt = dwb[0:9, 8 * g:8 * g + 8, :].reshape(72, 128)
            a = []
            for j in range(3):
                t = None
                for i in range(3):
                    w = wt[8 * (3 * i + j):8 * (3 * i + j) + 8]
                    w = jnp.concatenate([jnp.concatenate([w] * NT, axis=1)] * NREC, axis=0)
                    p = x[8 * i:8 * i + n] * w
                    t = p if t is None else t + p
                a.append(t)
            cbuf[n * g:n * (g + 1), :] = _shift_r(a[0]) + a[1] + _shift_l(a[2])

        def ln_rec(k):
            cols = []
            for t in range(NT):
                c = cbuf[:, t * 128:(t + 1) * 128].reshape(G, 8 * NREC, 128)[:, 8 * k:8 * k + 8]
                cols.append(c.reshape(C, 128) * _rsqrt(_var1(c))[7:8])
            return jnp.concatenate(cols, axis=1).astype(bf16)

        in2(2, 2).start()
        for cp in params[2:]:
            cp.wait()
        for tap, col in enumerate(tap_columns()):
            dwb[tap] = col
        ssq = jnp.sum(acc[...].T, axis=0, keepdims=True) * (1.0 / (4.0 * GA * GA))
        gx = jnp.sqrt(ssq + 1e-6)
        nx = gx / (jnp.sum(gx, axis=1, keepdims=True) * (1.0 / E) + 1e-6)
        gam = gam_ref[...].astype(f32).reshape(1, E)
        bet = bet_ref[...].astype(f32).reshape(1, E)
        scale = (gam * nx + 1.0) * (1.0 / (2.0 * GA))
        w2f = w_ref[...].astype(f32)
        w2s[...] = _pack(w2f * scale)
        dwb[9] = jnp.broadcast_to(jnp.sum(w2f * bet, axis=1, keepdims=True), (C, 128))
        in2(0, 0).wait()

        def pass2(b, hrow):
            row0 = (b & 3) * TB
            nrow0 = ((b + 1) & 3) * TB
            oslot = b & 1

            @pl.when(b >= 2)
            def _():
                out2_wait(b - 2, oslot)

            @pl.when(b + 1 < NB)
            def _():
                in2(b + 1, (b + 1) & 3).wait()

            pending = list(range(G))
            plan = list(PLAN)

            def finish(r, hp, ngroups):
                o = jnp.dot(_unp(w2s[...]), _unp(hp), preferred_element_type=f32)
                for hf in range(2):
                    ls = slice(hf * 256, hf * 256 + 256)
                    for j in range((ngroups + 1 - hf) // 2):
                        t = 2 * hf + j
                        mark = o[0:8, t * 128:(t + 1) * 128]
                        xb[row0 + STO[0], zs[0]] = jnp.concatenate([mark] * NT, axis=1).astype(bf16)
                        conv_rec(nrow0, pending.pop(0))
                    xr = xb[row0 + r, :, :, ls].astype(f32).reshape(C, 256)
                    v = o[:, ls] + (xr + jnp.concatenate([dwb[9]] * 2, axis=1))
                    ob[oslot * TB + r, :, :, ls] = v.reshape(G, 8, 256).astype(bf16)

            def sto(k, ngroups):
                finish(STO[k], hbuf[pl.ds(pl.multiple_of(hrow + k * EH, 8), EH), :], ngroups)

            sto(0, 0)

            @pl.when(b + 3 < NB)
            def _():
                in2(b + 3, (b + 3) & 3).start()

            for k in range(NREC):
                y = jnp.dot(w1t(), ln_rec(k), preferred_element_type=f32)
                hre[k * EH:(k + 1) * EH, :] = _pack(_gelu2(y))
            for k in range(1, NSTO):
                sto(k, plan.pop(0))
            out2(b, oslot, 1).start()
            for k in range(NREC):
                finish(REC[k], hre[pl.ds(pl.multiple_of(zs[0] + k * EH, 8), EH), :], plan.pop(0))
            out2(b, oslot, 0).start()
            return hrow + NSTO * EH

        lax.fori_loop(0, NB, pass2, jnp.int32(0))
        out2_wait(NB - 2, 0)
        out2_wait(NB - 1, 1)

    pl.run_scoped(scope2,
                  pltpu.VMEM((2 * TB, G, 8, W), bf16),
                  pltpu.VMEM((NREC * EH, W), u32),
                  pltpu.VMEM((10, C, 128), f32),
                  pltpu.SemaphoreType.DMA((2,)))


@jax.jit
def pallas_standalone__modern_conv_block_convnext_v2__vision_kernel(
    x: jax.Array,
    dw: jax.Array,
    w1: jax.Array,
    w2: jax.Array,
    grn_gamma: jax.Array,
    grn_beta: jax.Array,
):
    xt = jnp.transpose(x, (0, 1, 3, 2)).reshape(H, G, 8, W)
    hbm = pl.BlockSpec(memory_space=pl.ANY)
    o = pl.pallas_call(
        _kernel,
        out_shape=jax.ShapeDtypeStruct((H, G, 8, W), bf16),
        in_specs=[hbm] * 6,
        out_specs=hbm,
        scratch_shapes=[
            pltpu.VMEM((NB * NSTO * EH, W), u32),
            pltpu.VMEM((NX * TB, G, 8, W), bf16),
            pltpu.VMEM((NREC * C, W), f32),
            pltpu.VMEM((C, 128), u32),
            pltpu.VMEM((EH, 128), u32),
            pltpu.VMEM((E, 128), f32),
            pltpu.VMEM((CH, E), u32),
            pltpu.VMEM((C, E), bf16),
            pltpu.VMEM((3, 3, C), bf16),
            pltpu.VMEM((E,), bf16),
            pltpu.VMEM((E,), bf16),
            pltpu.VMEM((PADV, 3, C), bf16),
            pltpu.SMEM((1,), jnp.int32),
            pltpu.SemaphoreType.DMA((NX,)),
            pltpu.SemaphoreType.DMA((5,)),
        ],
        compiler_params=pltpu.CompilerParams(vmem_limit_bytes=128 * 1024 * 1024,
                                             disable_bounds_checks=True),
        name="convnext",
    )(xt, dw, w1, w2.T, grn_gamma, grn_beta)
    return jnp.transpose(o.reshape(1, H, C, W), (0, 1, 3, 2))
```
